```python
import jax
import jax.numpy as jnp

def _softmax(x, axis=-1):
    return jax.nn.softmax(x, axis=axis)
def _gelu(x):
    return jax.nn.gelu(x, approximate=True)
def _silu(x):
    return jax.nn.silu(x)
def _sigmoid(x):
    return jax.nn.sigmoid(x)
def _layernorm(x, axis=-1, eps=1e-5):
    m = jnp.mean(x, axis=axis, keepdims=True)
    v = jnp.var(x, axis=axis, keepdims=True)
    return (x - m) / jnp.sqrt(v + eps)
def _scatter_add(tgt, idx, src, axis=0):
    return tgt.at[idx].add(src)
def _segment_sum(src, seg, n):
    return jax.ops.segment_sum(src, seg, n)
class _Rng:
    def __init__(self, key):
        self._k = key
    def _next(self):
        self._k, sub = jax.random.split(self._k)
        return sub
    def normal(self, shape):
        return jax.random.normal(self._next(), shape, dtype=jnp.bfloat16)
    def randint(self, lo, hi, shape):
        return jax.random.randint(self._next(), shape, lo, hi, dtype=jnp.int32)
    def uniform(self, shape, lo=0.0, hi=1.0):
        return jax.random.uniform(self._next(), shape, jnp.bfloat16, lo, hi)
    def permutation(self, n):
        return jax.random.permutation(self._next(), n)


kernel_name = 'sequential_preLN__compressed_kv_cla__moe_arch_mod__prompt'

def setup_inputs():
    _rng = _Rng(jax.random.key(int.from_bytes(__import__("os").urandom(4), "little")))
    _w = (lambda a: (lambda t: t.astype(jnp.bfloat16) if jnp.issubdtype(t.dtype, jnp.floating) else t)(jnp.asarray(a)))
    def _A_setup():
        B, H, Sq, Sk, D, M = 1, 32, 2048, 2048, 128, 1024
        Dc = 4 * D
        return {
            "x": _w((lambda *s: _rng.normal(s) * 0.05)(B, Sq, M)),
            "c_kv": _w((lambda *s: _rng.normal(s) * 0.05)(B, Sk, Dc)),
            "w_q": _w((lambda *s: _rng.normal(s) * 0.05)(M, H, D) * (M ** -0.5)),
            "w_uk": _w((lambda *s: _rng.normal(s) * 0.05)(Dc, H, D) * (Dc ** -0.5)),
            "w_uv": _w((lambda *s: _rng.normal(s) * 0.05)(Dc, H, D) * (Dc ** -0.5)),
            "w_o": _w((lambda *s: _rng.normal(s) * 0.05)(H, D, M) * ((H * D) ** -0.5)),
        }
    _A_in = _A_setup()

    def _B_setup():
        B, S, D, F, C = 1, 2048, 1024, 3584, 2
        return {
            "x": _w((lambda *s: _rng.normal(s) * 0.05)(B, S, D)),
            "w_r": _w((lambda *s: _rng.normal(s) * 0.05)(D)),
            "w_gate": _w((lambda *s: _rng.normal(s) * 0.05)(D, F)),
            "w_up": _w((lambda *s: _rng.normal(s) * 0.05)(D, F)),
            "w_down": _w((lambda *s: _rng.normal(s) * 0.05)(F, D)),
        }
    _B_in = _B_setup()

    return {
        "A_x": _A_in["x"],
        "A_c_kv": _A_in["c_kv"],
        "A_w_q": _A_in["w_q"],
        "A_w_uk": _A_in["w_uk"],
        "A_w_uv": _A_in["w_uv"],
        "A_w_o": _A_in["w_o"],
        "B_x": _B_in["x"],
        "B_w_r": _B_in["w_r"],
        "B_w_gate": _B_in["w_gate"],
        "B_w_up": _B_in["w_up"],
        "B_w_down": _B_in["w_down"],
    }

def reference(A_x, A_c_kv, A_w_q, A_w_uk, A_w_uv, A_w_o, B_x, B_w_r, B_w_gate, B_w_up, B_w_down):
    def _A_ref(x, c_kv, w_q, w_uk, w_uv, w_o):
        B, Sq, M = x.shape[0], x.shape[1], x.shape[2]
        Sk = c_kv.shape[1]
        H, D = w_q.shape[1], w_q.shape[2]
        q = jnp.einsum("bqm,mhd->bhqd", x, w_q)
        k = jnp.einsum("bkc,chd->bhkd", c_kv, w_uk)
        v = jnp.einsum("bkc,chd->bhkd", c_kv, w_uv)
        scores = jnp.einsum("bhqd,bhkd->bhqk", q, k) * (D ** -0.5)
        off = Sk - Sq
        qi = jnp.arange(Sq)[:, None]
        kj = jnp.arange(Sk)[None, :]
        cmask = kj <= (qi + off)
        scores = jnp.where(cmask[None, None], scores, -1e9)
        p = _softmax(scores, axis=-1)
        ctx = jnp.einsum("bhqk,bhkd->bhqd", p, v)
        return jnp.einsum("bhqd,hdm->bqm", ctx, w_o)

    def _B_ref(x, w_r, w_gate, w_up, w_down):
        B, S, D = x.shape
        C = 2
        r = x @ w_r
        idx = jnp.argsort(-r, axis=-1)[:, :C]
        idx_e = jnp.repeat(idx.reshape(B, C, 1), D, axis=2)
        x_sel = jnp.take_along_axis(x, idx_e, axis=1)
        g = _silu(x_sel @ w_gate)
        u = x_sel @ w_up
        y = (g * u) @ w_down
        r_sel = _sigmoid(jnp.take_along_axis(r, idx, axis=1))
        y = y * r_sel.reshape(B, C, 1)
        b_off = (jnp.arange(B) * S).reshape(B, 1)
        flat_idx = (idx + b_off).reshape(B * C)
        zero = (x * 0.0).reshape(B * S, D)
        upd = _scatter_add(zero, flat_idx, y.reshape(B * C, D), axis=0)
        return x + upd.reshape(B, S, D)

    x = A_x
    h = x + _A_ref(_layernorm(x, axis=-1), A_c_kv, A_w_q, A_w_uk, A_w_uv, A_w_o)
    h2 = h + _B_ref(_layernorm(h, axis=-1), B_w_r, B_w_gate, B_w_up, B_w_down)
    return h2
```

```python
import functools
import math
import jax
import jax.numpy as jnp
from jax import lax
from jax.experimental import pallas as pl
from jax.experimental.pallas import tpu as pltpu

BF = jnp.bfloat16
F32 = jnp.float32
NT = (((1,), (1,)), ((), ()))
NEG = -1e30
EPS = 1e-5

CFG = dict(TQ=256, TE=256, order="desc")


def _rb(x):
    return x.astype(BF).astype(F32)


def _ln_rows(x):
    n = x.shape[-1]
    mu = jnp.sum(x, axis=-1, keepdims=True) * (1.0 / n)
    xc = x - mu
    var = jnp.sum(xc * xc, axis=-1, keepdims=True) * (1.0 / n)
    den = _rb(jnp.sqrt(_rb(_rb(var) + EPS)))
    num = _rb(x - _rb(mu))
    return (num / den).astype(BF)


def make(cfg):
    TQ, TE = cfg["TQ"], cfg["TE"]

    def kernel(x_hbm, c_hbm, wq_hbm, wk_hbm, wv_hbm, wo_hbm, wr_ref, wg_hbm, wu_hbm, wd_hbm,
               out_hbm,
               x_s, c_s, wq_raw, wk_raw, wv_raw, wq_s, wk_s, wv_s, wo_s, wg_s, wu_s, wd_s,
               xn_s, ctx_s, h_s, hn_s, o_s, r_s, sem, osem):
        S, M = x_s.shape
        C = c_s.shape[1]
        H, _, D = wq_s.shape
        scale = (D ** -0.5) * math.log2(math.e)

        copies = [pltpu.make_async_copy(src, dst, sem.at[i]) for i, (src, dst) in enumerate([
            (x_hbm, x_s), (c_hbm, c_s), (wk_hbm, wk_raw), (wv_hbm, wv_raw), (wq_hbm, wq_raw),
            (wo_hbm, wo_s), (wg_hbm, wg_s), (wu_hbm, wu_s), (wd_hbm, wd_s)])]
        for c in copies:
            c.start()

        def relayout(raw, dst, g, ch):
            R = dst.shape[1] // 8
            ru = raw.bitcast(jnp.uint32)
            base = pl.multiple_of(ch * (R * 16), 16)
            sub = ru.at[pl.ds(base, R * 16), :]
            r0 = pl.multiple_of(ch * R, R)
            sub = sub.at[pl.ds(pl.multiple_of(g * 4, 4), R * 16 - 12), :]
            for j in range(4):
                u = sub[pl.ds(j, R, stride=16), :]
                lo = pltpu.bitcast(u << 16, F32).astype(BF)
                hi = pltpu.bitcast(u & jnp.uint32(0xFFFF0000), F32).astype(BF)
                dst[g * 8 + 2 * j, pl.ds(r0, R), :] = lo
                dst[g * 8 + 2 * j + 1, pl.ds(r0, R), :] = hi

        copies[0].wait()

        def ln1(i, c):
            r0 = pl.multiple_of(i * TE, TE)
            xn_s[pl.ds(r0, TE), :] = _ln_rows(x_s[pl.ds(r0, TE), :].astype(F32))
            return c
        lax.fori_loop(0, S // TE, ln1, 0)
        for i in range(1, 5):
            copies[i].wait()

        def rl0(ch, c):
            relayout(wq_raw, wq_s, 0, ch)
            relayout(wk_raw, wk_s, 0, ch)
            relayout(wv_raw, wv_s, 0, ch)
            return c
        lax.fori_loop(0, 8, rl0, 0)

        def head(h, carry):
            gn = jnp.minimum(lax.shift_right_logical(h, 3) + 1, H // 8 - 1)
            ch = h & 7
            wq = wq_s[h]
            wkv = jnp.concatenate([wk_s[h], wv_s[h]], axis=1)
            kv = jnp.dot(c_s[...], wkv, preferred_element_type=F32).astype(BF)
            k = kv[:, :D]
            v = kv[:, D:]
            row = lax.broadcasted_iota(jnp.int32, (TQ, TQ), 0)
            col = lax.broadcasted_iota(jnp.int32, (TQ, TQ), 1)
            causal = col <= row
            nq = S // TQ
            order = range(nq - 1, -1, -1) if cfg["order"] == "desc" else range(nq)
            for i in order:
                n = (i + 1) * TQ
                q = (jnp.dot(xn_s[i * TQ:(i + 1) * TQ, :], wq, preferred_element_type=F32) * scale).astype(BF)
                s = lax.dot_general(q, k[:n], NT, preferred_element_type=F32)
                sd = jnp.where(causal, s[:, n - TQ:], NEG)
                s = jnp.concatenate([s[:, :n - TQ], sd], axis=1) if i > 0 else sd
                m = jnp.max(s, axis=1, keepdims=True)
                p = jnp.exp2(s - m)
                l = jnp.sum(p, axis=1, keepdims=True)
                o = jnp.dot(p.astype(BF), v[:n], preferred_element_type=F32)
                ctx_s[h, i * TQ:(i + 1) * TQ, :] = (o * (1.0 / l)).astype(BF)
            relayout(wq_raw, wq_s, gn, ch)
            relayout(wk_raw, wk_s, gn, ch)
            relayout(wv_raw, wv_s, gn, ch)
            return carry
        lax.fori_loop(0, H, head, 0)

        copies[5].wait()
        wr = wr_ref[...].astype(F32)

        def out_copy(i):
            r0 = pl.multiple_of(i * TE, TE)
            return pltpu.make_async_copy(o_s.at[pl.ds(r0, TE), :], out_hbm.at[pl.ds(r0, TE), :], osem.at[i])

        def epi(i, c):
            r0 = pl.multiple_of(i * TE, TE)
            ctx = jnp.concatenate([ctx_s[hh, pl.ds(r0, TE), :] for hh in range(H)], axis=1)
            a = jnp.dot(ctx, wo_s[...], preferred_element_type=F32)
            hb = (x_s[pl.ds(r0, TE), :].astype(F32) + _rb(a)).astype(BF)
            hf = hb.astype(F32)
            hn = _ln_rows(hf)
            hnf = hn.astype(F32)
            r_s[pl.ds(r0, TE), :] = _rb(jnp.sum(hnf * wr, axis=-1, keepdims=True))
            h_s[pl.ds(r0, TE), :] = hb
            hn_s[pl.ds(r0, TE), :] = hn
            o_s[pl.ds(r0, TE), :] = (hf + hnf).astype(BF)
            out_copy(i).start()
            return c
        lax.fori_loop(0, S // TE, epi, 0)

        r = r_s[...]
        idx = lax.broadcasted_iota(jnp.int32, r.shape, 0)
        m1 = jnp.max(r, axis=0, keepdims=True)
        i1v = jnp.min(jnp.where(r == m1, idx, S), axis=0, keepdims=True)
        r2 = jnp.where(idx == i1v, -jnp.inf, r)
        m2 = jnp.max(r2, axis=0, keepdims=True)
        i2v = jnp.min(jnp.where((r2 == m2) & (idx != i1v), idx, S), axis=0, keepdims=True)
        i1 = jnp.minimum(jnp.min(i1v), S - 1)
        i2 = jnp.minimum(jnp.min(i2v), S - 1)
        b1 = pl.multiple_of(i1 & (-16), 16)
        b2 = pl.multiple_of(i2 & (-16), 16)
        rows16 = lax.broadcasted_iota(jnp.int32, (16, M), 0)
        hn1 = hn_s[pl.ds(b1, 16), :].astype(F32)
        hn2 = hn_s[pl.ds(b2, 16), :].astype(F32)
        x1 = jnp.sum(jnp.where(rows16 == i1 - b1, hn1, 0.0), axis=0, keepdims=True)
        x2 = jnp.sum(jnp.where(rows16 == i2 - b2, hn2, 0.0), axis=0, keepdims=True)
        xs = jnp.where(rows16 == 0, x1, jnp.where(rows16 == 1, x2, 0.0)).astype(BF)
        for i in range(6, 9):
            copies[i].wait()
        g = _rb(jnp.dot(xs, wg_s[...], preferred_element_type=F32))
        u = _rb(jnp.dot(xs, wu_s[...], preferred_element_type=F32))
        g = _rb(g * jax.nn.sigmoid(g))
        y = _rb(jnp.dot((g * u).astype(BF), wd_s[...], preferred_element_type=F32))
        y1 = _rb(y[0:1, :] * _rb(jax.nn.sigmoid(m1)))
        y2 = _rb(y[1:2, :] * _rb(jax.nn.sigmoid(m2)))
        for i in range(S // TE):
            out_copy(i).wait()
        for b, hnb in ((b1, hn1), (b2, hn2)):
            rows = rows16 + b
            upd = jnp.where(rows == i1, y1, jnp.where(rows == i2, y2, 0.0))
            o_s[pl.ds(b, 16), :] = (h_s[pl.ds(b, 16), :].astype(F32) + _rb(hnb + upd)).astype(BF)
            cp = pltpu.make_async_copy(o_s.at[pl.ds(b, 16), :], out_hbm.at[pl.ds(b, 16), :], osem.at[0])
            cp.start()
            cp.wait()

    @jax.jit
    def run(A_x, A_c_kv, A_w_q, A_w_uk, A_w_uv, A_w_o, B_x, B_w_r, B_w_gate, B_w_up, B_w_down):
        B, S, M = A_x.shape
        C = A_c_kv.shape[2]
        _, H, D = A_w_q.shape
        Fd = B_w_gate.shape[1]
        anyspec = pl.BlockSpec(memory_space=pl.ANY)
        out = pl.pallas_call(
            kernel,
            in_specs=[anyspec] * 6 + [pl.BlockSpec(memory_space=pltpu.VMEM)] + [anyspec] * 3,
            out_specs=anyspec,
            out_shape=jax.ShapeDtypeStruct((S, M), BF),
            scratch_shapes=[
                pltpu.VMEM((S, M), BF), pltpu.VMEM((S, C), BF),
                pltpu.VMEM((M * H, D), BF), pltpu.VMEM((C * H, D), BF), pltpu.VMEM((C * H, D), BF),
                pltpu.VMEM((H, M, D), BF), pltpu.VMEM((H, C, D), BF), pltpu.VMEM((H, C, D), BF),
                pltpu.VMEM((H * D, M), BF),
                pltpu.VMEM((M, Fd), BF), pltpu.VMEM((M, Fd), BF), pltpu.VMEM((Fd, M), BF),
                pltpu.VMEM((S, M), BF), pltpu.VMEM((H, S, D), BF),
                pltpu.VMEM((S, M), BF), pltpu.VMEM((S, M), BF), pltpu.VMEM((S, M), BF),
                pltpu.VMEM((S, 1), F32),
                pltpu.SemaphoreType.DMA((9,)), pltpu.SemaphoreType.DMA((S // TE,)),
            ],
            compiler_params=pltpu.CompilerParams(vmem_limit_bytes=120 * 1024 * 1024),
        )(A_x.reshape(S, M), A_c_kv.reshape(S, C), A_w_q.reshape(M * H, D), A_w_uk.reshape(C * H, D),
          A_w_uv.reshape(C * H, D), A_w_o.reshape(H * D, M), B_w_r.reshape(1, M), B_w_gate, B_w_up, B_w_down)
        return out.reshape(B, S, M)

    return run


_RUN = make(dict(CFG, **{}))


@jax.jit
def pallas_sequential_preLN__compressed_kv_cla__moe_arch_mod__prompt_kernel(A_x, A_c_kv, A_w_q, A_w_uk, A_w_uv, A_w_o, B_x, B_w_r, B_w_gate, B_w_up, B_w_down):
    return _RUN(A_x, A_c_kv, A_w_q, A_w_uk, A_w_uv, A_w_o, B_x, B_w_r, B_w_gate, B_w_up, B_w_down)
```

```python
import contextlib
import functools
import math
import jax
import jax.numpy as jnp
from jax import lax
from jax.experimental import pallas as pl
from jax.experimental.pallas import tpu as pltpu

BF = jnp.bfloat16
F32 = jnp.float32
NT = (((1,), (1,)), ((), ()))
NEG = -1e30
EPS = 1e-5
G = 8
BIG = 3e38

CFG = dict(TQ=256, TE=256, CN=16, dist=2, L1=16)


def _rb(x):
    return x.astype(BF).astype(F32)


def _after(x, dep):
    return x if dep is None else jnp.maximum(x, dep - BIG)


def _ln_rows(x, dep=None):
    n = x.shape[-1]
    mu = _after(jnp.sum(x, axis=-1, keepdims=True), dep) * (1.0 / n)
    xc = x - mu
    var = jnp.sum(xc * xc, axis=-1, keepdims=True) * (1.0 / n)
    den = _rb(jnp.sqrt(_rb(_rb(var) + EPS)))
    num = _rb(x - _rb(mu))
    return (num * (1.0 / den)).astype(BF)


def make(cfg):
    TQ, TE, CN, L1 = cfg["TQ"], cfg["TE"], cfg["CN"], cfg["L1"]
    scope = jax.named_scope if cfg.get("scopes") else (lambda n: contextlib.nullcontext())

    def kernel(x_hbm, c_hbm, wq_hbm, wk_hbm, wv_hbm, wo_hbm, wr_ref, wg_hbm, wu_hbm, wd_hbm,
               out_hbm,
               x_s, c_s, wq_raw, wk_raw, wv_raw, wq_s, wk_s, wv_s, wo_s, wg_s, wu_s, wd_s,
               xn_s, q_s, k_s, v_s, ctx_s, h_s, hn_s, o_s, sem, xsem, wsem, osem):
        S, M = x_s.shape
        H, _, D = ctx_s.shape
        NG = H // G
        nq = S // TQ
        scale = (D ** -0.5) * math.log2(math.e)

        def wcopies(g):
            return [pltpu.make_async_copy(src.at[:, pl.ds(pl.multiple_of(g * G, G), G), :], dst.at[g & 1], wsem.at[3 * g + i])
                    for i, (src, dst) in enumerate([(wk_hbm, wk_raw), (wv_hbm, wv_raw), (wq_hbm, wq_raw)])]

        Fd = wg_s.shape[1]
        big = [pltpu.make_async_copy(src, dst, sem.at[i]) for i, (src, dst) in enumerate([
            (c_hbm, c_s), (wo_hbm, wo_s), (wg_hbm, wg_s), (wu_hbm, wu_s), (wd_hbm, wd_s.at[:, 0:M])])]

        def x_copy(i):
            rows = pl.ds(pl.multiple_of(i * TQ, TQ), TQ)
            return pltpu.make_async_copy(x_hbm.at[rows, :], x_s.at[rows, :], xsem.at[i])

        w0 = wcopies(0)
        for c in (w0[0], w0[1], big[0], w0[2]):
            c.start()
        for i in range(nq):
            x_copy(i).start(priority=1)

        def relayout(raw, dst, g, r0, R):
            r0 = pl.multiple_of(r0, 16)
            dst[pl.ds(pl.multiple_of((g & 1) * G, G), G), pl.ds(r0, R), :] = jnp.swapaxes(raw[g & 1, pl.ds(r0, R), :, :], 0, 1)

        def relayout_chunk(g, ch):
            for raw, dst in ((wk_raw, wk_s), (wv_raw, wv_s), (wq_raw, wq_s)):
                R = dst.shape[1] // G
                relayout(raw, dst, g, ch * R, R)

        def kv_piece(hn, r0):
            w = hn & (2 * G - 1)
            wkv = jnp.concatenate([wk_s[w], wv_s[w]], axis=1)
            kv = jnp.dot(c_s[pl.ds(r0, TQ), :], wkv, preferred_element_type=F32).astype(BF)
            k_s[pl.ds(r0, TQ), :] = kv[:, :D]
            v_s[pl.ds(r0, TQ), :] = kv[:, D:]

        def q_piece(hn, r0):
            q = jnp.dot(xn_s[pl.ds(r0, TQ), :], wq_s[hn & (2 * G - 1)], preferred_element_type=F32)
            q_s[pl.ds(r0, TQ), :] = (q * scale).astype(BF)

        def rl_loop(pairs):
            def body(ch, c):
                for raw, dst in pairs:
                    R = dst.shape[1] // G
                    relayout(raw, dst, 0, ch * R, R)
                return c
            lax.fori_loop(0, G, body, 0)

        def ln1(i):
            for j in range(TQ // L1):
                rows = pl.ds(pl.multiple_of(i * TQ + j * L1, L1), L1)
                x = x_s[rows, :].astype(F32)
                xc = x - jnp.sum(x, axis=-1, keepdims=True) * (1.0 / M)
                var = jnp.sum(xc * xc, axis=-1, keepdims=True) * (1.0 / M)
                xn_s[rows, :] = (xc * lax.rsqrt(var + EPS)).astype(BF)

        with scope("p_wkv"):
            w0[0].wait()
            w0[1].wait()
            rl_loop(((wk_raw, wk_s), (wv_raw, wv_s)))
        with scope("p_kv"):
            big[0].wait()
            for c in wcopies(1):
                c.start(priority=1)
            for i in range(nq):
                kv_piece(0, i * TQ)
        with scope("p_wq"):
            w0[2].wait()
            rl_loop(((wq_raw, wq_s),))
        with scope("p_x"):
            x_copy(0).wait()
            ln1(0)

            def pro(i, c):
                x_copy(i).wait()
                q_piece(0, pl.multiple_of((i - 1) * TQ, TQ))
                ln1(i)
                return c
            lax.fori_loop(1, nq, pro, 0)
            q_piece(0, (nq - 1) * TQ)

        def attention(h, gap, tail):
            HB = TQ // 2
            row = lax.broadcasted_iota(jnp.int32, (HB, HB), 0)
            col = lax.broadcasted_iota(jnp.int32, (HB, HB), 1)
            tri = col <= row
            deps = [(None, None)] * cfg['dist']
            for i in range(nq - 1, -1, -1):
                n0 = i * TQ
                n1 = n0 + HB
                q = q_s[n0:n0 + TQ, :]
                s = lax.dot_general(q, k_s[:n1, :], NT, preferred_element_type=F32)
                s2 = lax.dot_general(q[HB:], k_s[n1:n1 + HB, :], NT, preferred_element_type=F32)
                gap(i)
                sa = jnp.where(tri, s[:HB, n0:], NEG)
                sa = jnp.concatenate([s[:HB, :n0], sa], axis=1) if i > 0 else sa
                sb = s[HB:]
                s2 = jnp.where(tri, s2, NEG)
                da, db = deps.pop(0)
                ma = _after(jnp.max(sa, axis=1, keepdims=True), da)
                mb = _after(jnp.max(jnp.concatenate([sb, s2], axis=1), axis=1, keepdims=True), db)
                pa = jnp.exp2(sa - ma)
                pb = jnp.exp2(sb - mb)
                p2 = jnp.exp2(s2 - mb)
                la = 1.0 / jnp.sum(pa, axis=1, keepdims=True)
                lb = 1.0 / jnp.sum(jnp.concatenate([pb, p2], axis=1), axis=1, keepdims=True)
                deps.append((la, lb))
                p = jnp.concatenate([pa, pb], axis=0).astype(BF)
                o = jnp.dot(p, v_s[:n1, :], preferred_element_type=F32)
                o2 = jnp.dot(p2.astype(BF), v_s[n1:n1 + HB, :], preferred_element_type=F32)
                ctx_s[h, n0:n1, :] = (o[:HB] * la).astype(BF)
                ctx_s[h, n1:n1 + HB, :] = ((o[HB:] + o2) * lb).astype(BF)
            tail()

        def head(h, carry):
            hn = h + 1
            g = lax.shift_right_logical(hn, 3)
            ch = hn & (G - 1)

            @pl.when(jnp.logical_and(ch == 0, g + 1 < NG))
            def _():
                for c in wcopies(g + 1):
                    c.wait()

            @pl.when(h == 1)
            def _():
                for c in wcopies(1):
                    c.wait()
                relayout_chunk(1, 0)
                relayout_chunk(1, 1)

            @pl.when(jnp.logical_and(ch == 2, g + 2 < NG))
            def _():
                for c in wcopies(g + 2):
                    c.start()

            @pl.when(h == G * (NG - 2))
            def _():
                for c in big[1:]:
                    c.start()

            gr = jnp.where(h == 0, 0, jnp.minimum(g + 1, NG - 1))
            RQ = wq_s.shape[1] // G
            RK = wk_s.shape[1] // G

            def rl_kv(j):
                raw, dst = ((wk_raw, wk_s), (wv_raw, wv_s))[j % 2]
                P = 2 * RK // nq
                relayout(raw, dst, gr, ch * RK + (j // 2) * P, P)

            def gap(i):
                relayout(wq_raw, wq_s, gr, ch * RQ + i * (RQ // nq), RQ // nq)
                q_piece(hn, i * TQ)
                if i + 1 < nq:
                    rl_kv(i + 1)
                    kv_piece(hn, (i + 1) * TQ)

            def tail():
                rl_kv(0)
                kv_piece(hn, 0)

            attention(h, gap, tail)
            return carry
        with scope("m_loop"):
            lax.fori_loop(0, H - 1, head, 0)
        with scope("m_last"):
            attention(H - 1, lambda i: None, lambda: None)

        big[1].wait()
        wr = wr_ref[...].astype(F32)
        ne = S // TE

        def out_copy(i):
            r0 = pl.multiple_of(i * TE, TE)
            return pltpu.make_async_copy(o_s.at[pl.ds(r0 + TE, TE), :], out_hbm.at[pl.ds(r0, TE), :], osem.at[i])

        def post(r0, chain, top):
            dep = None
            b1, j1, b2, j2 = top
            for j in range(TE // CN):
                rows = pl.ds(r0 + j * CN, CN)
                hf = h_s[rows, :].astype(F32)
                hn = _ln_rows(hf, dep)
                hnf = hn.astype(F32)
                r = _rb(jnp.sum(hnf * wr, axis=-1, keepdims=True))
                hn_s[rows, :] = hn
                o_s[rows, :] = (hf + hnf).astype(BF)
                dep = r if chain else None
                tok = lax.broadcasted_iota(jnp.int32, (CN, 1), 0) + (r0 + j * CN - TE)
                r = jnp.where(tok >= 0, r, -jnp.inf)
                gt1 = r > b1
                gt2 = r > b2
                b2 = jnp.where(gt1, b1, jnp.where(gt2, r, b2))
                j2 = jnp.where(gt1, j1, jnp.where(gt2, tok, j2))
                b1 = jnp.where(gt1, r, b1)
                j1 = jnp.where(gt1, tok, j1)
            return b1, j1, b2, j2

        h_s[0:TE, :] = jnp.zeros((TE, M), BF)

        def epi(i, top):
            r0 = pl.multiple_of(i * TE, TE)
            top = post(r0, True, top)
            ctx = jnp.concatenate([ctx_s[hh, pl.ds(r0, TE), :] for hh in range(H)], axis=1)
            a = jnp.dot(ctx, wo_s[...], preferred_element_type=F32)
            h_s[pl.ds(r0 + TE, TE), :] = (x_s[pl.ds(r0, TE), :].astype(F32) + _rb(a)).astype(BF)

            @pl.when(i > 0)
            def _():
                out_copy(i - 1).start()
            return top
        ninf = jnp.full((CN, 1), -jnp.inf, F32)
        none = jnp.full((CN, 1), S, jnp.int32)
        with scope("e_loop"):
            top = lax.fori_loop(0, ne, epi, (ninf, none, ninf, none))
        with scope("e_post"):
            top = post(S, False, top)
            out_copy(ne - 1).start()

        with scope("t_top2"):
            r = jnp.concatenate([top[0], top[2]], axis=0)
            idx = jnp.concatenate([top[1], top[3]], axis=0)
            m1 = jnp.max(r, axis=0, keepdims=True)
            i1v = jnp.min(jnp.where(r == m1, idx, S), axis=0, keepdims=True)
            r2 = jnp.where(idx == i1v, -jnp.inf, r)
            m2 = jnp.max(r2, axis=0, keepdims=True)
            i2v = jnp.min(jnp.where((r2 == m2) & (idx != i1v), idx, S), axis=0, keepdims=True)
            i1 = jnp.minimum(jnp.min(i1v), S - 1)
            i2 = jnp.minimum(jnp.min(i2v), S - 1)
            b1 = pl.multiple_of(i1 & (-16), 16)
            b2 = pl.multiple_of(i2 & (-16), 16)
            rows16 = lax.broadcasted_iota(jnp.int32, (16, M), 0)
            hn1 = hn_s[pl.ds(b1 + TE, 16), :].astype(F32)
            hn2 = hn_s[pl.ds(b2 + TE, 16), :].astype(F32)
            x1 = jnp.sum(jnp.where(rows16 == i1 - b1, hn1, 0.0), axis=0, keepdims=True)
            x2 = jnp.sum(jnp.where(rows16 == i2 - b2, hn2, 0.0), axis=0, keepdims=True)
            xs = jnp.where(rows16 == 0, x1, jnp.where(rows16 == 1, x2, 0.0)).astype(BF)
        with scope("t_ffn"):
            for c in big[2:]:
                c.wait()
            g = _rb(jnp.dot(xs, wg_s[...], preferred_element_type=F32)[:8])
            u = _rb(jnp.dot(xs, wu_s[...], preferred_element_type=F32)[:8])
            g = _rb(g * jax.nn.sigmoid(g))
            gu = jnp.concatenate([g * u, jnp.zeros_like(g)], axis=0).astype(BF)
            y = _rb(jnp.dot(gu, wd_s[:, 0:M], preferred_element_type=F32)[:8])
            y1 = _rb(y[0:1, :] * _rb(jax.nn.sigmoid(m1)))
            y2 = _rb(y[1:2, :] * _rb(jax.nn.sigmoid(m2)))
        with scope("t_patch"):
            for i in range(ne):
                out_copy(i).wait()
            cps = []
            for n, (b, hnb) in enumerate(((b1, hn1), (b2, hn2))):
                rows = rows16 + b
                upd = jnp.where(rows == i1, y1, jnp.where(rows == i2, y2, 0.0))
                o_s[pl.ds(b + TE, 16), :] = (h_s[pl.ds(b + TE, 16), :].astype(F32) + _rb(hnb + upd)).astype(BF)
                cps.append(pltpu.make_async_copy(o_s.at[pl.ds(b + TE, 16), :], out_hbm.at[pl.ds(b, 16), :], osem.at[n]))
            cps[0].start()

            @pl.when(b1 != b2)
            def _():
                cps[1].start()
                cps[1].wait()
            cps[0].wait()

    @jax.jit
    def run(A_x, A_c_kv, A_w_q, A_w_uk, A_w_uv, A_w_o, B_x, B_w_r, B_w_gate, B_w_up, B_w_down):
        B, S, M = A_x.shape
        C = A_c_kv.shape[2]
        _, H, D = A_w_q.shape
        Fd = B_w_gate.shape[1]
        NG = H // G
        anyspec = pl.BlockSpec(memory_space=pl.ANY)
        out = pl.pallas_call(
            kernel,
            in_specs=[anyspec] * 6 + [pl.BlockSpec(memory_space=pltpu.VMEM)] + [anyspec] * 3,
            out_specs=anyspec,
            out_shape=jax.ShapeDtypeStruct((S, M), BF),
            scratch_shapes=[
                pltpu.VMEM((S, M), BF), pltpu.VMEM((S, C), BF),
                pltpu.VMEM((2, M, G, D), BF), pltpu.VMEM((2, C, G, D), BF), pltpu.VMEM((2, C, G, D), BF),
                pltpu.VMEM((2 * G, M, D), BF), pltpu.VMEM((2 * G, C, D), BF), pltpu.VMEM((2 * G, C, D), BF),
                pltpu.VMEM((H * D, M), BF),
                pltpu.VMEM((M, Fd), BF), pltpu.VMEM((M, Fd), BF), pltpu.VMEM((Fd, M + 128), BF),
                pltpu.VMEM((S, M), BF),
                pltpu.VMEM((S, D), BF), pltpu.VMEM((S, D), BF), pltpu.VMEM((S, D), BF),
                pltpu.VMEM((H, S, D), BF),
                pltpu.VMEM((S + TE, M), BF), pltpu.VMEM((S + TE, M), BF), pltpu.VMEM((S + TE, M), BF),
                pltpu.SemaphoreType.DMA((5,)), pltpu.SemaphoreType.DMA((S // TQ,)), pltpu.SemaphoreType.DMA((3 * NG,)), pltpu.SemaphoreType.DMA((S // TE,)),
            ],
            compiler_params=pltpu.CompilerParams(vmem_limit_bytes=120 * 1024 * 1024),
        )(A_x.reshape(S, M), A_c_kv.reshape(S, C), A_w_q, A_w_uk, A_w_uv,
          A_w_o.reshape(H * D, M), B_w_r.reshape(1, M), B_w_gate, B_w_up, B_w_down)
        return out.reshape(B, S, M)

    return run


_RUN = make(dict(CFG, **{}))


@jax.jit
def pallas_sequential_preLN__compressed_kv_cla__moe_arch_mod__prompt_kernel(A_x, A_c_kv, A_w_q, A_w_uk, A_w_uv, A_w_o, B_x, B_w_r, B_w_gate, B_w_up, B_w_down):
    return _RUN(A_x, A_c_kv, A_w_q, A_w_uk, A_w_uv, A_w_o, B_x, B_w_r, B_w_gate, B_w_up, B_w_down)
```

```python
import contextlib
import math
import jax
import jax.numpy as jnp
from jax import lax
from jax.experimental import pallas as pl
from jax.experimental.pallas import tpu as pltpu

BF = jnp.bfloat16
F32 = jnp.float32
NT = (((1,), (1,)), ((), ()))
NEG = -1e30
EPS = 1e-5
BIG = 3e38

CFG = dict(TQ=256, TE=256, CN=16, dist=2, L1=16, TC=512)


def _rb(x):
    return x.astype(BF).astype(F32)


def _after(x, dep):
    return x if dep is None else jnp.maximum(x, dep - BIG)


def _ln_rows(x, dep=None):
    n = x.shape[-1]
    mu = _after(jnp.sum(x, axis=-1, keepdims=True), dep) * (1.0 / n)
    xc = x - mu
    var = jnp.sum(xc * xc, axis=-1, keepdims=True) * (1.0 / n)
    den = _rb(jnp.sqrt(_rb(_rb(var) + EPS)))
    num = _rb(x - _rb(mu))
    return (num * (1.0 / den)).astype(BF)


def _unpack(z, odd):
    u = pltpu.bitcast(z, jnp.uint32)
    u = u.reshape(u.shape[0] * u.shape[1], u.shape[2])
    u = (u & jnp.uint32(0xFFFF0000)) if odd else (u << 16)
    return pltpu.bitcast(u, F32).astype(BF)


def make(cfg):
    TQ, TE, CN, L1, TC = cfg["TQ"], cfg["TE"], cfg["CN"], cfg["L1"], cfg["TC"]
    scope = jax.named_scope if cfg.get("scopes") else (lambda n: contextlib.nullcontext())

    def kernel(x_hbm, c_hbm, wq_hbm, wk_hbm, wv_hbm, wo_hbm, wr_ref, wg_hbm, wu_hbm, wd_hbm,
               out_hbm,
               x_s, c_s, zq, zk, zv, wo_s, wg_s, wu_s, wd_s,
               xn_s, q_s, k_s, v_s, k0_s, v0_s, w4_s, ctx_s, h_s, hn_s, o_s, sem, xsem, csem, wsem, osem):
        S, M = x_s.shape
        H, _, D = ctx_s.shape
        nq = S // TQ
        scale = (D ** -0.5) * math.log2(math.e)
        W = ((wk_hbm, zk), (wv_hbm, zv), (wq_hbm, zq))

        PG = (0, 1, 4, H // 2)

        def w_start(i, g, priority):
            src, z = W[i]
            for r in range(8):
                pltpu.make_async_copy(src.at[:, r, PG[g]:PG[g + 1]], z.at[:, PG[g]:PG[g + 1], 2 * r:2 * r + 2, :],
                                      wsem.at[3 * g + i]).start(priority=priority)

        def w_wait(i, g):
            z = W[i][1].at[:, PG[g]:PG[g + 1]]
            pltpu.make_async_copy(z, z, wsem.at[3 * g + i]).wait()

        def x_copy(i):
            rows = pl.ds(pl.multiple_of(i * TQ, TQ), TQ)
            return pltpu.make_async_copy(x_hbm.at[rows, :], x_s.at[rows, :], xsem.at[i])

        def c_copy(i):
            rows = pl.ds(pl.multiple_of(i * TC, TC), TC)
            return pltpu.make_async_copy(c_hbm.at[rows, :], c_s.at[rows, :], csem.at[i])

        big = [pltpu.make_async_copy(src, dst, sem.at[i]) for i, (src, dst) in enumerate([
            (wo_hbm, wo_s), (wg_hbm, wg_s), (wu_hbm, wu_s), (wd_hbm, wd_s.at[:, 0:M])])]

        def start_loop(lo, hi, fn):
            def body(i, c):
                fn(i)
                return c
            lax.fori_loop(lo, hi, body, 0)

        w_start(0, 0, 0)
        w_start(1, 0, 0)
        c_copy(0).start()
        start_loop(1, S // TC, lambda j: c_copy(j).start(priority=1))
        w_start(2, 0, 1)
        start_loop(0, nq, lambda j: x_copy(nq - 1 - j).start(priority=1))

        def kv_piece(wkv, r0):
            kv = jnp.dot(c_s[r0:r0 + TQ, :], wkv, preferred_element_type=F32).astype(BF)
            k_s[r0:r0 + TQ, :] = kv[:, :D]
            v_s[r0:r0 + TQ, :] = kv[:, D:]

        def q_piece(wq, r0):
            q = jnp.dot(xn_s[r0:r0 + TQ, :], wq, preferred_element_type=F32)
            q_s[r0:r0 + TQ, :] = (q * scale).astype(BF)

        def ln1(i):
            for j in range(TQ // L1):
                rows = slice(i * TQ + j * L1, i * TQ + (j + 1) * L1)
                x = x_s[rows, :].astype(F32)
                xc = x - jnp.sum(x, axis=-1, keepdims=True) * (1.0 / M)
                var = jnp.sum(xc * xc, axis=-1, keepdims=True) * (1.0 / M)
                xn_s[rows, :] = (xc * lax.rsqrt(var + EPS)).astype(BF)

        def attention(h, kr, vr, pre, gap, tail, deps):
            HB = TQ // 2
            row = lax.broadcasted_iota(jnp.int32, (HB, HB), 0)
            col = lax.broadcasted_iota(jnp.int32, (HB, HB), 1)
            tri = col <= row
            deps = list(deps)
            for i in range(nq - 1, -1, -1):
                n0 = i * TQ
                n1 = n0 + HB
                pre(i)
                q = q_s[n0:n0 + TQ, :]
                s = lax.dot_general(q, kr[:n1, :], NT, preferred_element_type=F32)
                s2 = lax.dot_general(q[HB:], kr[n1:n1 + HB, :], NT, preferred_element_type=F32)
                gap(i)
                sa = jnp.where(tri, s[:HB, n0:], NEG)
                sa = jnp.concatenate([s[:HB, :n0], sa], axis=1) if i > 0 else sa
                sb = s[HB:]
                s2 = jnp.where(tri, s2, NEG)
                da, db = deps.pop(0)
                ma = _after(jnp.max(sa, axis=1, keepdims=True), da)
                mb = _after(jnp.max(jnp.concatenate([sb, s2], axis=1), axis=1, keepdims=True), db)
                pa = jnp.exp2(sa - ma)
                pb = jnp.exp2(sb - mb)
                p2 = jnp.exp2(s2 - mb)
                la = 1.0 / jnp.sum(pa, axis=1, keepdims=True)
                lb = 1.0 / jnp.sum(jnp.concatenate([pb, p2], axis=1), axis=1, keepdims=True)
                deps.append((la, lb))
                p = jnp.concatenate([pa, pb], axis=0).astype(BF)
                o = jnp.dot(p, vr[:n1, :], preferred_element_type=F32)
                o2 = jnp.dot(p2.astype(BF), vr[n1:n1 + HB, :], preferred_element_type=F32)
                ctx_s[h, n0:n1, :] = (o[:HB] * la).astype(BF)
                ctx_s[h, n1:n1 + HB, :] = ((o[HB:] + o2) * lb).astype(BF)
            tail()
            return deps

        nodeps = [(None, None)] * cfg["dist"]
        nop = lambda *a: None

        with scope("p_kv"):
            w_wait(0, 0)
            w_wait(1, 0)
            w4_s[...] = jnp.concatenate([_unpack(z[:, 0], odd) for odd in (0, 1) for z in (zk, zv)], axis=1)

            def kv01(j):
                rows = pl.ds(pl.multiple_of(j * TC, TC), TC)
                kv = jnp.dot(c_s[rows, :], w4_s[...], preferred_element_type=F32).astype(BF)
                for n, dst in enumerate((k0_s, v0_s, k_s, v_s)):
                    dst[rows, :] = kv[:, n * D:(n + 1) * D]

            def kv_body(j, c):
                c_copy(j).wait()
                kv01(j)
                return c
            lax.fori_loop(0, S // TC - 1, kv_body, 0)
            c_copy(S // TC - 1).wait()
            w_wait(2, 0)
            x_copy(nq - 1).wait()
            ln1(nq - 1)
            kv01(S // TC - 1)
            wq0 = _unpack(zq[:, 0], 0)
            wq1 = _unpack(zq[:, 0], 1)
            q_piece(wq0, (nq - 1) * TQ)

        def wb(r):
            for i in range(3):
                src, z = W[i]
                pltpu.make_async_copy(src.at[:, r, PG[1]:PG[2]], z.at[:, PG[1]:PG[2], pl.ds(pl.multiple_of(2 * r, 2), 2), :],
                                      wsem.at[3 + i]).start(priority=1)
        start_loop(0, 8, wb)
        with scope("m_first"):
            def pre0(i):
                if i == nq - 1:
                    for j in range(nq // 2, nq - 1):
                        x_copy(j).wait()
                if i == nq // 2:
                    for j in range(nq // 2):
                        x_copy(j).wait()

            def gap0(i):
                q_piece(wq1, i * TQ)
                if i > 0:
                    ln1(i - 1)
                    q_piece(wq0, (i - 1) * TQ)
            attention(0, k0_s, v0_s, pre0, gap0, nop, nodeps)

        def head(h, p, odd, deps):
            wq = _unpack(zq[:, p], odd)
            wkv = jnp.concatenate([_unpack(zk[:, p], odd), _unpack(zv[:, p], odd)], axis=1)

            def gap(i):
                if i > 0:
                    q_piece(wq, i * TQ)
                if i + 1 < nq:
                    kv_piece(wkv, (i + 1) * TQ)

            def tail():
                kv_piece(wkv, 0)
                q_piece(wq, 0)

            return attention(h, k_s, v_s, nop, gap, tail, deps)

        def heads(t, carry):
            p = t + 1

            @pl.when(p == 1)
            def _():
                for i in range(3):
                    w_start(i, 2, 1)

            @pl.when(p == PG[2])
            def _():
                for i in range(3):
                    w_wait(i, 2)
                for c in big:
                    c.start(priority=1)

            with scope("m_iter"):
                deps = head(2 * t + 1, p, 0, nodeps)
                head(2 * t + 2, p, 1, deps)
            return carry
        for i in range(3):
            w_wait(i, 1)
        with scope("m_loop"):
            lax.fori_loop(0, H // 2 - 1, heads, 0)
        with scope("m_last"):
            attention(H - 1, k_s, v_s, nop, nop, nop, nodeps)

        big[0].wait()
        wr = wr_ref[...].astype(F32)
        ne = S // TE

        def out_copy(i):
            r0 = pl.multiple_of(i * TE, TE)
            return pltpu.make_async_copy(o_s.at[pl.ds(r0 + TE, TE), :], out_hbm.at[pl.ds(r0, TE), :], osem.at[i])

        def post(r0, chain, top):
            dep = None
            b1, j1, b2, j2 = top
            for j in range(TE // CN):
                rows = pl.ds(r0 + j * CN, CN)
                hf = h_s[rows, :].astype(F32)
                hn = _ln_rows(hf, dep)
                hnf = hn.astype(F32)
                r = _rb(jnp.sum(hnf * wr, axis=-1, keepdims=True))
                hn_s[rows, :] = hn
                o_s[rows, :] = (hf + hnf).astype(BF)
                dep = r if chain else None
                tok = lax.broadcasted_iota(jnp.int32, (CN, 1), 0) + (r0 + j * CN - TE)
                r = jnp.where(tok >= 0, r, -jnp.inf)
                gt1 = r > b1
                gt2 = r > b2
                b2 = jnp.where(gt1, b1, jnp.where(gt2, r, b2))
                j2 = jnp.where(gt1, j1, jnp.where(gt2, tok, j2))
                b1 = jnp.where(gt1, r, b1)
                j1 = jnp.where(gt1, tok, j1)
            return b1, j1, b2, j2

        h_s[0:TE, :] = jnp.zeros((TE, M), BF)

        def epi(i, top):
            r0 = pl.multiple_of(i * TE, TE)
            top = post(r0, True, top)
            ctx = jnp.concatenate([ctx_s[hh, pl.ds(r0, TE), :] for hh in range(H)], axis=1)
            a = jnp.dot(ctx, wo_s[...], preferred_element_type=F32)
            h_s[pl.ds(r0 + TE, TE), :] = (x_s[pl.ds(r0, TE), :].astype(F32) + _rb(a)).astype(BF)

            @pl.when(i > 0)
            def _():
                out_copy(i - 1).start()
            return top
        ninf = jnp.full((CN, 1), -jnp.inf, F32)
        none = jnp.full((CN, 1), S, jnp.int32)
        with scope("e_loop"):
            top = lax.fori_loop(0, ne, epi, (ninf, none, ninf, none))
        with scope("e_post"):
            top = post(S, False, top)
            out_copy(ne - 1).start()

        with scope("t_top2"):
            r = jnp.concatenate([top[0], top[2]], axis=0)
            idx = jnp.concatenate([top[1], top[3]], axis=0)
            m1 = jnp.max(r, axis=0, keepdims=True)
            i1v = jnp.min(jnp.where(r == m1, idx, S), axis=0, keepdims=True)
            r2 = jnp.where(idx == i1v, -jnp.inf, r)
            m2 = jnp.max(r2, axis=0, keepdims=True)
            i2v = jnp.min(jnp.where((r2 == m2) & (idx != i1v), idx, S), axis=0, keepdims=True)
            i1 = jnp.minimum(jnp.min(i1v), S - 1)
            i2 = jnp.minimum(jnp.min(i2v), S - 1)
            b1 = pl.multiple_of(i1 & (-16), 16)
            b2 = pl.multiple_of(i2 & (-16), 16)
            rows16 = lax.broadcasted_iota(jnp.int32, (16, M), 0)
            hn1 = hn_s[pl.ds(b1 + TE, 16), :].astype(F32)
            hn2 = hn_s[pl.ds(b2 + TE, 16), :].astype(F32)
            x1 = jnp.sum(jnp.where(rows16 == i1 - b1, hn1, 0.0), axis=0, keepdims=True)
            x2 = jnp.sum(jnp.where(rows16 == i2 - b2, hn2, 0.0), axis=0, keepdims=True)
            xs = jnp.where(rows16 == 0, x1, jnp.where(rows16 == 1, x2, 0.0)).astype(BF)
        with scope("t_ffn"):
            for c in big[1:]:
                c.wait()
            g = _rb(jnp.dot(xs, wg_s[...], preferred_element_type=F32)[:8])
            u = _rb(jnp.dot(xs, wu_s[...], preferred_element_type=F32)[:8])
            g = _rb(g * jax.nn.sigmoid(g))
            gu = jnp.concatenate([g * u, jnp.zeros_like(g)], axis=0).astype(BF)
            y = _rb(jnp.dot(gu, wd_s[:, 0:M], preferred_element_type=F32)[:8])
            y1 = _rb(y[0:1, :] * _rb(jax.nn.sigmoid(m1)))
            y2 = _rb(y[1:2, :] * _rb(jax.nn.sigmoid(m2)))
        with scope("t_patch"):
            for i in range(ne):
                out_copy(i).wait()
            cps = []
            for n, (b, hnb) in enumerate(((b1, hn1), (b2, hn2))):
                rows = rows16 + b
                upd = jnp.where(rows == i1, y1, jnp.where(rows == i2, y2, 0.0))
                o_s[pl.ds(b + TE, 16), :] = (h_s[pl.ds(b + TE, 16), :].astype(F32) + _rb(hnb + upd)).astype(BF)
                cps.append(pltpu.make_async_copy(o_s.at[pl.ds(b + TE, 16), :], out_hbm.at[pl.ds(b, 16), :], osem.at[n]))
            cps[0].start()

            @pl.when(b1 != b2)
            def _():
                cps[1].start()
                cps[1].wait()
            cps[0].wait()

    @jax.jit
    def run(A_x, A_c_kv, A_w_q, A_w_uk, A_w_uv, A_w_o, B_x, B_w_r, B_w_gate, B_w_up, B_w_down):
        B, S, M = A_x.shape
        C = A_c_kv.shape[2]
        _, H, D = A_w_q.shape
        Fd = B_w_gate.shape[1]
        anyspec = pl.BlockSpec(memory_space=pl.ANY)
        out = pl.pallas_call(
            kernel,
            in_specs=[anyspec] * 6 + [pl.BlockSpec(memory_space=pltpu.VMEM)] + [anyspec] * 3,
            out_specs=anyspec,
            out_shape=jax.ShapeDtypeStruct((S, M), BF),
            scratch_shapes=[
                pltpu.VMEM((S, M), BF), pltpu.VMEM((S, C), BF),
                pltpu.VMEM((M // 8, H // 2, 16, D), BF), pltpu.VMEM((C // 8, H // 2, 16, D), BF), pltpu.VMEM((C // 8, H // 2, 16, D), BF),
                pltpu.VMEM((H * D, M), BF),
                pltpu.VMEM((M, Fd), BF), pltpu.VMEM((M, Fd), BF), pltpu.VMEM((Fd, M + 128), BF),
                pltpu.VMEM((S, M), BF),
                pltpu.VMEM((S, D), BF), pltpu.VMEM((S, D), BF), pltpu.VMEM((S, D), BF),
                pltpu.VMEM((S, D), BF), pltpu.VMEM((S, D), BF), pltpu.VMEM((C, 4 * D), BF),
                pltpu.VMEM((H, S, D), BF),
                pltpu.VMEM((S + TE, M), BF), pltpu.VMEM((S + TE, M), BF), pltpu.VMEM((S + TE, M), BF),
                pltpu.SemaphoreType.DMA((4,)), pltpu.SemaphoreType.DMA((S // TQ,)), pltpu.SemaphoreType.DMA((S // TC,)),
                pltpu.SemaphoreType.DMA((9,)), pltpu.SemaphoreType.DMA((S // TE,)),
            ],
            compiler_params=pltpu.CompilerParams(vmem_limit_bytes=120 * 1024 * 1024),
            interpret=cfg.get("interpret", False),
        )(A_x.reshape(S, M), A_c_kv.reshape(S, C), A_w_q.reshape(M // 8, 8, H // 2, 2, D), A_w_uk.reshape(C // 8, 8, H // 2, 2, D),
          A_w_uv.reshape(C // 8, 8, H // 2, 2, D), A_w_o.reshape(H * D, M), B_w_r.reshape(1, M), B_w_gate, B_w_up, B_w_down)
        return out.reshape(B, S, M)

    return run


_RUN = make(dict(CFG, **{}))


@jax.jit
def pallas_sequential_preLN__compressed_kv_cla__moe_arch_mod__prompt_kernel(A_x, A_c_kv, A_w_q, A_w_uk, A_w_uv, A_w_o, B_x, B_w_r, B_w_gate, B_w_up, B_w_down):
    return _RUN(A_x, A_c_kv, A_w_q, A_w_uk, A_w_uv, A_w_o, B_x, B_w_r, B_w_gate, B_w_up, B_w_down)
```

```python
import contextlib
import math
import jax
import jax.numpy as jnp
from jax import lax
from jax.experimental import pallas as pl
from jax.experimental.pallas import tpu as pltpu

BF = jnp.bfloat16
F32 = jnp.float32
U32 = jnp.uint32
NT = (((1,), (1,)), ((), ()))
NEG = -1e30
EPS = 1e-5
BIG = 3e38

CFG = dict(TQ=256, TE=256, CN=16, dist=2, L1=16, TC=512)


def _rb(x):
    return x.astype(BF).astype(F32)


def _after(x, dep):
    return x if dep is None else jnp.maximum(x, dep - BIG)


def _recip(l):
    r = pl.reciprocal(l, approx=True)
    return r * (2.0 - l * r)


def _ln_rows(x, dep=None):
    n = x.shape[-1]
    mu = _after(jnp.sum(x, axis=-1, keepdims=True), dep) * (1.0 / n)
    xc = x - mu
    var = jnp.sum(xc * xc, axis=-1, keepdims=True) * (1.0 / n)
    den = _rb(jnp.sqrt(_rb(_rb(var) + EPS)))
    num = _rb(x - _rb(mu))
    return (num * (1.0 / den)).astype(BF)


def _unpack(z, odd):
    u = pltpu.bitcast(z, jnp.uint32)
    u = u.reshape(u.shape[0] * u.shape[1], u.shape[2])
    u = (u & jnp.uint32(0xFFFF0000)) if odd else (u << 16)
    return pltpu.bitcast(u, F32).astype(BF)


def _pk(x):
    return pltpu.bitcast(x, jnp.uint32)


def _up(u):
    return pltpu.bitcast(u, BF)


def make(cfg):
    TQ, TE, CN, L1, TC = cfg["TQ"], cfg["TE"], cfg["CN"], cfg["L1"], cfg["TC"]
    scope = jax.named_scope if cfg.get("scopes") else (lambda n: contextlib.nullcontext())

    def kernel(x_hbm, c_hbm, wq_hbm, wk_hbm, wv_hbm, wo_hbm, wr_hbm, wg_hbm, wu_hbm, wd_hbm,
               out_hbm,
               x_s, c_s, cu_s, zq, zk, zv, wo_s, wg_s, wu_s, wd_s, wr_ref,
               xn_s, q_s, k_s, v_s, k0_s, v0_s, w4_s, ctx_s, h_s, hn_s, o_s, sem, xsem, csem, wsem, osem):
        S, M = x_s.shape
        H, _, D = ctx_s.shape
        nq = S // TQ
        scale = (D ** -0.5) * math.log2(math.e)
        W = ((wk_hbm, zk), (wv_hbm, zv), (wq_hbm, zq))

        PG = (0, 1, 2, 5, H // 2)

        def w_start(i, g, priority):
            src, z = W[i]
            for r in range(8):
                pltpu.make_async_copy(src.at[:, r, PG[g]:PG[g + 1]], z.at[:, PG[g]:PG[g + 1], 2 * r:2 * r + 2, :],
                                      wsem.at[3 * g + i]).start(priority=priority)

        def w_wait(i, g):
            z = W[i][1].at[:, PG[g]:PG[g + 1]]
            pltpu.make_async_copy(z, z, wsem.at[3 * g + i]).wait()

        def x_copy(i):
            rows = pl.ds(pl.multiple_of(i * TQ, TQ), TQ)
            return pltpu.make_async_copy(x_hbm.at[rows, :], x_s.at[rows, :], xsem.at[i])

        def c_copy(i):
            rows = pl.ds(pl.multiple_of(i * TC, TC), TC)
            return pltpu.make_async_copy(c_hbm.at[rows, :], c_s.at[rows, :], csem.at[i])

        big = [pltpu.make_async_copy(src, dst, sem.at[i]) for i, (src, dst) in enumerate([
            (wo_hbm, wo_s), (wr_hbm, wr_ref), (wg_hbm, wg_s), (wu_hbm, wu_s), (wd_hbm, wd_s.at[:, 0:M])])]

        def start_loop(lo, hi, fn):
            def body(i, c):
                fn(i)
                return c
            lax.fori_loop(lo, hi, body, 0)

        w_start(0, 0, 0)
        w_start(1, 0, 0)
        c_copy(0).start()
        start_loop(1, S // TC, lambda j: c_copy(j).start(priority=1))
        w_start(2, 0, 1)
        start_loop(0, nq, lambda j: x_copy(nq - 1 - j).start(priority=1))

        def kv_piece(wkv, r0):
            rows = slice(r0 // 2, (r0 + TQ) // 2)
            kv = jnp.dot(_up(cu_s[rows, :]), wkv, preferred_element_type=F32)
            k_s[rows, :] = _pk(kv[:, :D].astype(BF))
            v_s[rows, :] = _pk(kv[:, D:].astype(BF))

        def q_piece(wq, r0):
            rows = slice(r0 // 2, (r0 + TQ) // 2)
            q = jnp.dot(_up(xn_s[rows, :]), wq, preferred_element_type=F32)
            q_s[r0:r0 + TQ, :] = (q * scale).astype(BF)

        def ln1(i):
            for j in range(TQ // L1):
                rows = slice(i * TQ + j * L1, i * TQ + (j + 1) * L1)
                x = x_s[rows, :].astype(F32)
                xc = x - jnp.sum(x, axis=-1, keepdims=True) * (1.0 / M)
                var = jnp.sum(xc * xc, axis=-1, keepdims=True) * (1.0 / M)
                xn_s[rows.start // 2:rows.stop // 2, :] = _pk((xc * lax.rsqrt(var + EPS)).astype(BF))

        def attention(h, kr, vr, pre, gap, tail, deps):
            HB = TQ // 2
            row = lax.broadcasted_iota(jnp.int32, (HB, HB), 0)
            col = lax.broadcasted_iota(jnp.int32, (HB, HB), 1)
            tri = col <= row
            deps = list(deps)
            for i in range(nq - 1, -1, -1):
                n0 = i * TQ
                n1 = n0 + HB
                pre(i)
                n2 = n0 + TQ
                q = q_s[n0:n2, :]
                s = lax.dot_general(q, _up(kr[:n1 // 2, :]), NT, preferred_element_type=F32)
                s2 = lax.dot_general(q[HB:], _up(kr[n1 // 2:n2 // 2, :]), NT, preferred_element_type=F32)
                gap(i)
                sa = jnp.where(tri, s[:HB, n0:], NEG)
                sa = jnp.concatenate([s[:HB, :n0], sa], axis=1) if i > 0 else sa
                sb = s[HB:]
                s2 = jnp.where(tri, s2, NEG)
                da, db = deps.pop(0)
                ma = _after(jnp.max(sa, axis=1, keepdims=True), da)
                mb = _after(jnp.max(jnp.concatenate([sb, s2], axis=1), axis=1, keepdims=True), db)
                pa = jnp.exp2(sa - ma)
                pb = jnp.exp2(sb - mb)
                p2 = jnp.exp2(s2 - mb)
                la = _recip(jnp.sum(pa, axis=1, keepdims=True))
                lb = _recip(jnp.sum(jnp.concatenate([pb, p2], axis=1), axis=1, keepdims=True))
                deps.append((la, lb))
                p = jnp.concatenate([pa, pb], axis=0).astype(BF)
                o = jnp.dot(p, _up(vr[:n1 // 2, :]), preferred_element_type=F32)
                o2 = jnp.dot(p2.astype(BF), _up(vr[n1 // 2:n2 // 2, :]), preferred_element_type=F32)
                ctx_s[h, n0:n1, :] = (o[:HB] * la).astype(BF)
                ctx_s[h, n1:n2, :] = ((o[HB:] + o2) * lb).astype(BF)
            tail()
            return deps

        nodeps = [(None, None)] * cfg["dist"]
        nop = lambda *a: None

        with scope("p_kv"):
            with scope("w_kv"):
                w_wait(0, 0)
                w_wait(1, 0)
            w4_s[...] = _pk(jnp.concatenate([_unpack(z[:, 0], odd) for odd in (0, 1) for z in (zk, zv)], axis=1))

            def kv01(j):
                c = c_s[pl.ds(pl.multiple_of(j * TC, TC), TC), :]
                rows = pl.ds(pl.multiple_of(j * (TC // 2), TC // 2), TC // 2)
                cu_s[rows, :] = _pk(c)
                kv = jnp.dot(c, _up(w4_s[...]), preferred_element_type=F32)
                for n, dst in enumerate((k0_s, v0_s, k_s, v_s)):
                    dst[rows, :] = _pk(kv[:, n * D:(n + 1) * D].astype(BF))

            def kv_body(j, c):
                with scope("w_c"):
                    c_copy(j).wait()
                kv01(j)
                return c
            lax.fori_loop(0, S // TC - 1, kv_body, 0)
            with scope("w_x0"):
                c_copy(S // TC - 1).wait()
                w_wait(2, 0)
                x_copy(nq - 1).wait()
            ln1(nq - 1)
            kv01(S // TC - 1)
            wq0 = _unpack(zq[:, 0], 0)
            wq1 = _unpack(zq[:, 0], 1)
            q_piece(wq0, (nq - 1) * TQ)

        start_loop(nq // 2, nq - 1, lambda j: x_copy(j).wait())
        with scope("m_first"):
            def pre0(i):
                if i == nq - 1:
                    for j in range(3):
                        w_start(j, 1, 1)
                if i == nq // 2:
                    with scope("w_x2"):
                        for j in range(nq // 2):
                            x_copy(j).wait()

            def gap0(i):
                q_piece(wq1, i * TQ)
                if i > 0:
                    ln1(i - 1)
                    q_piece(wq0, (i - 1) * TQ)
            attention(0, k0_s, v0_s, pre0, gap0, nop, nodeps)

        def head(h, p, odd, deps):
            wq = _unpack(zq[:, p], odd)
            wkv = jnp.concatenate([_unpack(zk[:, p], odd), _unpack(zv[:, p], odd)], axis=1)

            def gap(i):
                if i > 0:
                    q_piece(wq, i * TQ)
                if i + 1 < nq:
                    kv_piece(wkv, (i + 1) * TQ)

            def tail():
                kv_piece(wkv, 0)
                q_piece(wq, 0)

            return attention(h, k_s, v_s, nop, gap, tail, deps)

        def heads(t, carry):
            p = t + 1

            @pl.when(p == PG[1])
            def _():
                for i in range(3):
                    w_start(i, 2, 1)

            @pl.when(p == PG[2])
            def _():
                for i in range(3):
                    w_wait(i, 2)
                for i in range(3):
                    w_start(i, 3, 1)

            @pl.when(p == PG[3])
            def _():
                for i in range(3):
                    w_wait(i, 3)
                for c in big:
                    c.start(priority=1)

            with scope("m_iter"):
                deps = head(2 * t + 1, p, 0, nodeps)
                head(2 * t + 2, p, 1, deps)
            return carry
        for i in range(3):
            w_wait(i, 1)
        with scope("m_loop"):
            lax.fori_loop(0, H // 2 - 1, heads, 0)
        with scope("m_last"):
            attention(H - 1, k_s, v_s, nop, nop, nop, nodeps)

        big[0].wait()
        big[1].wait()
        wr = wr_ref[...].astype(F32).reshape(1, M)
        ne = S // TE

        def out_copy(i):
            r0 = pl.multiple_of(i * TE, TE)
            return pltpu.make_async_copy(o_s.at[pl.ds(r0 + TE, TE), :], out_hbm.at[pl.ds(r0, TE), :], osem.at[i])

        def post(r0, hv, chain, top):
            dep = None
            b1, j1, b2, j2 = top
            for j in range(TE // CN):
                rows = pl.ds(r0 + j * CN, CN)
                hf = hv[j * CN:(j + 1) * CN, :].astype(F32)
                hn = _ln_rows(hf, dep)
                hnf = hn.astype(F32)
                r = _rb(jnp.sum(hnf * wr, axis=-1, keepdims=True))
                hn_s[rows, :] = hn
                o_s[rows, :] = (hf + hnf).astype(BF)
                dep = r if chain else None
                tok = lax.broadcasted_iota(jnp.int32, (CN, 1), 0) + (r0 + j * CN - TE)
                r = jnp.where(tok >= 0, r, -jnp.inf)
                gt1 = r > b1
                gt2 = r > b2
                b2 = jnp.where(gt1, b1, jnp.where(gt2, r, b2))
                j2 = jnp.where(gt1, j1, jnp.where(gt2, tok, j2))
                b1 = jnp.where(gt1, r, b1)
                j1 = jnp.where(gt1, tok, j1)
            return b1, j1, b2, j2

        h_s[0:TE, :] = jnp.zeros((TE, M), BF)

        def epi(i, top):
            r0 = pl.multiple_of(i * TE, TE)
            hv = h_s.at[pl.ds(r0, 2 * TE), :]
            top = post(r0, hv, True, top)
            ctx = jnp.concatenate([ctx_s[hh, pl.ds(r0, TE), :] for hh in range(H)], axis=1)
            a = jnp.dot(ctx, wo_s[...], preferred_element_type=F32)
            hv[TE:2 * TE, :] = (x_s[pl.ds(r0, TE), :].astype(F32) + _rb(a)).astype(BF)

            @pl.when(i > 0)
            def _():
                out_copy(i - 1).start()
            return top
        ninf = jnp.full((CN, 1), -jnp.inf, F32)
        none = jnp.full((CN, 1), S, jnp.int32)
        with scope("e_loop"):
            top = lax.fori_loop(0, ne, epi, (ninf, none, ninf, none))
        with scope("e_post"):
            top = post(S, h_s.at[S:S + TE, :], False, top)
            out_copy(ne - 1).start()

        with scope("t_top2"):
            r = jnp.concatenate([top[0], top[2]], axis=0)
            idx = jnp.concatenate([top[1], top[3]], axis=0)
            m1 = jnp.max(r, axis=0, keepdims=True)
            i1v = jnp.min(jnp.where(r == m1, idx, S), axis=0, keepdims=True)
            r2 = jnp.where(idx == i1v, -jnp.inf, r)
            m2 = jnp.max(r2, axis=0, keepdims=True)
            i2v = jnp.min(jnp.where((r2 == m2) & (idx != i1v), idx, S), axis=0, keepdims=True)
            i1 = jnp.minimum(jnp.min(i1v), S - 1)
            i2 = jnp.minimum(jnp.min(i2v), S - 1)
            b1 = pl.multiple_of(i1 & (-16), 16)
            b2 = pl.multiple_of(i2 & (-16), 16)
            rows16 = lax.broadcasted_iota(jnp.int32, (16, M), 0)
            hn1 = hn_s[pl.ds(b1 + TE, 16), :].astype(F32)
            hn2 = hn_s[pl.ds(b2 + TE, 16), :].astype(F32)
            x1 = jnp.sum(jnp.where(rows16 == i1 - b1, hn1, 0.0), axis=0, keepdims=True)
            x2 = jnp.sum(jnp.where(rows16 == i2 - b2, hn2, 0.0), axis=0, keepdims=True)
            xs = jnp.where(rows16 == 0, x1, jnp.where(rows16 == 1, x2, 0.0)).astype(BF)
        with scope("t_ffn"):
            for c in big[2:]:
                c.wait()
            g = _rb(jnp.dot(xs, wg_s[...], preferred_element_type=F32)[:8])
            u = _rb(jnp.dot(xs, wu_s[...], preferred_element_type=F32)[:8])
            g = _rb(g * jax.nn.sigmoid(g))
            gu = jnp.concatenate([g * u, jnp.zeros_like(g)], axis=0).astype(BF)
            y = _rb(jnp.dot(gu, wd_s[:, 0:M], preferred_element_type=F32)[:8])
            y1 = _rb(y[0:1, :] * _rb(jax.nn.sigmoid(m1)))
            y2 = _rb(y[1:2, :] * _rb(jax.nn.sigmoid(m2)))
        with scope("t_patch"):
            for i in range(ne):
                out_copy(i).wait()
            cps = []
            for n, (b, hnb) in enumerate(((b1, hn1), (b2, hn2))):
                rows = rows16 + b
                upd = jnp.where(rows == i1, y1, jnp.where(rows == i2, y2, 0.0))
                o_s[pl.ds(b + TE, 16), :] = (h_s[pl.ds(b + TE, 16), :].astype(F32) + _rb(hnb + upd)).astype(BF)
                cps.append(pltpu.make_async_copy(o_s.at[pl.ds(b + TE, 16), :], out_hbm.at[pl.ds(b, 16), :], osem.at[n]))
            cps[0].start()

            @pl.when(b1 != b2)
            def _():
                cps[1].start()
                cps[1].wait()
            cps[0].wait()

    @jax.jit
    def run(A_x, A_c_kv, A_w_q, A_w_uk, A_w_uv, A_w_o, B_x, B_w_r, B_w_gate, B_w_up, B_w_down):
        B, S, M = A_x.shape
        C = A_c_kv.shape[2]
        _, H, D = A_w_q.shape
        Fd = B_w_gate.shape[1]
        anyspec = pl.BlockSpec(memory_space=pl.ANY)
        out = pl.pallas_call(
            kernel,
            in_specs=[anyspec] * 10,
            out_specs=anyspec,
            out_shape=jax.ShapeDtypeStruct((S, M), BF),
            scratch_shapes=[
                pltpu.VMEM((S, M), BF), pltpu.VMEM((S, C), BF), pltpu.VMEM((S // 2, C), U32),
                pltpu.VMEM((M // 8, H // 2, 16, D), BF), pltpu.VMEM((C // 8, H // 2, 16, D), BF), pltpu.VMEM((C // 8, H // 2, 16, D), BF),
                pltpu.VMEM((H * D, M), BF),
                pltpu.VMEM((M, Fd), BF), pltpu.VMEM((M, Fd), BF), pltpu.VMEM((Fd, M + 128), BF), pltpu.VMEM((M,), BF),
                pltpu.VMEM((S // 2, M), U32),
                pltpu.VMEM((S, D), BF), pltpu.VMEM((S // 2, D), U32), pltpu.VMEM((S // 2, D), U32),
                pltpu.VMEM((S // 2, D), U32), pltpu.VMEM((S // 2, D), U32), pltpu.VMEM((C // 2, 4 * D), U32),
                pltpu.VMEM((H, S, D), BF),
                pltpu.VMEM((S + TE, M), BF), pltpu.VMEM((S + TE, M), BF), pltpu.VMEM((S + TE, M), BF),
                pltpu.SemaphoreType.DMA((5,)), pltpu.SemaphoreType.DMA((S // TQ,)), pltpu.SemaphoreType.DMA((S // TC,)),
                pltpu.SemaphoreType.DMA((12,)), pltpu.SemaphoreType.DMA((S // TE,)),
            ],
            compiler_params=pltpu.CompilerParams(vmem_limit_bytes=120 * 1024 * 1024),
            interpret=cfg.get("interpret", False),
        )(A_x.reshape(S, M), A_c_kv.reshape(S, C), A_w_q.reshape(M // 8, 8, H // 2, 2, D), A_w_uk.reshape(C // 8, 8, H // 2, 2, D),
          A_w_uv.reshape(C // 8, 8, H // 2, 2, D), A_w_o.reshape(H * D, M), B_w_r, B_w_gate, B_w_up, B_w_down)
        return out.reshape(B, S, M)

    return run


_RUN = make(dict(CFG, **{}))


@jax.jit
def pallas_sequential_preLN__compressed_kv_cla__moe_arch_mod__prompt_kernel(A_x, A_c_kv, A_w_q, A_w_uk, A_w_uv, A_w_o, B_x, B_w_r, B_w_gate, B_w_up, B_w_down):
    return _RUN(A_x, A_c_kv, A_w_q, A_w_uk, A_w_uv, A_w_o, B_x, B_w_r, B_w_gate, B_w_up, B_w_down)
```

```python
import contextlib
import math
import jax
import jax.numpy as jnp
from jax import lax
from jax.experimental import pallas as pl
from jax.experimental.pallas import tpu as pltpu

BF = jnp.bfloat16
F32 = jnp.float32
U32 = jnp.uint32
NT = (((1,), (1,)), ((), ()))
NEG = -1e30
EPS = 1e-5
BIG = 3e38

CFG = dict(TQ=256, TE=256, CN=16, dist=2, L1=16, TC=512)


def _rb(x):
    return x.astype(BF).astype(F32)


def _after(x, dep):
    return x if dep is None else jnp.maximum(x, dep - BIG)


def _recip(l):
    r = pl.reciprocal(l, approx=True)
    return r * (2.0 - l * r)


def _ln_rows(x, dep=None):
    n = x.shape[-1]
    mu = _after(jnp.sum(x, axis=-1, keepdims=True), dep) * (1.0 / n)
    xc = x - mu
    var = jnp.sum(xc * xc, axis=-1, keepdims=True) * (1.0 / n)
    den = _rb(jnp.sqrt(_rb(_rb(var) + EPS)))
    num = _rb(x - _rb(mu))
    return (num * (1.0 / den)).astype(BF)


def _unpack(z, odd):
    u = pltpu.bitcast(z, jnp.uint32)
    u = u.reshape(u.shape[0] * u.shape[1], u.shape[2])
    u = (u & jnp.uint32(0xFFFF0000)) if odd else (u << 16)
    return pltpu.bitcast(u, F32).astype(BF)


def _pk(x):
    return pltpu.bitcast(x, jnp.uint32)


def _up(u):
    return pltpu.bitcast(u, BF)


def make(cfg):
    TQ, TE, CN, L1, TC = cfg["TQ"], cfg["TE"], cfg["CN"], cfg["L1"], cfg["TC"]
    scope = jax.named_scope if cfg.get("scopes") else (lambda n: contextlib.nullcontext())

    def kernel(x_hbm, c_hbm, wq_hbm, wk_hbm, wv_hbm, wo_hbm, wr_hbm, wg_hbm, wu_hbm, wd_hbm,
               out_hbm,
               x_s, c_s, cu_s, zq, zk, zv, wo_s, wg_s, wu_s, wd_s, wr_ref,
               xn_s, q_s, k_s, v_s, k0_s, v0_s, w4_s, ctx_s, h_s, hn_s, o_s, sem, xsem, csem, wsem, osem):
        S, M = x_s.shape
        H, _, D = ctx_s.shape
        nq = S // TQ
        scale = (D ** -0.5) * math.log2(math.e)
        W = ((wk_hbm, zk), (wv_hbm, zv), (wq_hbm, zq))

        PG = (0, 1, 2, 5, H // 2)

        def w_start(i, g, priority):
            src, z = W[i]
            for r in range(8):
                pltpu.make_async_copy(src.at[:, r, PG[g]:PG[g + 1]], z.at[:, PG[g]:PG[g + 1], 2 * r:2 * r + 2, :],
                                      wsem.at[3 * g + i]).start(priority=priority)

        def w_wait(i, g):
            z = W[i][1].at[:, PG[g]:PG[g + 1]]
            pltpu.make_async_copy(z, z, wsem.at[3 * g + i]).wait()

        def x_copy(i):
            rows = pl.ds(pl.multiple_of(i * TQ, TQ), TQ)
            return pltpu.make_async_copy(x_hbm.at[rows, :], x_s.at[rows, :], xsem.at[i])

        def c_copy(i):
            rows = pl.ds(pl.multiple_of(i * TC, TC), TC)
            return pltpu.make_async_copy(c_hbm.at[rows, :], c_s.at[rows, :], csem.at[i])

        big = [pltpu.make_async_copy(src, dst, sem.at[i]) for i, (src, dst) in enumerate([
            (wo_hbm, wo_s), (wr_hbm, wr_ref), (wg_hbm, wg_s), (wu_hbm, wu_s), (wd_hbm, wd_s.at[:, 0:M])])]

        def start_loop(lo, hi, fn):
            def body(i, c):
                fn(i)
                return c
            lax.fori_loop(lo, hi, body, 0)

        w_start(0, 0, 0)
        w_start(1, 0, 0)
        c_copy(0).start()
        start_loop(1, S // TC, lambda j: c_copy(j).start(priority=1))
        w_start(2, 0, 1)
        start_loop(0, nq, lambda j: x_copy(nq - 1 - j).start(priority=1))

        def kv_piece(wkv, r0):
            rows = slice(r0 // 2, (r0 + TQ) // 2)
            kv = jnp.dot(_up(cu_s[rows, :]), wkv, preferred_element_type=F32)
            k_s[rows, :] = _pk(kv[:, :D].astype(BF))
            v_s[rows, :] = _pk(kv[:, D:].astype(BF))

        def q_piece(wq, r0):
            rows = slice(r0 // 2, (r0 + TQ) // 2)
            q = jnp.dot(_up(xn_s[rows, :]), wq, preferred_element_type=F32)
            q_s[r0:r0 + TQ, :] = (q * scale).astype(BF)

        def ln1(i):
            for j in range(TQ // L1):
                rows = slice(i * TQ + j * L1, i * TQ + (j + 1) * L1)
                x = x_s[rows, :].astype(F32)
                xc = x - jnp.sum(x, axis=-1, keepdims=True) * (1.0 / M)
                var = jnp.sum(xc * xc, axis=-1, keepdims=True) * (1.0 / M)
                xn_s[rows.start // 2:rows.stop // 2, :] = _pk((xc * lax.rsqrt(var + EPS)).astype(BF))

        def attention(h, kr, vr, pre, gap, tail, deps):
            HB = TQ // 2
            row = lax.broadcasted_iota(jnp.int32, (HB, HB), 0)
            col = lax.broadcasted_iota(jnp.int32, (HB, HB), 1)
            tri = col <= row
            deps = list(deps)
            for i in range(nq - 1, -1, -1):
                n0 = i * TQ
                n1 = n0 + HB
                pre(i)
                n2 = n0 + TQ
                q = q_s[n0:n2, :]
                s = lax.dot_general(q, _up(kr[:n1 // 2, :]), NT, preferred_element_type=F32)
                s2 = lax.dot_general(q[HB:], _up(kr[n1 // 2:n2 // 2, :]), NT, preferred_element_type=F32)
                gap(i)
                sa = jnp.where(tri, s[:HB, n0:], NEG)
                sa = jnp.concatenate([s[:HB, :n0], sa], axis=1) if i > 0 else sa
                sb = s[HB:]
                s2 = jnp.where(tri, s2, NEG)
                da, db = deps.pop(0)
                ma = _after(jnp.max(sa, axis=1, keepdims=True), da)
                mb = _after(jnp.max(jnp.concatenate([sb, s2], axis=1), axis=1, keepdims=True), db)
                pa = jnp.exp2(sa - ma)
                pb = jnp.exp2(sb - mb)
                p2 = jnp.exp2(s2 - mb)
                la = _recip(jnp.sum(pa, axis=1, keepdims=True))
                lb = _recip(jnp.sum(jnp.concatenate([pb, p2], axis=1), axis=1, keepdims=True))
                deps.append((la, lb))
                p = jnp.concatenate([pa, pb], axis=0).astype(BF)
                o = jnp.dot(p, _up(vr[:n1 // 2, :]), preferred_element_type=F32)
                o2 = jnp.dot(p2.astype(BF), _up(vr[n1 // 2:n2 // 2, :]), preferred_element_type=F32)
                ctx_s[h, n0:n1, :] = (o[:HB] * la).astype(BF)
                ctx_s[h, n1:n2, :] = ((o[HB:] + o2) * lb).astype(BF)
            tail()
            return deps

        nodeps = [(None, None)] * cfg["dist"]
        nop = lambda *a: None

        with scope("p_kv"):
            with scope("w_kv"):
                w_wait(0, 0)
                w_wait(1, 0)
            w4_s[...] = _pk(jnp.concatenate([_unpack(z[:, 0], odd) for odd in (0, 1) for z in (zk, zv)], axis=1))

            def kv01(j):
                c = c_s[pl.ds(pl.multiple_of(j * TC, TC), TC), :]
                rows = pl.ds(pl.multiple_of(j * (TC // 2), TC // 2), TC // 2)
                cu_s[rows, :] = _pk(c)
                kv = jnp.dot(c, _up(w4_s[...]), preferred_element_type=F32)
                for n, dst in enumerate((k0_s, v0_s, k_s, v_s)):
                    dst[rows, :] = _pk(kv[:, n * D:(n + 1) * D].astype(BF))

            def kv_body(j, c):
                with scope("w_c"):
                    c_copy(j).wait()
                kv01(j)
                return c
            lax.fori_loop(0, S // TC - 1, kv_body, 0)
            with scope("w_x0"):
                c_copy(S // TC - 1).wait()
                w_wait(2, 0)
                x_copy(nq - 1).wait()
            ln1(nq - 1)
            kv01(S // TC - 1)
            wq0 = _unpack(zq[:, 0], 0)
            wq1 = _unpack(zq[:, 0], 1)
            q_piece(wq0, (nq - 1) * TQ)

        start_loop(nq // 2, nq - 1, lambda j: x_copy(j).wait())
        with scope("m_first"):
            def pre0(i):
                if i == nq - 1:
                    for j in range(3):
                        w_start(j, 1, 1)
                if i == nq // 2:
                    with scope("w_x2"):
                        for j in range(nq // 2):
                            x_copy(j).wait()

            def gap0(i):
                q_piece(wq1, i * TQ)
                if i > 0:
                    ln1(i - 1)
                    q_piece(wq0, (i - 1) * TQ)
            attention(0, k0_s, v0_s, pre0, gap0, nop, nodeps)

        def head(h, p, odd, deps):
            wq = _unpack(zq[:, p], odd)
            wkv = jnp.concatenate([_unpack(zk[:, p], odd), _unpack(zv[:, p], odd)], axis=1)

            def gap(i):
                if i > 0:
                    q_piece(wq, i * TQ)
                if i + 1 < nq:
                    kv_piece(wkv, (i + 1) * TQ)

            def tail():
                kv_piece(wkv, 0)
                q_piece(wq, 0)

            return attention(h, k_s, v_s, nop, gap, tail, deps)

        def heads(t, carry):
            p = t + 1

            @pl.when(p == PG[1])
            def _():
                for i in range(3):
                    w_start(i, 2, 1)

            @pl.when(p == PG[2])
            def _():
                for i in range(3):
                    w_wait(i, 2)
                for i in range(3):
                    w_start(i, 3, 1)

            @pl.when(p == PG[3])
            def _():
                for i in range(3):
                    w_wait(i, 3)
                for c in big:
                    c.start(priority=1)

            with scope("m_iter"):
                deps = head(2 * t + 1, p, 0, nodeps)
                head(2 * t + 2, p, 1, deps)
            return carry
        for i in range(3):
            w_wait(i, 1)
        with scope("m_loop"):
            lax.fori_loop(0, H // 2 - 1, heads, 0)

        big[0].wait()
        big[1].wait()
        wr = wr_ref[...].astype(F32).reshape(1, M)
        ne = S // TE

        def out_copy(i):
            rows = pl.ds(pl.multiple_of(i * TE, TE), TE)
            return pltpu.make_async_copy(o_s.at[rows, :], out_hbm.at[rows, :], osem.at[i])

        def post(r0, hv, chain, top):
            dep = None
            b1, j1, b2, j2 = top
            for j in range(TE // CN - 1, -1, -1):
                rows = pl.ds(r0 + j * CN, CN)
                hf = hv[j * CN:(j + 1) * CN, :].astype(F32)
                hn = _ln_rows(hf, dep)
                hnf = hn.astype(F32)
                r = _rb(jnp.sum(hnf * wr, axis=-1, keepdims=True))
                hn_s[rows, :] = hn
                o_s[rows, :] = (hf + hnf).astype(BF)
                dep = r if chain else None
                tok = lax.broadcasted_iota(jnp.int32, (CN, 1), 0) + (r0 + j * CN)
                ge1 = r >= b1
                ge2 = r >= b2
                b2 = jnp.where(ge1, b1, jnp.where(ge2, r, b2))
                j2 = jnp.where(ge1, j1, jnp.where(ge2, tok, j2))
                b1 = jnp.where(ge1, r, b1)
                j1 = jnp.where(ge1, tok, j1)
            return b1, j1, b2, j2

        def o_piece(n):
            rows = slice(S - TE, S)
            cols = slice(n * (M // nq), (n + 1) * (M // nq))
            ctx = jnp.concatenate([ctx_s[hh, rows, :] for hh in range(H)], axis=1)
            a = jnp.dot(ctx, wo_s[:, cols], preferred_element_type=F32)
            h_s[rows, cols] = (x_s[rows, cols].astype(F32) + _rb(a)).astype(BF)

        with scope("m_last"):
            attention(H - 1, k_s, v_s, nop, lambda i: o_piece(i + 1) if i + 1 < nq else None, lambda: o_piece(0), nodeps)

        def epi(t, top):
            i = ne - 2 - t
            r0 = pl.multiple_of(i * TE, TE)
            hv = h_s.at[pl.ds(r0, 2 * TE), :]
            top = post(r0 + TE, hv.at[TE:2 * TE, :], True, top)
            ctx = jnp.concatenate([ctx_s[hh, pl.ds(r0, TE), :] for hh in range(H)], axis=1)
            a = jnp.dot(ctx, wo_s[...], preferred_element_type=F32)
            hv[0:TE, :] = (x_s[pl.ds(r0, TE), :].astype(F32) + _rb(a)).astype(BF)
            out_copy(i + 1).start()
            return top
        ninf = jnp.full((CN, 1), -jnp.inf, F32)
        none = jnp.full((CN, 1), S, jnp.int32)
        with scope("e_loop"):
            top = lax.fori_loop(0, ne - 1, epi, (ninf, none, ninf, none))
        with scope("e_post"):
            top = post(0, h_s.at[0:TE, :], False, top)
            out_copy(0).start()

        with scope("t_top2"):
            r = jnp.concatenate([top[0], top[2]], axis=0)
            idx = jnp.concatenate([top[1], top[3]], axis=0)
            m1 = jnp.max(r, axis=0, keepdims=True)
            i1v = jnp.min(jnp.where(r == m1, idx, S), axis=0, keepdims=True)
            r2 = jnp.where(idx == i1v, -jnp.inf, r)
            m2 = jnp.max(r2, axis=0, keepdims=True)
            i2v = jnp.min(jnp.where((r2 == m2) & (idx != i1v), idx, S), axis=0, keepdims=True)
            i1 = jnp.minimum(jnp.min(i1v), S - 1)
            i2 = jnp.minimum(jnp.min(i2v), S - 1)
            b1 = pl.multiple_of(i1 & (-16), 16)
            b2 = pl.multiple_of(i2 & (-16), 16)
            rows16 = lax.broadcasted_iota(jnp.int32, (16, M), 0)
            hn1 = hn_s[pl.ds(b1, 16), :].astype(F32)
            hn2 = hn_s[pl.ds(b2, 16), :].astype(F32)
            x1 = jnp.sum(jnp.where(rows16 == i1 - b1, hn1, 0.0), axis=0, keepdims=True)
            x2 = jnp.sum(jnp.where(rows16 == i2 - b2, hn2, 0.0), axis=0, keepdims=True)
            xs = jnp.where(rows16 == 0, x1, jnp.where(rows16 == 1, x2, 0.0)).astype(BF)
        with scope("t_ffn"):
            for c in big[2:]:
                c.wait()
            g = _rb(jnp.dot(xs, wg_s[...], preferred_element_type=F32)[:8])
            u = _rb(jnp.dot(xs, wu_s[...], preferred_element_type=F32)[:8])
            g = _rb(g * jax.nn.sigmoid(g))
            gu = jnp.concatenate([g * u, jnp.zeros_like(g)], axis=0).astype(BF)
            y = _rb(jnp.dot(gu, wd_s[:, 0:M], preferred_element_type=F32)[:8])
            y1 = _rb(y[0:1, :] * _rb(jax.nn.sigmoid(m1)))
            y2 = _rb(y[1:2, :] * _rb(jax.nn.sigmoid(m2)))
        with scope("t_patch"):
            for i in range(ne):
                out_copy(i).wait()
            cps = []
            for n, (b, hnb) in enumerate(((b1, hn1), (b2, hn2))):
                rows = rows16 + b
                upd = jnp.where(rows == i1, y1, jnp.where(rows == i2, y2, 0.0))
                o_s[pl.ds(b, 16), :] = (h_s[pl.ds(b, 16), :].astype(F32) + _rb(hnb + upd)).astype(BF)
                cps.append(pltpu.make_async_copy(o_s.at[pl.ds(b, 16), :], out_hbm.at[pl.ds(b, 16), :], osem.at[n]))
            cps[0].start()

            @pl.when(b1 != b2)
            def _():
                cps[1].start()
                cps[1].wait()
            cps[0].wait()

    @jax.jit
    def run(A_x, A_c_kv, A_w_q, A_w_uk, A_w_uv, A_w_o, B_x, B_w_r, B_w_gate, B_w_up, B_w_down):
        B, S, M = A_x.shape
        C = A_c_kv.shape[2]
        _, H, D = A_w_q.shape
        Fd = B_w_gate.shape[1]
        anyspec = pl.BlockSpec(memory_space=pl.ANY)
        out = pl.pallas_call(
            kernel,
            in_specs=[anyspec] * 10,
            out_specs=anyspec,
            out_shape=jax.ShapeDtypeStruct((S, M), BF),
            scratch_shapes=[
                pltpu.VMEM((S, M), BF), pltpu.VMEM((S, C), BF), pltpu.VMEM((S // 2, C), U32),
                pltpu.VMEM((M // 8, H // 2, 16, D), BF), pltpu.VMEM((C // 8, H // 2, 16, D), BF), pltpu.VMEM((C // 8, H // 2, 16, D), BF),
                pltpu.VMEM((H * D, M), BF),
                pltpu.VMEM((M, Fd), BF), pltpu.VMEM((M, Fd), BF), pltpu.VMEM((Fd, M + 128), BF), pltpu.VMEM((M,), BF),
                pltpu.VMEM((S // 2, M), U32),
                pltpu.VMEM((S, D), BF), pltpu.VMEM((S // 2, D), U32), pltpu.VMEM((S // 2, D), U32),
                pltpu.VMEM((S // 2, D), U32), pltpu.VMEM((S // 2, D), U32), pltpu.VMEM((C // 2, 4 * D), U32),
                pltpu.VMEM((H, S, D), BF),
                pltpu.VMEM((S, M), BF), pltpu.VMEM((S, M), BF), pltpu.VMEM((S, M), BF),
                pltpu.SemaphoreType.DMA((5,)), pltpu.SemaphoreType.DMA((S // TQ,)), pltpu.SemaphoreType.DMA((S // TC,)),
                pltpu.SemaphoreType.DMA((12,)), pltpu.SemaphoreType.DMA((S // TE,)),
            ],
            compiler_params=pltpu.CompilerParams(vmem_limit_bytes=120 * 1024 * 1024),
            interpret=cfg.get("interpret", False),
        )(A_x.reshape(S, M), A_c_kv.reshape(S, C), A_w_q.reshape(M // 8, 8, H // 2, 2, D), A_w_uk.reshape(C // 8, 8, H // 2, 2, D),
          A_w_uv.reshape(C // 8, 8, H // 2, 2, D), A_w_o.reshape(H * D, M), B_w_r, B_w_gate, B_w_up, B_w_down)
        return out.reshape(B, S, M)

    return run


_RUN = make(dict(CFG, **{}))


@jax.jit
def pallas_sequential_preLN__compressed_kv_cla__moe_arch_mod__prompt_kernel(A_x, A_c_kv, A_w_q, A_w_uk, A_w_uv, A_w_o, B_x, B_w_r, B_w_gate, B_w_up, B_w_down):
    return _RUN(A_x, A_c_kv, A_w_q, A_w_uk, A_w_uv, A_w_o, B_x, B_w_r, B_w_gate, B_w_up, B_w_down)
```

```python
import contextlib
import math
import jax
import jax.numpy as jnp
from jax import lax
from jax.experimental import pallas as pl
from jax.experimental.pallas import tpu as pltpu

BF = jnp.bfloat16
F32 = jnp.float32
U32 = jnp.uint32
NT = (((1,), (1,)), ((), ()))
NEG = -1e30
EPS = 1e-5
BIG = 3e38

CFG = dict(TQ=256, TE=256, CN=16, dist=2, L1=16, TC=512, UE=1, TB=64, nch=1)


def _rb(x):
    return x.astype(BF).astype(F32)


def _after(x, dep):
    return x if dep is None else jnp.maximum(x, dep - BIG)


def _recip(l):
    r = pl.reciprocal(l, approx=True)
    return r * (2.0 - l * r)


def _ln_rows(x, dep=None):
    n = x.shape[-1]
    mu = _after(jnp.sum(x, axis=-1, keepdims=True), dep) * (1.0 / n)
    xc = x - mu
    var = jnp.sum(xc * xc, axis=-1, keepdims=True) * (1.0 / n)
    den = _rb(jnp.sqrt(_rb(_rb(var) + EPS)))
    num = _rb(x - _rb(mu))
    return (num * (1.0 / den)).astype(BF)


def _unpack(z, odd):
    u = pltpu.bitcast(z, jnp.uint32)
    u = u.reshape(u.shape[0] * u.shape[1], u.shape[2])
    u = (u & jnp.uint32(0xFFFF0000)) if odd else (u << 16)
    return pltpu.bitcast(u, F32).astype(BF)


def _pk(x):
    return pltpu.bitcast(x, jnp.uint32)


def _up(u):
    return pltpu.bitcast(u, BF)


def make(cfg):
    TQ, TE, CN, L1, TC = cfg["TQ"], cfg["TE"], cfg["CN"], cfg["L1"], cfg["TC"]
    scope = jax.named_scope if cfg.get("scopes") else (lambda n: contextlib.nullcontext())

    def kernel(x_hbm, c_hbm, wq_hbm, wk_hbm, wv_hbm, wo_hbm, wr_hbm, wg_hbm, wu_hbm, wd_hbm,
               out_hbm,
               x_s, c_s, cu_s, zq, zk, zv, wo_s, wg_s, wu_s, wd_s, wr_ref,
               xn_s, q_s, k_s, v_s, k0_s, v0_s, w4_s, ctx_s, h_s, hn_s, o_s, sem, xsem, csem, wsem, osem):
        S, M = x_s.shape
        H, _, D = ctx_s.shape
        nq = S // TQ
        scale = (D ** -0.5) * math.log2(math.e)
        W = ((wk_hbm, zk), (wv_hbm, zv), (wq_hbm, zq))

        PG = (0, 1, 2, 5, H // 2)

        def w_start(i, g, priority):
            src, z = W[i]
            for r in range(8):
                pltpu.make_async_copy(src.at[:, r, PG[g]:PG[g + 1]], z.at[:, PG[g]:PG[g + 1], 2 * r:2 * r + 2, :],
                                      wsem.at[3 * g + i]).start(priority=priority)

        def w_wait(i, g):
            z = W[i][1].at[:, PG[g]:PG[g + 1]]
            pltpu.make_async_copy(z, z, wsem.at[3 * g + i]).wait()

        def x_copy(i):
            rows = pl.ds(pl.multiple_of(i * TQ, TQ), TQ)
            return pltpu.make_async_copy(x_hbm.at[rows, :], x_s.at[rows, :], xsem.at[i])

        def c_copy(i):
            rows = pl.ds(pl.multiple_of(i * TC, TC), TC)
            return pltpu.make_async_copy(c_hbm.at[rows, :], c_s.at[rows, :], csem.at[i])

        big = [pltpu.make_async_copy(src, dst, sem.at[i]) for i, (src, dst) in enumerate([
            (wo_hbm, wo_s.at[:, 0:M]), (wr_hbm, wr_ref), (wg_hbm, wg_s), (wu_hbm, wu_s), (wd_hbm, wd_s.at[:, 0:M])])]

        def start_loop(lo, hi, fn):
            def body(i, c):
                fn(i)
                return c
            lax.fori_loop(lo, hi, body, 0)

        w_start(0, 0, 0)
        w_start(1, 0, 0)
        c_copy(0).start()
        start_loop(1, S // TC, lambda j: c_copy(j).start(priority=1))
        w_start(2, 0, 1)
        start_loop(0, nq, lambda j: x_copy(nq - 1 - j).start(priority=1))

        def kv_piece(wkv, r0):
            rows = slice(r0 // 2, (r0 + TQ) // 2)
            kv = jnp.dot(_up(cu_s[rows, :]), wkv, preferred_element_type=F32)
            k_s[rows, :] = _pk(kv[:, :D].astype(BF))
            v_s[rows, :] = _pk(kv[:, D:].astype(BF))

        def q_piece(wq, r0):
            rows = slice(r0 // 2, (r0 + TQ) // 2)
            q = jnp.dot(_up(xn_s[rows, :]), wq, preferred_element_type=F32)
            q_s[r0:r0 + TQ, :] = (q * scale).astype(BF)

        def ln1(i):
            for j in range(TQ // L1):
                rows = slice(i * TQ + j * L1, i * TQ + (j + 1) * L1)
                x = x_s[rows, :].astype(F32)
                xc = x - jnp.sum(x, axis=-1, keepdims=True) * (1.0 / M)
                var = jnp.sum(xc * xc, axis=-1, keepdims=True) * (1.0 / M)
                xn_s[rows.start // 2:rows.stop // 2, :] = _pk((xc * lax.rsqrt(var + EPS)).astype(BF))

        def attention(h, kr, vr, pre, gap, tail, deps):
            HB = TQ // 2
            row = lax.broadcasted_iota(jnp.int32, (HB, HB), 0)
            col = lax.broadcasted_iota(jnp.int32, (HB, HB), 1)
            tri = col <= row
            deps = list(deps)
            for i in range(nq - 1, -1, -1):
                n0 = i * TQ
                n1 = n0 + HB
                pre(i)
                n2 = n0 + TQ
                q = q_s[n0:n2, :]
                s = lax.dot_general(q, _up(kr[:n1 // 2, :]), NT, preferred_element_type=F32)
                s2 = lax.dot_general(q[HB:], _up(kr[n1 // 2:n2 // 2, :]), NT, preferred_element_type=F32)
                gap(i)
                sa = jnp.where(tri, s[:HB, n0:], NEG)
                sa = jnp.concatenate([s[:HB, :n0], sa], axis=1) if i > 0 else sa
                sb = s[HB:]
                s2 = jnp.where(tri, s2, NEG)
                da, db = deps.pop(0)
                ma = _after(jnp.max(sa, axis=1, keepdims=True), da)
                mb = _after(jnp.max(jnp.concatenate([sb, s2], axis=1), axis=1, keepdims=True), db)
                pa = jnp.exp2(sa - ma)
                pb = jnp.exp2(sb - mb)
                p2 = jnp.exp2(s2 - mb)
                la = _recip(jnp.sum(pa, axis=1, keepdims=True))
                lb = _recip(jnp.sum(jnp.concatenate([pb, p2], axis=1), axis=1, keepdims=True))
                deps.append((la, lb))
                p = jnp.concatenate([pa, pb], axis=0).astype(BF)
                o = jnp.dot(p, _up(vr[:n1 // 2, :]), preferred_element_type=F32)
                o2 = jnp.dot(p2.astype(BF), _up(vr[n1 // 2:n2 // 2, :]), preferred_element_type=F32)
                ctx_s[h, n0:n1, :] = (o[:HB] * la).astype(BF)
                ctx_s[h, n1:n2, :] = ((o[HB:] + o2) * lb).astype(BF)
            tail()
            return deps

        nodeps = [(None, None)] * cfg["dist"]
        nop = lambda *a: None

        with scope("p_kv"):
            with scope("w_kv"):
                w_wait(0, 0)
                w_wait(1, 0)
            w4_s[...] = _pk(jnp.concatenate([_unpack(z[:, 0], odd) for odd in (0, 1) for z in (zk, zv)], axis=1))

            def kv01(j):
                c = c_s[pl.ds(pl.multiple_of(j * TC, TC), TC), :]
                rows = pl.ds(pl.multiple_of(j * (TC // 2), TC // 2), TC // 2)
                cu_s[rows, :] = _pk(c)
                kv = jnp.dot(c, _up(w4_s[...]), preferred_element_type=F32)
                for n, dst in enumerate((k0_s, v0_s, k_s, v_s)):
                    dst[rows, :] = _pk(kv[:, n * D:(n + 1) * D].astype(BF))

            def kv_body(j, c):
                with scope("w_c"):
                    c_copy(j).wait()
                kv01(j)
                return c
            lax.fori_loop(0, S // TC - 1, kv_body, 0)
            with scope("w_x0"):
                c_copy(S // TC - 1).wait()
                w_wait(2, 0)
                x_copy(nq - 1).wait()
            ln1(nq - 1)
            kv01(S // TC - 1)
            wq0 = _unpack(zq[:, 0], 0)
            wq1 = _unpack(zq[:, 0], 1)
            q_piece(wq0, (nq - 1) * TQ)

        start_loop(nq // 2, nq - 1, lambda j: x_copy(j).wait())
        with scope("m_first"):
            def pre0(i):
                if i == nq - 1:
                    for j in range(3):
                        w_start(j, 1, 1)
                if i == nq // 2:
                    with scope("w_x2"):
                        for j in range(nq // 2):
                            x_copy(j).wait()

            def gap0(i):
                q_piece(wq1, i * TQ)
                if i > 0:
                    ln1(i - 1)
                    q_piece(wq0, (i - 1) * TQ)
            attention(0, k0_s, v0_s, pre0, gap0, nop, nodeps)

        def head(h, p, odd, deps):
            wq = _unpack(zq[:, p], odd)
            wkv = jnp.concatenate([_unpack(zk[:, p], odd), _unpack(zv[:, p], odd)], axis=1)

            def gap(i):
                if i > 0:
                    q_piece(wq, i * TQ)
                if i + 1 < nq:
                    kv_piece(wkv, (i + 1) * TQ)

            def tail():
                kv_piece(wkv, 0)
                q_piece(wq, 0)

            return attention(h, k_s, v_s, nop, gap, tail, deps)

        def heads(t, carry):
            p = t + 1

            @pl.when(p == PG[1])
            def _():
                for i in range(3):
                    w_start(i, 2, 1)

            @pl.when(p == PG[2])
            def _():
                for i in range(3):
                    w_wait(i, 2)
                for i in range(3):
                    w_start(i, 3, 1)

            @pl.when(p == PG[3])
            def _():
                for i in range(3):
                    w_wait(i, 3)
                for c in big:
                    c.start(priority=1)

            with scope("m_iter"):
                deps = head(2 * t + 1, p, 0, nodeps)
                head(2 * t + 2, p, 1, deps)
            return carry
        for i in range(3):
            w_wait(i, 1)
        with scope("m_loop"):
            lax.fori_loop(0, H // 2 - 1, heads, 0)

        big[0].wait()
        big[1].wait()
        wr = wr_ref[...].astype(F32).reshape(1, M)
        ne = S // TE

        def out_copy(i):
            rows = pl.ds(pl.multiple_of(i * TE, TE), TE)
            return pltpu.make_async_copy(o_s.at[rows, :], out_hbm.at[rows, :], osem.at[i])

        def post(r0, hv, n, deps, top):
            b1, j1, b2, j2 = top
            for j in range(n // CN - 1, -1, -1):
                rows = pl.ds(r0 + j * CN, CN)
                hf = hv[j * CN:(j + 1) * CN, :].astype(F32)
                hn = _ln_rows(hf, deps.pop(0))
                hnf = hn.astype(F32)
                r = _rb(jnp.sum(hnf * wr, axis=-1, keepdims=True))
                hn_s[rows, :] = hn
                o_s[rows, :] = (hf + hnf).astype(BF)
                deps.append(r)
                tok = lax.broadcasted_iota(jnp.int32, (CN, 1), 0) + (r0 + j * CN)
                ge1 = r >= b1
                ge2 = r >= b2
                b2 = jnp.where(ge1, b1, jnp.where(ge2, r, b2))
                j2 = jnp.where(ge1, j1, jnp.where(ge2, tok, j2))
                b1 = jnp.where(ge1, r, b1)
                j1 = jnp.where(ge1, tok, j1)
            return b1, j1, b2, j2

        def o_proj(r0, n, hv, cols=slice(0, M)):
            rows = pl.ds(r0, n)
            ctx = jnp.concatenate([ctx_s[hh, rows, :] for hh in range(H)], axis=1)
            a = jnp.dot(ctx, wo_s[:, cols], preferred_element_type=F32)
            hv[:, cols] = (x_s[rows, cols].astype(F32) + _rb(a)).astype(BF)

        def o_piece(n):
            o_proj(S - TE, TE, h_s.at[S - TE:S, :], slice(n * (M // nq), (n + 1) * (M // nq)))

        with scope("m_last"):
            attention(H - 1, k_s, v_s, nop, lambda i: o_piece(i + 1) if i + 1 < nq else None, lambda: o_piece(0), nodeps)

        UE = cfg["UE"]

        def epi(t, top):
            lo = ne - 1 - UE * (t + 1)
            r0 = pl.multiple_of(lo * TE, TE)
            hv = h_s.at[pl.ds(r0, (UE + 1) * TE), :]
            deps = [None]
            for u in range(UE - 1, -1, -1):
                top = post(r0 + (u + 1) * TE, hv.at[(u + 1) * TE:(u + 2) * TE, :], TE, deps, top)
                o_proj(r0 + u * TE, TE, hv.at[u * TE:(u + 1) * TE, :])
            for u in range(UE):
                out_copy(lo + u + 1).start()
            return top
        ninf = jnp.full((CN, 1), -jnp.inf, F32)
        none = jnp.full((CN, 1), S, jnp.int32)
        with scope("e_loop"):
            top = lax.fori_loop(0, (ne - 2) // UE, epi, (ninf, none, ninf, none))
        for c in big[2:]:
            c.wait()
        with scope("e_post"):
            TB = cfg["TB"]
            deps = [None]
            top = post(TE, h_s.at[TE:2 * TE, :], TE, deps, top)
            o_proj(TB, TE - TB, h_s.at[TB:TE, :])
            out_copy(1).start()
            deps = deps * cfg["nch"]
            top = post(TB, h_s.at[TB:TE, :], TE - TB, deps, top)
            o_proj(0, TB, h_s.at[0:TB, :])
            top = post(0, h_s.at[0:TB, :], TB, [deps[-1]] * (TB // CN), top)
            out_copy(0).start()

        with scope("t_top2"):
            r = jnp.concatenate([top[0], top[2]], axis=0)
            idx = jnp.concatenate([top[1], top[3]], axis=0)
            m1 = jnp.max(r, axis=0, keepdims=True)
            i1v = jnp.min(jnp.where(r == m1, idx, S), axis=0, keepdims=True)
            r2 = jnp.where(idx == i1v, -jnp.inf, r)
            m2 = jnp.max(r2, axis=0, keepdims=True)
            i2v = jnp.min(jnp.where((r2 == m2) & (idx != i1v), idx, S), axis=0, keepdims=True)
            i1 = jnp.minimum(jnp.min(i1v), S - 1)
            i2 = jnp.minimum(jnp.min(i2v), S - 1)
            b1 = pl.multiple_of(i1 & (-16), 16)
            b2 = pl.multiple_of(i2 & (-16), 16)
            rows16 = lax.broadcasted_iota(jnp.int32, (16, M), 0)
            hn1 = hn_s[pl.ds(b1, 16), :].astype(F32)
            hn2 = hn_s[pl.ds(b2, 16), :].astype(F32)
            x1 = jnp.sum(jnp.where(rows16 == i1 - b1, hn1, 0.0), axis=0, keepdims=True)
            x2 = jnp.sum(jnp.where(rows16 == i2 - b2, hn2, 0.0), axis=0, keepdims=True)
            xs = jnp.where(rows16 == 0, x1, jnp.where(rows16 == 1, x2, 0.0)).astype(BF)
        with scope("t_ffn"):
            g = _rb(jnp.dot(xs, wg_s[...], preferred_element_type=F32)[:8])
            u = _rb(jnp.dot(xs, wu_s[...], preferred_element_type=F32)[:8])
            g = _rb(g * jax.nn.sigmoid(g))
            gu = jnp.concatenate([g * u, jnp.zeros_like(g)], axis=0).astype(BF)
            y = _rb(jnp.dot(gu, wd_s[:, 0:M], preferred_element_type=F32)[:8])
            y1 = _rb(y[0:1, :] * _rb(jax.nn.sigmoid(m1)))
            y2 = _rb(y[1:2, :] * _rb(jax.nn.sigmoid(m2)))
        with scope("t_patch"):
            for i in range(ne):
                out_copy(i).wait()
            cps = []
            for n, (b, hnb) in enumerate(((b1, hn1), (b2, hn2))):
                rows = rows16 + b
                upd = jnp.where(rows == i1, y1, jnp.where(rows == i2, y2, 0.0))
                o_s[pl.ds(b, 16), :] = (h_s[pl.ds(b, 16), :].astype(F32) + _rb(hnb + upd)).astype(BF)
                cps.append(pltpu.make_async_copy(o_s.at[pl.ds(b, 16), :], out_hbm.at[pl.ds(b, 16), :], osem.at[n]))
            cps[0].start()

            @pl.when(b1 != b2)
            def _():
                cps[1].start()
                cps[1].wait()
            cps[0].wait()

    @jax.jit
    def run(A_x, A_c_kv, A_w_q, A_w_uk, A_w_uv, A_w_o, B_x, B_w_r, B_w_gate, B_w_up, B_w_down):
        B, S, M = A_x.shape
        C = A_c_kv.shape[2]
        _, H, D = A_w_q.shape
        Fd = B_w_gate.shape[1]
        anyspec = pl.BlockSpec(memory_space=pl.ANY)
        out = pl.pallas_call(
            kernel,
            in_specs=[anyspec] * 10,
            out_specs=anyspec,
            out_shape=jax.ShapeDtypeStruct((S, M), BF),
            scratch_shapes=[
                pltpu.VMEM((S, M), BF), pltpu.VMEM((S, C), BF), pltpu.VMEM((S // 2, C), U32),
                pltpu.VMEM((M // 8, H // 2, 16, D), BF), pltpu.VMEM((C // 8, H // 2, 16, D), BF), pltpu.VMEM((C // 8, H // 2, 16, D), BF),
                pltpu.VMEM((H * D, M + 128), BF),
                pltpu.VMEM((M, Fd), BF), pltpu.VMEM((M, Fd), BF), pltpu.VMEM((Fd, M + 128), BF), pltpu.VMEM((M,), BF),
                pltpu.VMEM((S // 2, M), U32),
                pltpu.VMEM((S, D), BF), pltpu.VMEM((S // 2, D), U32), pltpu.VMEM((S // 2, D), U32),
                pltpu.VMEM((S // 2, D), U32), pltpu.VMEM((S // 2, D), U32), pltpu.VMEM((C // 2, 4 * D), U32),
                pltpu.VMEM((H, S, D), BF),
                pltpu.VMEM((S, M), BF), pltpu.VMEM((S, M), BF), pltpu.VMEM((S, M), BF),
                pltpu.SemaphoreType.DMA((5,)), pltpu.SemaphoreType.DMA((S // TQ,)), pltpu.SemaphoreType.DMA((S // TC,)),
                pltpu.SemaphoreType.DMA((12,)), pltpu.SemaphoreType.DMA((S // TE,)),
            ],
            compiler_params=pltpu.CompilerParams(vmem_limit_bytes=120 * 1024 * 1024),
            interpret=cfg.get("interpret", False),
        )(A_x.reshape(S, M), A_c_kv.reshape(S, C), A_w_q.reshape(M // 8, 8, H // 2, 2, D), A_w_uk.reshape(C // 8, 8, H // 2, 2, D),
          A_w_uv.reshape(C // 8, 8, H // 2, 2, D), A_w_o.reshape(H * D, M), B_w_r, B_w_gate, B_w_up, B_w_down)
        return out.reshape(B, S, M)

    return run


_RUN = make(dict(CFG, **{}))


@jax.jit
def pallas_sequential_preLN__compressed_kv_cla__moe_arch_mod__prompt_kernel(A_x, A_c_kv, A_w_q, A_w_uk, A_w_uv, A_w_o, B_x, B_w_r, B_w_gate, B_w_up, B_w_down):
    return _RUN(A_x, A_c_kv, A_w_q, A_w_uk, A_w_uv, A_w_o, B_x, B_w_r, B_w_gate, B_w_up, B_w_down)
```

```python
import math

import jax
import jax.numpy as jnp
from jax import lax
from jax.experimental import pallas as pl
from jax.experimental.pallas import tpu as pltpu

BF = jnp.bfloat16
F32 = jnp.float32
U32 = jnp.uint32
NT = (((1,), (1,)), ((), ()))
NEG = -1e30
EPS = 1e-5
BIG = 3e38

TQ = 256
TC = 512
TE = 256
TB = 64
CN = 16
DIST = 2


def _rb(x):
    return x.astype(BF).astype(F32)


def _after(x, dep):
    return x if dep is None else jnp.maximum(x, dep - BIG)


def _recip(l):
    r = pl.reciprocal(l, approx=True)
    return r * (2.0 - l * r)


def _ln_rows(x, dep):
    n = x.shape[-1]
    mu = _after(jnp.sum(x, axis=-1, keepdims=True), dep) * (1.0 / n)
    xc = x - mu
    var = jnp.sum(xc * xc, axis=-1, keepdims=True) * (1.0 / n)
    den = _rb(jnp.sqrt(_rb(_rb(var) + EPS)))
    num = _rb(x - _rb(mu))
    return (num * (1.0 / den)).astype(BF)


def _unpack(z, odd):
    u = pltpu.bitcast(z, U32)
    u = u.reshape(u.shape[0] * u.shape[1], u.shape[2])
    u = (u & jnp.uint32(0xFFFF0000)) if odd else (u << 16)
    return pltpu.bitcast(u, F32).astype(BF)


def _pk(x):
    return pltpu.bitcast(x, U32)


def _up(u):
    return pltpu.bitcast(u, BF)


def _kernel(x_hbm, c_hbm, wq_hbm, wk_hbm, wv_hbm, wo_hbm, wr_hbm, wg_hbm, wu_hbm, wd_hbm,
            out_hbm,
            x_s, c_s, cu_s, zq, zk, zv, wo_s, wg_s, wu_s, wd_s, wr_s,
            xn_s, q_s, k_s, v_s, k0_s, v0_s, w4_s, ctx_s, h_s, hn_s, o_s,
            sem, xsem, csem, wsem, osem):
    S, M = x_s.shape
    H, _, D = ctx_s.shape
    nq = S // TQ
    ne = S // TE
    scale = (D ** -0.5) * math.log2(math.e)
    W = ((wk_hbm, zk), (wv_hbm, zv), (wq_hbm, zq))
    PG = (0, 1, 2, 3, H // 2)

    def w_start(i, g, priority):
        src, z = W[i]
        for r in range(8):
            pltpu.make_async_copy(src.at[:, r, PG[g]:PG[g + 1]], z.at[:, PG[g]:PG[g + 1], 2 * r:2 * r + 2, :],
                                  wsem.at[3 * g + i]).start(priority=priority)

    def w_wait(i, g):
        z = W[i][1].at[:, PG[g]:PG[g + 1]]
        pltpu.make_async_copy(z, z, wsem.at[3 * g + i]).wait()

    def x_copy(i):
        rows = pl.ds(pl.multiple_of(i * TQ, TQ), TQ)
        return pltpu.make_async_copy(x_hbm.at[rows, :], x_s.at[rows, :], xsem.at[i])

    def c_copy(i):
        rows = pl.ds(pl.multiple_of(i * TC, TC), TC)
        return pltpu.make_async_copy(c_hbm.at[rows, :], c_s.at[rows, :], csem.at[i])

    def out_copy(i):
        rows = pl.ds(pl.multiple_of(i * TE, TE), TE)
        return pltpu.make_async_copy(o_s.at[rows, :], out_hbm.at[rows, :], osem.at[i])

    late = [pltpu.make_async_copy(src, dst, sem.at[i]) for i, (src, dst) in enumerate([
        (wo_hbm, wo_s.at[:, 0:M]), (wr_hbm, wr_s), (wg_hbm, wg_s), (wu_hbm, wu_s), (wd_hbm, wd_s.at[:, 0:M])])]

    def for_each(lo, hi, fn):
        def body(i, c):
            fn(i)
            return c
        lax.fori_loop(lo, hi, body, 0)

    w_start(0, 0, 0)
    w_start(1, 0, 0)
    c_copy(0).start()
    for_each(1, S // TC, lambda j: c_copy(j).start(priority=1))
    w_start(2, 0, 1)
    for_each(0, nq, lambda j: x_copy(nq - 1 - j).start(priority=1))

    def kv_piece(wkv, r0):
        rows = slice(r0 // 2, (r0 + TQ) // 2)
        kv = jnp.dot(_up(cu_s[rows, :]), wkv, preferred_element_type=F32)
        k_s[rows, :] = _pk(kv[:, :D].astype(BF))
        v_s[rows, :] = _pk(kv[:, D:].astype(BF))

    def q_piece(wq, r0):
        rows = slice(r0 // 2, (r0 + TQ) // 2)
        q = jnp.dot(_up(xn_s[rows, :]), wq, preferred_element_type=F32)
        q_s[r0:r0 + TQ, :] = (q * scale).astype(BF)

    def ln1(i):
        for j in range(TQ // CN):
            r0 = i * TQ + j * CN
            x = x_s[r0:r0 + CN, :].astype(F32)
            xc = x - jnp.sum(x, axis=-1, keepdims=True) * (1.0 / M)
            var = jnp.sum(xc * xc, axis=-1, keepdims=True) * (1.0 / M)
            xn_s[r0 // 2:(r0 + CN) // 2, :] = _pk((xc * lax.rsqrt(var + EPS)).astype(BF))

    def attention(h, kr, vr, pre, gap, tail, deps):
        HB = TQ // 2
        row = lax.broadcasted_iota(jnp.int32, (HB, HB), 0)
        col = lax.broadcasted_iota(jnp.int32, (HB, HB), 1)
        tri = col <= row
        deps = list(deps)
        for i in range(nq - 1, -1, -1):
            n0 = i * TQ
            n1 = n0 + HB
            n2 = n0 + TQ
            pre(i)
            q = q_s[n0:n2, :]
            s = lax.dot_general(q, _up(kr[:n1 // 2, :]), NT, preferred_element_type=F32)
            s2 = lax.dot_general(q[HB:], _up(kr[n1 // 2:n2 // 2, :]), NT, preferred_element_type=F32)
            gap(i)
            sa = jnp.where(tri, s[:HB, n0:], NEG)
            sa = jnp.concatenate([s[:HB, :n0], sa], axis=1) if i > 0 else sa
            sb = s[HB:]
            s2 = jnp.where(tri, s2, NEG)
            da, db = deps.pop(0)
            ma = _after(jnp.max(sa, axis=1, keepdims=True), da)
            mb = _after(jnp.max(jnp.concatenate([sb, s2], axis=1), axis=1, keepdims=True), db)
            pa = jnp.exp2(sa - ma)
            pb = jnp.exp2(sb - mb)
            p2 = jnp.exp2(s2 - mb)
            la = _recip(jnp.sum(pa, axis=1, keepdims=True))
            lb = _recip(jnp.sum(jnp.concatenate([pb, p2], axis=1), axis=1, keepdims=True))
            deps.append((la, lb))
            p = jnp.concatenate([pa, pb], axis=0).astype(BF)
            o = jnp.dot(p, _up(vr[:n1 // 2, :]), preferred_element_type=F32)
            o2 = jnp.dot(p2.astype(BF), _up(vr[n1 // 2:n2 // 2, :]), preferred_element_type=F32)
            ctx_s[h, n0:n1, :] = (o[:HB] * la).astype(BF)
            ctx_s[h, n1:n2, :] = ((o[HB:] + o2) * lb).astype(BF)
        tail()
        return deps

    nodeps = [(None, None)] * DIST

    def nop(*_):
        return None

    w_wait(0, 0)
    w_wait(1, 0)
    w4_s[...] = _pk(jnp.concatenate([_unpack(z[:, 0], odd) for odd in (0, 1) for z in (zk, zv)], axis=1))

    def kv01(j):
        c = c_s[pl.ds(pl.multiple_of(j * TC, TC), TC), :]
        rows = pl.ds(pl.multiple_of(j * (TC // 2), TC // 2), TC // 2)
        cu_s[rows, :] = _pk(c)
        kv = jnp.dot(c, _up(w4_s[...]), preferred_element_type=F32)
        for n, dst in enumerate((k0_s, v0_s, k_s, v_s)):
            dst[rows, :] = _pk(kv[:, n * D:(n + 1) * D].astype(BF))

    for_each(0, S // TC - 1, lambda j: (c_copy(j).wait(), kv01(j)))
    c_copy(S // TC - 1).wait()
    w_wait(2, 0)
    x_copy(nq - 1).wait()
    ln1(nq - 1)
    kv01(S // TC - 1)
    wq0 = _unpack(zq[:, 0], 0)
    wq1 = _unpack(zq[:, 0], 1)
    q_piece(wq0, (nq - 1) * TQ)
    for_each(nq // 2, nq - 1, lambda j: x_copy(j).wait())

    def pre0(i):
        if i == nq - 1:
            for j in range(3):
                w_start(j, 1, 1)
        if i == nq // 2:
            for j in range(nq // 2):
                x_copy(j).wait()
            for j in range(3):
                w_start(j, 2, 0)
            for j in range(3):
                w_start(j, 3, 1)

    def gap0(i):
        q_piece(wq1, i * TQ)
        if i > 0:
            ln1(i - 1)
            q_piece(wq0, (i - 1) * TQ)

    attention(0, k0_s, v0_s, pre0, gap0, nop, nodeps)

    def head(h, p, odd, deps):
        wq = _unpack(zq[:, p], odd)
        wkv = jnp.concatenate([_unpack(zk[:, p], odd), _unpack(zv[:, p], odd)], axis=1)

        def gap(i):
            if i > 0:
                q_piece(wq, i * TQ)
            if i + 1 < nq:
                kv_piece(wkv, (i + 1) * TQ)

        def tail():
            kv_piece(wkv, 0)
            q_piece(wq, 0)

        return attention(h, k_s, v_s, nop, gap, tail, deps)

    def two_heads(t):
        p = t + 1

        @pl.when(p == PG[3])
        def _():
            for i in range(3):
                w_wait(i, 3)
            for c in late:
                c.start(priority=1)

        head(2 * t + 2, p, 1, head(2 * t + 1, p, 0, nodeps))

    for i in range(3):
        w_wait(i, 1)
        w_wait(i, 2)
    for_each(0, H // 2 - 1, two_heads)

    late[0].wait()
    late[1].wait()
    wr = wr_s[...].astype(F32).reshape(1, M)

    def post(r0, hv, n, deps, top):
        b1, j1, b2, j2 = top
        for j in range(n // CN - 1, -1, -1):
            rows = pl.ds(r0 + j * CN, CN)
            hf = hv[j * CN:(j + 1) * CN, :].astype(F32)
            hn = _ln_rows(hf, deps.pop(0))
            hnf = hn.astype(F32)
            r = _rb(jnp.sum(hnf * wr, axis=-1, keepdims=True))
            hn_s[rows, :] = hn
            o_s[rows, :] = (hf + hnf).astype(BF)
            deps.append(r)
            tok = lax.broadcasted_iota(jnp.int32, (CN, 1), 0) + (r0 + j * CN)
            ge1 = r >= b1
            ge2 = r >= b2
            b2 = jnp.where(ge1, b1, jnp.where(ge2, r, b2))
            j2 = jnp.where(ge1, j1, jnp.where(ge2, tok, j2))
            b1 = jnp.where(ge1, r, b1)
            j1 = jnp.where(ge1, tok, j1)
        return b1, j1, b2, j2

    def o_proj(r0, n, hv, cols=slice(0, M)):
        rows = pl.ds(r0, n)
        ctx = jnp.concatenate([ctx_s[hh, rows, :] for hh in range(H)], axis=1)
        a = jnp.dot(ctx, wo_s[:, cols], preferred_element_type=F32)
        hv[:, cols] = (x_s[rows, cols].astype(F32) + _rb(a)).astype(BF)

    def o_piece(n):
        o_proj(S - TE, TE, h_s.at[S - TE:S, :], slice(n * (M // nq), (n + 1) * (M // nq)))

    attention(H - 1, k_s, v_s, nop, lambda i: o_piece(i + 1) if i + 1 < nq else None, lambda: o_piece(0), nodeps)

    def epi(t, top):
        i = ne - 1 - (t + 1)
        r0 = pl.multiple_of(i * TE, TE)
        hv = h_s.at[pl.ds(r0, 2 * TE), :]
        top = post(r0 + TE, hv.at[TE:2 * TE, :], TE, [None], top)
        o_proj(r0, TE, hv.at[0:TE, :])
        out_copy(i + 1).start()
        return top

    ninf = jnp.full((CN, 1), -jnp.inf, F32)
    none = jnp.full((CN, 1), S, jnp.int32)
    top = lax.fori_loop(0, ne - 2, epi, (ninf, none, ninf, none))
    for c in late[2:]:
        c.wait()
    deps = [None]
    top = post(TE, h_s.at[TE:2 * TE, :], TE, deps, top)
    o_proj(TB, TE - TB, h_s.at[TB:TE, :])
    out_copy(1).start()
    top = post(TB, h_s.at[TB:TE, :], TE - TB, deps, top)
    o_proj(0, TB, h_s.at[0:TB, :])
    top = post(0, h_s.at[0:TB, :], TB, deps * (TB // CN), top)
    out_copy(0).start()

    r = jnp.concatenate([top[0], top[2]], axis=0)
    idx = jnp.concatenate([top[1], top[3]], axis=0)
    m1 = jnp.max(r, axis=0, keepdims=True)
    i1v = jnp.min(jnp.where(r == m1, idx, S), axis=0, keepdims=True)
    r2 = jnp.where(idx == i1v, -jnp.inf, r)
    m2 = jnp.max(r2, axis=0, keepdims=True)
    i2v = jnp.min(jnp.where((r2 == m2) & (idx != i1v), idx, S), axis=0, keepdims=True)
    i1 = jnp.minimum(jnp.min(i1v), S - 1)
    i2 = jnp.minimum(jnp.min(i2v), S - 1)
    b1 = pl.multiple_of(i1 & (-16), 16)
    b2 = pl.multiple_of(i2 & (-16), 16)
    rows16 = lax.broadcasted_iota(jnp.int32, (16, M), 0)
    hn1 = hn_s[pl.ds(b1, 16), :].astype(F32)
    hn2 = hn_s[pl.ds(b2, 16), :].astype(F32)
    x1 = jnp.sum(jnp.where(rows16 == i1 - b1, hn1, 0.0), axis=0, keepdims=True)
    x2 = jnp.sum(jnp.where(rows16 == i2 - b2, hn2, 0.0), axis=0, keepdims=True)
    xs = jnp.where(rows16 == 0, x1, jnp.where(rows16 == 1, x2, 0.0)).astype(BF)

    g = _rb(jnp.dot(xs, wg_s[...], preferred_element_type=F32)[:8])
    u = _rb(jnp.dot(xs, wu_s[...], preferred_element_type=F32)[:8])
    g = _rb(g * jax.nn.sigmoid(g))
    gu = jnp.concatenate([g * u, jnp.zeros_like(g)], axis=0).astype(BF)
    y = _rb(jnp.dot(gu, wd_s[:, 0:M], preferred_element_type=F32)[:8])
    y1 = _rb(y[0:1, :] * _rb(jax.nn.sigmoid(m1)))
    y2 = _rb(y[1:2, :] * _rb(jax.nn.sigmoid(m2)))

    for i in range(ne):
        out_copy(i).wait()
    patch = []
    for n, (b, hnb) in enumerate(((b1, hn1), (b2, hn2))):
        rows = rows16 + b
        upd = jnp.where(rows == i1, y1, jnp.where(rows == i2, y2, 0.0))
        o_s[pl.ds(b, 16), :] = (h_s[pl.ds(b, 16), :].astype(F32) + _rb(hnb + upd)).astype(BF)
        patch.append(pltpu.make_async_copy(o_s.at[pl.ds(b, 16), :], out_hbm.at[pl.ds(b, 16), :], osem.at[n]))
    patch[0].start()

    @pl.when(b1 != b2)
    def _():
        patch[1].start()
        patch[1].wait()
    patch[0].wait()


@jax.jit
def pallas_sequential_preLN__compressed_kv_cla__moe_arch_mod__prompt_kernel(
        A_x, A_c_kv, A_w_q, A_w_uk, A_w_uv, A_w_o, B_x, B_w_r, B_w_gate, B_w_up, B_w_down):
    del B_x
    B, S, M = A_x.shape
    C = A_c_kv.shape[2]
    _, H, D = A_w_q.shape
    Fd = B_w_gate.shape[1]
    assert B == 1 and A_c_kv.shape[1] == S
    vmem = pltpu.VMEM
    dma = pltpu.SemaphoreType.DMA
    anyspec = pl.BlockSpec(memory_space=pl.ANY)
    out = pl.pallas_call(
        _kernel,
        in_specs=[anyspec] * 10,
        out_specs=anyspec,
        out_shape=jax.ShapeDtypeStruct((S, M), BF),
        scratch_shapes=[
            vmem((S, M), BF), vmem((S, C), BF), vmem((S // 2, C), U32),
            vmem((M // 8, H // 2, 16, D), BF), vmem((C // 8, H // 2, 16, D), BF),
            vmem((C // 8, H // 2, 16, D), BF),
            vmem((H * D, M + 128), BF),
            vmem((M, Fd), BF), vmem((M, Fd), BF), vmem((Fd, M + 128), BF), vmem((M,), BF),
            vmem((S // 2, M), U32),
            vmem((S, D), BF), vmem((S // 2, D), U32), vmem((S // 2, D), U32),
            vmem((S // 2, D), U32), vmem((S // 2, D), U32), vmem((C // 2, 4 * D), U32),
            vmem((H, S, D), BF),
            vmem((S, M), BF), vmem((S, M), BF), vmem((S, M), BF),
            dma((5,)), dma((S // TQ,)), dma((S // TC,)), dma((12,)), dma((S // TE,)),
        ],
        compiler_params=pltpu.CompilerParams(vmem_limit_bytes=120 * 1024 * 1024),
    )(A_x.reshape(S, M), A_c_kv.reshape(S, C),
      A_w_q.reshape(M // 8, 8, H // 2, 2, D), A_w_uk.reshape(C // 8, 8, H // 2, 2, D),
      A_w_uv.reshape(C // 8, 8, H // 2, 2, D), A_w_o.reshape(H * D, M),
      B_w_r, B_w_gate, B_w_up, B_w_down)
    return out.reshape(B, S, M)
```

```python
import math

import jax
import jax.numpy as jnp
from jax import lax
from jax.experimental import pallas as pl
from jax.experimental.pallas import tpu as pltpu

BF = jnp.bfloat16
F32 = jnp.float32
U32 = jnp.uint32
NT = (((1,), (1,)), ((), ()))
NEG = -1e30
EPS = 1e-5
BIG = 3e38

TQ = 256
TC = 512
TE = 256
TB = 64
CN = 16
XW = 5
DIST = 2


def _rb(x):
    return x.astype(BF).astype(F32)


def _after(x, dep):
    return x if dep is None else jnp.maximum(x, dep - BIG)


def _recip(l):
    r = pl.reciprocal(l, approx=True)
    return r * (2.0 - l * r)


def _ln_rows(x, dep):
    n = x.shape[-1]
    mu = _after(jnp.sum(x, axis=-1, keepdims=True), dep) * (1.0 / n)
    xc = x - mu
    var = jnp.sum(xc * xc, axis=-1, keepdims=True) * (1.0 / n)
    den = _rb(jnp.sqrt(_rb(_rb(var) + EPS)))
    num = _rb(x - _rb(mu))
    return (num * (1.0 / den)).astype(BF)


def _unpack(z, odd):
    u = pltpu.bitcast(z, U32)
    u = u.reshape(u.shape[0] * u.shape[1], u.shape[2])
    u = (u & jnp.uint32(0xFFFF0000)) if odd else (u << 16)
    return pltpu.bitcast(u, F32).astype(BF)


def _pk(x):
    return pltpu.bitcast(x, U32)


def _up(u):
    return pltpu.bitcast(u, BF)


def _kernel(x_hbm, c_hbm, wq_hbm, wk_hbm, wv_hbm, wo_hbm, wr_hbm, wg_hbm, wu_hbm, wd_hbm,
            out_hbm,
            x_s, c_s, cu_s, zq, zk, zv, wo_s, wg_s, wu_s, wd_s, wr_s,
            xn_s, q_s, k_s, v_s, k0_s, v0_s, w4_s, ctx_s, h_s, hn_s, o_s,
            sem, xsem, csem, wsem, osem):
    S, M = x_s.shape
    H, _, D = ctx_s.shape
    nq = S // TQ
    ne = S // TE
    scale = (D ** -0.5) * math.log2(math.e)
    W = ((wk_hbm, zk), (wv_hbm, zv), (wq_hbm, zq))
    PG = (0, 1, 3, H // 2)

    def w_start(i, g, priority):
        src, z = W[i]
        for r in range(8):
            pltpu.make_async_copy(src.at[:, r, PG[g]:PG[g + 1]], z.at[:, PG[g]:PG[g + 1], 2 * r:2 * r + 2, :],
                                  wsem.at[3 * g + i]).start(priority=priority)

    def w_wait(i, g):
        z = W[i][1].at[:, PG[g]:PG[g + 1]]
        pltpu.make_async_copy(z, z, wsem.at[3 * g + i]).wait()

    def x_copy(i):
        rows = pl.ds(pl.multiple_of(i * TQ, TQ), TQ)
        return pltpu.make_async_copy(x_hbm.at[rows, :], x_s.at[rows, :], xsem.at[i])

    def c_copy(i):
        rows = pl.ds(pl.multiple_of(i * TC, TC), TC)
        return pltpu.make_async_copy(c_hbm.at[rows, :], c_s.at[rows, :], csem.at[i])

    def out_copy(i):
        rows = pl.ds(pl.multiple_of(i * TE, TE), TE)
        return pltpu.make_async_copy(o_s.at[rows, :], out_hbm.at[rows, :], osem.at[i])

    late = [pltpu.make_async_copy(src, dst, sem.at[i]) for i, (src, dst) in enumerate([
        (wo_hbm, wo_s.at[:, 0:M]), (wr_hbm, wr_s), (wg_hbm, wg_s), (wu_hbm, wu_s), (wd_hbm, wd_s.at[:, 0:M])])]

    def for_each(lo, hi, fn):
        def body(i, c):
            fn(i)
            return c
        lax.fori_loop(lo, hi, body, 0)

    w_start(0, 0, 0)
    w_start(1, 0, 0)
    c_copy(0).start()
    for_each(1, S // TC, lambda j: c_copy(j).start())
    w_start(2, 0, 0)
    for_each(0, nq, lambda j: x_copy(nq - 1 - j).start())
    for j in range(3):
        w_start(j, 1, 0)
    for j in range(3):
        w_start(j, 2, 1)

    def kv_piece(wkv, r0):
        rows = slice(r0 // 2, (r0 + TQ) // 2)
        kv = jnp.dot(_up(cu_s[rows, :]), wkv, preferred_element_type=F32)
        k_s[rows, :] = _pk(kv[:, :D].astype(BF))
        v_s[rows, :] = _pk(kv[:, D:].astype(BF))

    def q_piece(wq, r0):
        rows = slice(r0 // 2, (r0 + TQ) // 2)
        q = jnp.dot(_up(xn_s[rows, :]), wq, preferred_element_type=F32)
        q_s[r0:r0 + TQ, :] = (q * scale).astype(BF)

    def ln1(i):
        for j in range(TQ // CN):
            r0 = i * TQ + j * CN
            x = x_s[r0:r0 + CN, :].astype(F32)
            xc = x - jnp.sum(x, axis=-1, keepdims=True) * (1.0 / M)
            var = jnp.sum(xc * xc, axis=-1, keepdims=True) * (1.0 / M)
            xn_s[r0 // 2:(r0 + CN) // 2, :] = _pk((xc * lax.rsqrt(var + EPS)).astype(BF))

    def attention(h, kr, vr, pre, gap, tail, deps):
        HB = TQ // 2
        row = lax.broadcasted_iota(jnp.int32, (HB, HB), 0)
        col = lax.broadcasted_iota(jnp.int32, (HB, HB), 1)
        tri = col <= row
        deps = list(deps)
        for i in range(nq - 1, -1, -1):
            n0 = i * TQ
            n1 = n0 + HB
            n2 = n0 + TQ
            pre(i)
            q = q_s[n0:n2, :]
            s = lax.dot_general(q, _up(kr[:n1 // 2, :]), NT, preferred_element_type=F32)
            s2 = lax.dot_general(q[HB:], _up(kr[n1 // 2:n2 // 2, :]), NT, preferred_element_type=F32)
            gap(i)
            sa = jnp.where(tri, s[:HB, n0:], NEG)
            sa = jnp.concatenate([s[:HB, :n0], sa], axis=1) if i > 0 else sa
            sb = s[HB:]
            s2 = jnp.where(tri, s2, NEG)
            da, db = deps.pop(0)
            ma = _after(jnp.max(sa, axis=1, keepdims=True), da)
            mb = _after(jnp.max(jnp.concatenate([sb, s2], axis=1), axis=1, keepdims=True), db)
            pa = jnp.exp2(sa - ma)
            pb = jnp.exp2(sb - mb)
            p2 = jnp.exp2(s2 - mb)
            la = _recip(jnp.sum(pa, axis=1, keepdims=True))
            lb = _recip(jnp.sum(jnp.concatenate([pb, p2], axis=1), axis=1, keepdims=True))
            deps.append((la, lb))
            p = jnp.concatenate([pa, pb], axis=0).astype(BF)
            o = jnp.dot(p, _up(vr[:n1 // 2, :]), preferred_element_type=F32)
            o2 = jnp.dot(p2.astype(BF), _up(vr[n1 // 2:n2 // 2, :]), preferred_element_type=F32)
            ctx_s[h, n0:n1, :] = (o[:HB] * la).astype(BF)
            ctx_s[h, n1:n2, :] = ((o[HB:] + o2) * lb).astype(BF)
        tail()
        return deps

    nodeps = [(None, None)] * DIST

    def nop(*_):
        return None

    w_wait(0, 0)
    w_wait(1, 0)
    w4_s[...] = _pk(jnp.concatenate([_unpack(z[:, 0], odd) for odd in (0, 1) for z in (zk, zv)], axis=1))

    def kv01(j):
        c = c_s[pl.ds(pl.multiple_of(j * TC, TC), TC), :]
        rows = pl.ds(pl.multiple_of(j * (TC // 2), TC // 2), TC // 2)
        cu_s[rows, :] = _pk(c)
        kv = jnp.dot(c, _up(w4_s[...]), preferred_element_type=F32)
        for n, dst in enumerate((k0_s, v0_s, k_s, v_s)):
            dst[rows, :] = _pk(kv[:, n * D:(n + 1) * D].astype(BF))

    for_each(0, S // TC - 1, lambda j: (c_copy(j).wait(), kv01(j)))
    c_copy(S // TC - 1).wait()
    w_wait(2, 0)
    x_copy(nq - 1).wait()
    ln1(nq - 1)
    kv01(S // TC - 1)
    wq0 = _unpack(zq[:, 0], 0)
    wq1 = _unpack(zq[:, 0], 1)
    q_piece(wq0, (nq - 1) * TQ)
    for j in range(XW, nq - 1):
        x_copy(j).wait()

    def pre0(i):
        if i == XW:
            for j in range(XW):
                x_copy(j).wait()

    def gap0(i):
        q_piece(wq1, i * TQ)
        if i > 0:
            ln1(i - 1)
            q_piece(wq0, (i - 1) * TQ)

    attention(0, k0_s, v0_s, pre0, gap0, nop, nodeps)

    def head(h, p, odd, deps):
        wq = _unpack(zq[:, p], odd)
        wkv = jnp.concatenate([_unpack(zk[:, p], odd), _unpack(zv[:, p], odd)], axis=1)

        def gap(i):
            if i > 0:
                q_piece(wq, i * TQ)
            if i + 1 < nq:
                kv_piece(wkv, (i + 1) * TQ)

        def tail():
            kv_piece(wkv, 0)
            q_piece(wq, 0)

        return attention(h, k_s, v_s, nop, gap, tail, deps)

    def two_heads(t):
        p = t + 1

        @pl.when(p == PG[2])
        def _():
            for i in range(3):
                w_wait(i, 2)
            for c in late:
                c.start(priority=1)

        head(2 * t + 2, p, 1, head(2 * t + 1, p, 0, nodeps))

    for i in range(3):
        w_wait(i, 1)
    for_each(0, H // 2 - 1, two_heads)

    late[0].wait()
    late[1].wait()
    wr = wr_s[...].astype(F32).reshape(1, M)

    def post(r0, hv, n, deps, top):
        b1, j1, b2, j2 = top
        for j in range(n // CN - 1, -1, -1):
            rows = pl.ds(r0 + j * CN, CN)
            hf = hv[j * CN:(j + 1) * CN, :].astype(F32)
            hn = _ln_rows(hf, deps.pop(0))
            hnf = hn.astype(F32)
            r = _rb(jnp.sum(hnf * wr, axis=-1, keepdims=True))
            hn_s[rows, :] = hn
            o_s[rows, :] = (hf + hnf).astype(BF)
            deps.append(r)
            tok = lax.broadcasted_iota(jnp.int32, (CN, 1), 0) + (r0 + j * CN)
            ge1 = r >= b1
            ge2 = r >= b2
            b2 = jnp.where(ge1, b1, jnp.where(ge2, r, b2))
            j2 = jnp.where(ge1, j1, jnp.where(ge2, tok, j2))
            b1 = jnp.where(ge1, r, b1)
            j1 = jnp.where(ge1, tok, j1)
        return b1, j1, b2, j2

    def o_proj(r0, n, hv, cols=slice(0, M)):
        rows = pl.ds(r0, n)
        ctx = jnp.concatenate([ctx_s[hh, rows, :] for hh in range(H)], axis=1)
        a = jnp.dot(ctx, wo_s[:, cols], preferred_element_type=F32)
        hv[:, cols] = (x_s[rows, cols].astype(F32) + _rb(a)).astype(BF)

    def o_piece(n):
        o_proj(S - TE, TE, h_s.at[S - TE:S, :], slice(n * (M // nq), (n + 1) * (M // nq)))

    attention(H - 1, k_s, v_s, nop, lambda i: o_piece(i + 1) if i + 1 < nq else None, lambda: o_piece(0), nodeps)

    def epi(t, top):
        i = ne - 1 - (t + 1)
        r0 = pl.multiple_of(i * TE, TE)
        hv = h_s.at[pl.ds(r0, 2 * TE), :]
        top = post(r0 + TE, hv.at[TE:2 * TE, :], TE, [None], top)
        o_proj(r0, TE, hv.at[0:TE, :])
        out_copy(i + 1).start()
        return top

    ninf = jnp.full((CN, 1), -jnp.inf, F32)
    none = jnp.full((CN, 1), S, jnp.int32)
    top = lax.fori_loop(0, ne - 2, epi, (ninf, none, ninf, none))
    for c in late[2:]:
        c.wait()
    deps = [None]
    top = post(TE, h_s.at[TE:2 * TE, :], TE, deps, top)
    o_proj(TB, TE - TB, h_s.at[TB:TE, :])
    out_copy(1).start()
    top = post(TB, h_s.at[TB:TE, :], TE - TB, deps, top)
    o_proj(0, TB, h_s.at[0:TB, :])
    top = post(0, h_s.at[0:TB, :], TB, deps * (TB // CN), top)
    out_copy(0).start()

    r = jnp.concatenate([top[0], top[2]], axis=0)
    idx = jnp.concatenate([top[1], top[3]], axis=0)
    m1 = jnp.max(r, axis=0, keepdims=True)
    i1v = jnp.min(jnp.where(r == m1, idx, S), axis=0, keepdims=True)
    r2 = jnp.where(idx == i1v, -jnp.inf, r)
    m2 = jnp.max(r2, axis=0, keepdims=True)
    i2v = jnp.min(jnp.where((r2 == m2) & (idx != i1v), idx, S), axis=0, keepdims=True)
    i1 = jnp.minimum(jnp.min(i1v), S - 1)
    i2 = jnp.minimum(jnp.min(i2v), S - 1)
    b1 = pl.multiple_of(i1 & (-16), 16)
    b2 = pl.multiple_of(i2 & (-16), 16)
    rows16 = lax.broadcasted_iota(jnp.int32, (16, M), 0)
    hn1 = hn_s[pl.ds(b1, 16), :].astype(F32)
    hn2 = hn_s[pl.ds(b2, 16), :].astype(F32)
    x1 = jnp.sum(jnp.where(rows16 == i1 - b1, hn1, 0.0), axis=0, keepdims=True)
    x2 = jnp.sum(jnp.where(rows16 == i2 - b2, hn2, 0.0), axis=0, keepdims=True)
    xs = jnp.where(rows16 == 0, x1, jnp.where(rows16 == 1, x2, 0.0)).astype(BF)

    g = _rb(jnp.dot(xs, wg_s[...], preferred_element_type=F32)[:8])
    u = _rb(jnp.dot(xs, wu_s[...], preferred_element_type=F32)[:8])
    g = _rb(g * jax.nn.sigmoid(g))
    gu = jnp.concatenate([g * u, jnp.zeros_like(g)], axis=0).astype(BF)
    y = _rb(jnp.dot(gu, wd_s[:, 0:M], preferred_element_type=F32)[:8])
    y1 = _rb(y[0:1, :] * _rb(jax.nn.sigmoid(m1)))
    y2 = _rb(y[1:2, :] * _rb(jax.nn.sigmoid(m2)))

    for i in range(ne):
        out_copy(i).wait()
    patch = []
    for n, (b, hnb) in enumerate(((b1, hn1), (b2, hn2))):
        rows = rows16 + b
        upd = jnp.where(rows == i1, y1, jnp.where(rows == i2, y2, 0.0))
        o_s[pl.ds(b, 16), :] = (h_s[pl.ds(b, 16), :].astype(F32) + _rb(hnb + upd)).astype(BF)
        patch.append(pltpu.make_async_copy(o_s.at[pl.ds(b, 16), :], out_hbm.at[pl.ds(b, 16), :], osem.at[n]))
    patch[0].start()

    @pl.when(b1 != b2)
    def _():
        patch[1].start()
        patch[1].wait()
    patch[0].wait()


@jax.jit
def pallas_sequential_preLN__compressed_kv_cla__moe_arch_mod__prompt_kernel(
        A_x, A_c_kv, A_w_q, A_w_uk, A_w_uv, A_w_o, B_x, B_w_r, B_w_gate, B_w_up, B_w_down):
    del B_x
    B, S, M = A_x.shape
    C = A_c_kv.shape[2]
    _, H, D = A_w_q.shape
    Fd = B_w_gate.shape[1]
    assert B == 1 and A_c_kv.shape[1] == S
    vmem = pltpu.VMEM
    dma = pltpu.SemaphoreType.DMA
    anyspec = pl.BlockSpec(memory_space=pl.ANY)
    out = pl.pallas_call(
        _kernel,
        in_specs=[anyspec] * 10,
        out_specs=anyspec,
        out_shape=jax.ShapeDtypeStruct((S, M), BF),
        scratch_shapes=[
            vmem((S, M), BF), vmem((S, C), BF), vmem((S // 2, C), U32),
            vmem((M // 8, H // 2, 16, D), BF), vmem((C // 8, H // 2, 16, D), BF),
            vmem((C // 8, H // 2, 16, D), BF),
            vmem((H * D, M + 128), BF),
            vmem((M, Fd), BF), vmem((M, Fd), BF), vmem((Fd, M + 128), BF), vmem((M,), BF),
            vmem((S // 2, M), U32),
            vmem((S, D), BF), vmem((S // 2, D), U32), vmem((S // 2, D), U32),
            vmem((S // 2, D), U32), vmem((S // 2, D), U32), vmem((C // 2, 4 * D), U32),
            vmem((H, S, D), BF),
            vmem((S, M), BF), vmem((S, M), BF), vmem((S, M), BF),
            dma((5,)), dma((S // TQ,)), dma((S // TC,)), dma((9,)), dma((S // TE,)),
        ],
        compiler_params=pltpu.CompilerParams(vmem_limit_bytes=120 * 1024 * 1024),
    )(A_x.reshape(S, M), A_c_kv.reshape(S, C),
      A_w_q.reshape(M // 8, 8, H // 2, 2, D), A_w_uk.reshape(C // 8, 8, H // 2, 2, D),
      A_w_uv.reshape(C // 8, 8, H // 2, 2, D), A_w_o.reshape(H * D, M),
      B_w_r, B_w_gate, B_w_up, B_w_down)
    return out.reshape(B, S, M)
```

```python
import math

import jax
import jax.numpy as jnp
from jax import lax
from jax.experimental import pallas as pl
from jax.experimental.pallas import tpu as pltpu

BF = jnp.bfloat16
F32 = jnp.float32
U32 = jnp.uint32
NT = (((1,), (1,)), ((), ()))
NEG = -1e30
EPS = 1e-5
BIG = 3e38

TQ = 256
TC = 512
TE = 256
TB = 64
CN = 16
XW = 5
DIST = 2


def _rb(x):
    return x.astype(BF).astype(F32)


def _after(x, dep):
    return x if dep is None else jnp.maximum(x, dep - BIG)


def _recip(l):
    r = pl.reciprocal(l, approx=True)
    return r * (2.0 - l * r)


def _ln_rows(x, dep):
    n = x.shape[-1]
    mu = _after(jnp.sum(x, axis=-1, keepdims=True), dep) * (1.0 / n)
    xc = x - mu
    var = jnp.sum(xc * xc, axis=-1, keepdims=True) * (1.0 / n)
    den = _rb(jnp.sqrt(_rb(_rb(var) + EPS)))
    num = _rb(x - _rb(mu))
    return (num * (1.0 / den)).astype(BF)


def _unpack(z, odd):
    u = pltpu.bitcast(z, U32)
    u = u.reshape(u.shape[0] * u.shape[1], u.shape[2])
    u = (u & jnp.uint32(0xFFFF0000)) if odd else (u << 16)
    return pltpu.bitcast(u, F32).astype(BF)


def _pk(x):
    return pltpu.bitcast(x, U32)


def _up(u):
    return pltpu.bitcast(u, BF)


def _kernel(x_hbm, c_hbm, wq_hbm, wk_hbm, wv_hbm, wo_hbm, wr_hbm, wg_hbm, wu_hbm, wd_hbm,
            out_hbm,
            x_s, c_s, cu_s, z_s, wo_s, wg_s, wu_s, wd_s, wr_s,
            xn_s, q_s, k_s, v_s, k0_s, v0_s, w4_s, ctx_s, h_s, hn_s, o_s,
            sem, xsem, csem, wsem, osem):
    S, M = x_s.shape
    H, _, D = ctx_s.shape
    nq = S // TQ
    ne = S // TE
    scale = (D ** -0.5) * math.log2(math.e)
    PG = (0, 1, 2, H // 2)

    def w_start(i, g, priority):
        lo, hi = PG[g], PG[g + 1]
        for r in range(8):
            two = slice(2 * r, 2 * r + 2)
            if i < 2:
                cps = [((wk_hbm, wv_hbm)[i].at[:, r, lo:hi], z_s.at[:, lo:hi, i, two, :])]
            elif hi - lo == 1:
                cps = [(wq_hbm.at[:, :, r, lo], z_s.at[:, lo, 2:4, two, :])]
            else:
                cps = [(wq_hbm.at[:, b, r, lo:hi], z_s.at[:, lo:hi, 2 + b, two, :]) for b in range(2)]
            for src, dst in cps:
                pltpu.make_async_copy(src, dst, wsem.at[3 * g + i]).start(priority=priority)

    def w_wait(i, g):
        z = z_s.at[:, PG[g]:PG[g + 1], i:(i + 1 if i < 2 else 4)]
        pltpu.make_async_copy(z, z, wsem.at[3 * g + i]).wait()

    def x_copy(i):
        rows = pl.ds(pl.multiple_of(i * TQ, TQ), TQ)
        return pltpu.make_async_copy(x_hbm.at[rows, :], x_s.at[rows, :], xsem.at[i])

    def c_copy(i):
        rows = pl.ds(pl.multiple_of(i * TC, TC), TC)
        return pltpu.make_async_copy(c_hbm.at[rows, :], c_s.at[rows, :], csem.at[i])

    def out_copy(i):
        rows = pl.ds(pl.multiple_of(i * TE, TE), TE)
        return pltpu.make_async_copy(o_s.at[rows, :], out_hbm.at[rows, :], osem.at[i])

    late = [pltpu.make_async_copy(src, dst, sem.at[i]) for i, (src, dst) in enumerate([
        (wo_hbm, wo_s.at[:, 0:M]), (wr_hbm, wr_s), (wg_hbm, wg_s), (wu_hbm, wu_s), (wd_hbm, wd_s.at[:, 0:M])])]

    def for_each(lo, hi, fn):
        def body(i, c):
            fn(i)
            return c
        lax.fori_loop(lo, hi, body, 0)

    w_start(0, 0, 0)
    w_start(1, 0, 0)
    c_copy(0).start()
    for_each(1, S // TC, lambda j: c_copy(j).start())
    w_start(2, 0, 0)
    for_each(0, nq, lambda j: x_copy(nq - 1 - j).start())
    for j in range(3):
        w_start(j, 1, 0)

    def get_wq(p, odd):
        z = z_s[:, p, 2:4]
        return _unpack(z.reshape(2 * z.shape[0], 16, D), odd)

    def kv_piece(wkv, r0):
        rows = slice(r0 // 2, (r0 + TQ) // 2)
        kv = jnp.dot(_up(cu_s[rows, :]), wkv, preferred_element_type=F32)
        k_s[rows, :] = _pk(kv[:, :D].astype(BF))
        v_s[rows, :] = _pk(kv[:, D:].astype(BF))

    def q_piece(wq, r0):
        rows = slice(r0 // 2, (r0 + TQ) // 2)
        q = jnp.dot(_up(xn_s[rows, :]), wq, preferred_element_type=F32)
        q_s[r0:r0 + TQ, :] = (q * scale).astype(BF)

    def ln1(i):
        for j in range(TQ // CN):
            r0 = i * TQ + j * CN
            x = x_s[r0:r0 + CN, :].astype(F32)
            xc = x - jnp.sum(x, axis=-1, keepdims=True) * (1.0 / M)
            var = jnp.sum(xc * xc, axis=-1, keepdims=True) * (1.0 / M)
            xn_s[r0 // 2:(r0 + CN) // 2, :] = _pk((xc * lax.rsqrt(var + EPS)).astype(BF))

    def attention(h, kr, vr, pre, gap, tail, deps):
        HB = TQ // 2
        row = lax.broadcasted_iota(jnp.int32, (HB, HB), 0)
        col = lax.broadcasted_iota(jnp.int32, (HB, HB), 1)
        tri = col <= row
        deps = list(deps)
        for i in range(nq - 1, -1, -1):
            n0 = i * TQ
            n1 = n0 + HB
            n2 = n0 + TQ
            pre(i)
            q = q_s[n0:n2, :]
            s = lax.dot_general(q, _up(kr[:n1 // 2, :]), NT, preferred_element_type=F32)
            s2 = lax.dot_general(q[HB:], _up(kr[n1 // 2:n2 // 2, :]), NT, preferred_element_type=F32)
            gap(i)
            sa = jnp.where(tri, s[:HB, n0:], NEG)
            sa = jnp.concatenate([s[:HB, :n0], sa], axis=1) if i > 0 else sa
            sb = s[HB:]
            s2 = jnp.where(tri, s2, NEG)
            da, db = deps.pop(0)
            ma = _after(jnp.max(sa, axis=1, keepdims=True), da)
            mb = _after(jnp.max(jnp.concatenate([sb, s2], axis=1), axis=1, keepdims=True), db)
            pa = jnp.exp2(sa - ma)
            pb = jnp.exp2(sb - mb)
            p2 = jnp.exp2(s2 - mb)
            la = _recip(jnp.sum(pa, axis=1, keepdims=True))
            lb = _recip(jnp.sum(jnp.concatenate([pb, p2], axis=1), axis=1, keepdims=True))
            deps.append((la, lb))
            p = jnp.concatenate([pa, pb], axis=0).astype(BF)
            o = jnp.dot(p, _up(vr[:n1 // 2, :]), preferred_element_type=F32)
            o2 = jnp.dot(p2.astype(BF), _up(vr[n1 // 2:n2 // 2, :]), preferred_element_type=F32)
            ctx_s[h, n0:n1, :] = (o[:HB] * la).astype(BF)
            ctx_s[h, n1:n2, :] = ((o[HB:] + o2) * lb).astype(BF)
        tail()
        return deps

    nodeps = [(None, None)] * DIST

    def nop(*_):
        return None

    w_wait(0, 0)
    w_wait(1, 0)
    for j in range(3):
        w_start(j, 2, 1)
    w4_s[...] = _pk(jnp.concatenate([_unpack(z_s[:, 0, i], odd) for odd in (0, 1) for i in (0, 1)], axis=1))

    def kv01(j):
        c = c_s[pl.ds(pl.multiple_of(j * TC, TC), TC), :]
        rows = pl.ds(pl.multiple_of(j * (TC // 2), TC // 2), TC // 2)
        cu_s[rows, :] = _pk(c)
        kv = jnp.dot(c, _up(w4_s[...]), preferred_element_type=F32)
        for n, dst in enumerate((k0_s, v0_s, k_s, v_s)):
            dst[rows, :] = _pk(kv[:, n * D:(n + 1) * D].astype(BF))

    for_each(0, S // TC - 1, lambda j: (c_copy(j).wait(), kv01(j)))
    c_copy(S // TC - 1).wait()
    w_wait(2, 0)
    x_copy(nq - 1).wait()
    ln1(nq - 1)
    kv01(S // TC - 1)
    wq0 = get_wq(0, 0)
    wq1 = get_wq(0, 1)
    q_piece(wq0, (nq - 1) * TQ)
    for j in range(XW, nq - 1):
        x_copy(j).wait()

    def pre0(i):
        if i == XW:
            for j in range(XW):
                x_copy(j).wait()

    def gap0(i):
        q_piece(wq1, i * TQ)
        if i > 0:
            ln1(i - 1)
            q_piece(wq0, (i - 1) * TQ)

    attention(0, k0_s, v0_s, pre0, gap0, nop, nodeps)

    def head(h, p, odd, deps):
        wq = get_wq(p, odd)
        wkv = jnp.concatenate([_unpack(z_s[:, p, 0], odd), _unpack(z_s[:, p, 1], odd)], axis=1)

        def gap(i):
            if i > 0:
                q_piece(wq, i * TQ)
            if i + 1 < nq:
                kv_piece(wkv, (i + 1) * TQ)

        def tail():
            kv_piece(wkv, 0)
            q_piece(wq, 0)

        return attention(h, k_s, v_s, nop, gap, tail, deps)

    def two_heads(t):
        p = t + 1

        @pl.when(p == PG[2])
        def _():
            for i in range(3):
                w_wait(i, 2)
            for c in late:
                c.start(priority=1)

        head(2 * t + 2, p, 1, head(2 * t + 1, p, 0, nodeps))

    for i in range(3):
        w_wait(i, 1)
    for_each(0, H // 2 - 1, two_heads)

    late[0].wait()
    late[1].wait()
    wr = wr_s[...].astype(F32).reshape(1, M)

    def post(r0, hv, n, deps, top):
        b1, j1, b2, j2 = top
        for j in range(n // CN - 1, -1, -1):
            rows = pl.ds(r0 + j * CN, CN)
            hf = hv[j * CN:(j + 1) * CN, :].astype(F32)
            hn = _ln_rows(hf, deps.pop(0))
            hnf = hn.astype(F32)
            r = _rb(jnp.sum(hnf * wr, axis=-1, keepdims=True))
            hn_s[rows, :] = hn
            o_s[rows, :] = (hf + hnf).astype(BF)
            deps.append(r)
            tok = lax.broadcasted_iota(jnp.int32, (CN, 1), 0) + (r0 + j * CN)
            ge1 = r >= b1
            ge2 = r >= b2
            b2 = jnp.where(ge1, b1, jnp.where(ge2, r, b2))
            j2 = jnp.where(ge1, j1, jnp.where(ge2, tok, j2))
            b1 = jnp.where(ge1, r, b1)
            j1 = jnp.where(ge1, tok, j1)
        return b1, j1, b2, j2

    def o_proj(r0, n, hv, cols=slice(0, M)):
        rows = pl.ds(r0, n)
        ctx = jnp.concatenate([ctx_s[hh, rows, :] for hh in range(H)], axis=1)
        a = jnp.dot(ctx, wo_s[:, cols], preferred_element_type=F32)
        hv[:, cols] = (x_s[rows, cols].astype(F32) + _rb(a)).astype(BF)

    def o_piece(n):
        o_proj(S - TE, TE, h_s.at[S - TE:S, :], slice(n * (M // nq), (n + 1) * (M // nq)))

    attention(H - 1, k_s, v_s, nop, lambda i: o_piece(i + 1) if i + 1 < nq else None, lambda: o_piece(0), nodeps)

    def epi(t, top):
        i = ne - 1 - (t + 1)
        r0 = pl.multiple_of(i * TE, TE)
        hv = h_s.at[pl.ds(r0, 2 * TE), :]
        top = post(r0 + TE, hv.at[TE:2 * TE, :], TE, [None], top)
        o_proj(r0, TE, hv.at[0:TE, :])
        out_copy(i + 1).start()
        return top

    ninf = jnp.full((CN, 1), -jnp.inf, F32)
    none = jnp.full((CN, 1), S, jnp.int32)
    top = lax.fori_loop(0, ne - 2, epi, (ninf, none, ninf, none))
    for c in late[2:]:
        c.wait()
    deps = [None]
    top = post(TE, h_s.at[TE:2 * TE, :], TE, deps, top)
    o_proj(TB, TE - TB, h_s.at[TB:TE, :])
    out_copy(1).start()
    top = post(TB, h_s.at[TB:TE, :], TE - TB, deps, top)
    o_proj(0, TB, h_s.at[0:TB, :])
    top = post(0, h_s.at[0:TB, :], TB, deps * (TB // CN), top)
    out_copy(0).start()

    r = jnp.concatenate([top[0], top[2]], axis=0)
    idx = jnp.concatenate([top[1], top[3]], axis=0)
    m1 = jnp.max(r, axis=0, keepdims=True)
    i1v = jnp.min(jnp.where(r == m1, idx, S), axis=0, keepdims=True)
    r2 = jnp.where(idx == i1v, -jnp.inf, r)
    m2 = jnp.max(r2, axis=0, keepdims=True)
    i2v = jnp.min(jnp.where((r2 == m2) & (idx != i1v), idx, S), axis=0, keepdims=True)
    i1 = jnp.minimum(jnp.min(i1v), S - 1)
    i2 = jnp.minimum(jnp.min(i2v), S - 1)
    b1 = pl.multiple_of(i1 & (-16), 16)
    b2 = pl.multiple_of(i2 & (-16), 16)
    rows16 = lax.broadcasted_iota(jnp.int32, (16, M), 0)
    hn1 = hn_s[pl.ds(b1, 16), :].astype(F32)
    hn2 = hn_s[pl.ds(b2, 16), :].astype(F32)
    x1 = jnp.sum(jnp.where(rows16 == i1 - b1, hn1, 0.0), axis=0, keepdims=True)
    x2 = jnp.sum(jnp.where(rows16 == i2 - b2, hn2, 0.0), axis=0, keepdims=True)
    xs = jnp.where(rows16 == 0, x1, jnp.where(rows16 == 1, x2, 0.0)).astype(BF)

    g = _rb(jnp.dot(xs, wg_s[...], preferred_element_type=F32)[:8])
    u = _rb(jnp.dot(xs, wu_s[...], preferred_element_type=F32)[:8])
    g = _rb(g * jax.nn.sigmoid(g))
    gu = jnp.concatenate([g * u, jnp.zeros_like(g)], axis=0).astype(BF)
    y = _rb(jnp.dot(gu, wd_s[:, 0:M], preferred_element_type=F32)[:8])
    y1 = _rb(y[0:1, :] * _rb(jax.nn.sigmoid(m1)))
    y2 = _rb(y[1:2, :] * _rb(jax.nn.sigmoid(m2)))

    for i in range(ne):
        out_copy(i).wait()
    patch = []
    for n, (b, hnb) in enumerate(((b1, hn1), (b2, hn2))):
        rows = rows16 + b
        upd = jnp.where(rows == i1, y1, jnp.where(rows == i2, y2, 0.0))
        o_s[pl.ds(b, 16), :] = (h_s[pl.ds(b, 16), :].astype(F32) + _rb(hnb + upd)).astype(BF)
        patch.append(pltpu.make_async_copy(o_s.at[pl.ds(b, 16), :], out_hbm.at[pl.ds(b, 16), :], osem.at[n]))
    patch[0].start()

    @pl.when(b1 != b2)
    def _():
        patch[1].start()
        patch[1].wait()
    patch[0].wait()


@jax.jit
def pallas_sequential_preLN__compressed_kv_cla__moe_arch_mod__prompt_kernel(
        A_x, A_c_kv, A_w_q, A_w_uk, A_w_uv, A_w_o, B_x, B_w_r, B_w_gate, B_w_up, B_w_down):
    del B_x
    B, S, M = A_x.shape
    C = A_c_kv.shape[2]
    _, H, D = A_w_q.shape
    Fd = B_w_gate.shape[1]
    assert B == 1 and A_c_kv.shape[1] == S and M == 2 * C
    vmem = pltpu.VMEM
    dma = pltpu.SemaphoreType.DMA
    anyspec = pl.BlockSpec(memory_space=pl.ANY)
    out = pl.pallas_call(
        _kernel,
        in_specs=[anyspec] * 10,
        out_specs=anyspec,
        out_shape=jax.ShapeDtypeStruct((S, M), BF),
        scratch_shapes=[
            vmem((S, M), BF), vmem((S, C), BF), vmem((S // 2, C), U32),
            vmem((C // 8, H // 2, 4, 16, D), BF),
            vmem((H * D, M + 128), BF),
            vmem((M, Fd), BF), vmem((M, Fd), BF), vmem((Fd, M + 128), BF), vmem((M,), BF),
            vmem((S // 2, M), U32),
            vmem((S, D), BF), vmem((S // 2, D), U32), vmem((S // 2, D), U32),
            vmem((S // 2, D), U32), vmem((S // 2, D), U32), vmem((C // 2, 4 * D), U32),
            vmem((H, S, D), BF),
            vmem((S, M), BF), vmem((S, M), BF), vmem((S, M), BF),
            dma((5,)), dma((S // TQ,)), dma((S // TC,)), dma((9,)), dma((S // TE,)),
        ],
        compiler_params=pltpu.CompilerParams(vmem_limit_bytes=120 * 1024 * 1024),
    )(A_x.reshape(S, M), A_c_kv.reshape(S, C),
      A_w_q.reshape(C // 8, 2, 8, H // 2, 2, D), A_w_uk.reshape(C // 8, 8, H // 2, 2, D),
      A_w_uv.reshape(C // 8, 8, H // 2, 2, D), A_w_o.reshape(H * D, M),
      B_w_r, B_w_gate, B_w_up, B_w_down)
    return out.reshape(B, S, M)
```

```python
import math

import jax
import jax.numpy as jnp
from jax import lax
from jax.experimental import pallas as pl
from jax.experimental.pallas import tpu as pltpu

BF = jnp.bfloat16
F32 = jnp.float32
U32 = jnp.uint32
NT = (((1,), (1,)), ((), ()))
NEG = -1e30
EPS = 1e-5
BIG = 3e38

TQ = 256
TC = 512
TE = 256
TB = 64
CN = 16
XW = 5
DIST = 2


def _rb(x):
    return x.astype(BF).astype(F32)


def _after(x, dep):
    return x if dep is None else jnp.maximum(x, dep - BIG)


def _recip(l):
    r = pl.reciprocal(l, approx=True)
    return r * (2.0 - l * r)


def _ln_rows(x, dep):
    n = x.shape[-1]
    mu = _after(jnp.sum(x, axis=-1, keepdims=True), dep) * (1.0 / n)
    xc = x - mu
    var = jnp.sum(xc * xc, axis=-1, keepdims=True) * (1.0 / n)
    den = _rb(jnp.sqrt(_rb(_rb(var) + EPS)))
    num = _rb(x - _rb(mu))
    return (num * (1.0 / den)).astype(BF)


def _unpack(z, odd):
    u = pltpu.bitcast(z, U32)
    u = u.reshape(u.shape[0] * u.shape[1], u.shape[2])
    u = (u & jnp.uint32(0xFFFF0000)) if odd else (u << 16)
    return pltpu.bitcast(u, F32).astype(BF)


def _pk(x):
    return pltpu.bitcast(x, U32)


def _up(u):
    return pltpu.bitcast(u, BF)


def _kernel(x_hbm, c_hbm, wq_hbm, wk_hbm, wv_hbm, wo_hbm, wr_hbm, wg_hbm, wu_hbm, wd_hbm,
            out_hbm,
            x_s, c_s, cu_s, z_s, wo_s, wg_s, wu_s, wd_s, wr_s,
            xn_s, q_s, k_s, v_s, k0_s, v0_s, w4_s, ctx_s, h_s, hn_s, o_s,
            sem, xsem, csem, wsem, osem):
    S, M = x_s.shape
    H, _, D = ctx_s.shape
    nq = S // TQ
    ne = S // TE
    nc = S // TC
    scale = (D ** -0.5) * math.log2(math.e)
    PG = (0, 1, 2, H // 2)

    def w_start(i, g, priority):
        lo, hi = PG[g], PG[g + 1]
        for r in range(8):
            two = slice(2 * r, 2 * r + 2)
            if i < 2:
                cps = [((wk_hbm, wv_hbm)[i].at[:, r, lo:hi], z_s.at[:, lo:hi, i, two, :])]
            elif hi - lo == 1:
                cps = [(wq_hbm.at[:, :, r, lo], z_s.at[:, lo, 2:4, two, :])]
            else:
                cps = [(wq_hbm.at[:, b, r, lo:hi], z_s.at[:, lo:hi, 2 + b, two, :]) for b in range(2)]
            for src, dst in cps:
                pltpu.make_async_copy(src, dst, wsem.at[3 * g + i]).start(priority=priority)

    def w_wait(i, g):
        z = z_s.at[:, PG[g]:PG[g + 1], i:(i + 1 if i < 2 else 4)]
        pltpu.make_async_copy(z, z, wsem.at[3 * g + i]).wait()

    def x_copy(i):
        rows = pl.ds(pl.multiple_of(i * TQ, TQ), TQ)
        return pltpu.make_async_copy(x_hbm.at[rows, :], x_s.at[rows, :], xsem.at[i])

    def c_rows(i, div=1):
        t = TC // div
        if isinstance(i, int):
            assert i in (0, nc)
            return pl.ds(0 if i == 0 else S // div - t // 2, t // 2)
        return pl.ds(pl.multiple_of(i * t - t // 2, t // 2), t)

    def c_copy(i):
        return pltpu.make_async_copy(c_hbm.at[c_rows(i), :], c_s.at[c_rows(i), :], csem.at[i])

    def out_copy(i):
        rows = pl.ds(pl.multiple_of(i * TE, TE), TE)
        return pltpu.make_async_copy(o_s.at[rows, :], out_hbm.at[rows, :], osem.at[i])

    late = [pltpu.make_async_copy(src, dst, sem.at[i]) for i, (src, dst) in enumerate([
        (wo_hbm, wo_s.at[:, 0:M]), (wr_hbm, wr_s), (wg_hbm, wg_s), (wu_hbm, wu_s), (wd_hbm, wd_s.at[:, 0:M])])]

    def for_each(lo, hi, fn):
        def body(i, c):
            fn(i)
            return c
        lax.fori_loop(lo, hi, body, 0)

    w_start(0, 0, 0)
    w_start(1, 0, 0)
    c_copy(0).start()
    for_each(1, nc, lambda j: c_copy(j).start())
    c_copy(nc).start()
    w_start(2, 0, 0)
    for_each(0, nq, lambda j: x_copy(nq - 1 - j).start())
    for j in range(3):
        w_start(j, 1, 0)

    def get_wq(p, odd):
        z = z_s[:, p, 2:4]
        return _unpack(z.reshape(2 * z.shape[0], 16, D), odd)

    def kv_piece(wkv, r0):
        rows = slice(r0 // 2, (r0 + TQ) // 2)
        kv = jnp.dot(_up(cu_s[rows, :]), wkv, preferred_element_type=F32)
        k_s[rows, :] = _pk(kv[:, :D].astype(BF))
        v_s[rows, :] = _pk(kv[:, D:].astype(BF))

    def q_piece(wq, r0):
        rows = slice(r0 // 2, (r0 + TQ) // 2)
        q = jnp.dot(_up(xn_s[rows, :]), wq, preferred_element_type=F32)
        q_s[r0:r0 + TQ, :] = (q * scale).astype(BF)

    def ln1(i):
        for j in range(TQ // CN):
            r0 = i * TQ + j * CN
            x = x_s[r0:r0 + CN, :].astype(F32)
            xc = x - jnp.sum(x, axis=-1, keepdims=True) * (1.0 / M)
            var = jnp.sum(xc * xc, axis=-1, keepdims=True) * (1.0 / M)
            xn_s[r0 // 2:(r0 + CN) // 2, :] = _pk((xc * lax.rsqrt(var + EPS)).astype(BF))

    def attention(h, kr, vr, pre, gap, tail, deps):
        HB = TQ // 2
        row = lax.broadcasted_iota(jnp.int32, (HB, HB), 0)
        col = lax.broadcasted_iota(jnp.int32, (HB, HB), 1)
        tri = col <= row
        deps = list(deps)
        for i in range(nq - 1, -1, -1):
            n0 = i * TQ
            n1 = n0 + HB
            n2 = n0 + TQ
            pre(i)
            q = q_s[n0:n2, :]
            s = lax.dot_general(q, _up(kr[:n1 // 2, :]), NT, preferred_element_type=F32)
            s2 = lax.dot_general(q[HB:], _up(kr[n1 // 2:n2 // 2, :]), NT, preferred_element_type=F32)
            gap(i)
            sa = jnp.where(tri, s[:HB, n0:], NEG)
            sa = jnp.concatenate([s[:HB, :n0], sa], axis=1) if i > 0 else sa
            sb = s[HB:]
            s2 = jnp.where(tri, s2, NEG)
            da, db = deps.pop(0)
            ma = _after(jnp.max(sa, axis=1, keepdims=True), da)
            mb = _after(jnp.max(jnp.concatenate([sb, s2], axis=1), axis=1, keepdims=True), db)
            pa = jnp.exp2(sa - ma)
            pb = jnp.exp2(sb - mb)
            p2 = jnp.exp2(s2 - mb)
            la = _recip(jnp.sum(pa, axis=1, keepdims=True))
            lb = _recip(jnp.sum(jnp.concatenate([pb, p2], axis=1), axis=1, keepdims=True))
            deps.append((la, lb))
            p = jnp.concatenate([pa, pb], axis=0).astype(BF)
            o = jnp.dot(p, _up(vr[:n1 // 2, :]), preferred_element_type=F32)
            o2 = jnp.dot(p2.astype(BF), _up(vr[n1 // 2:n2 // 2, :]), preferred_element_type=F32)
            ctx_s[h, n0:n1, :] = (o[:HB] * la).astype(BF)
            ctx_s[h, n1:n2, :] = ((o[HB:] + o2) * lb).astype(BF)
        tail()
        return deps

    nodeps = [(None, None)] * DIST

    def nop(*_):
        return None

    w_wait(0, 0)
    w_wait(1, 0)
    for j in range(3):
        w_start(j, 2, 1)
    w4_s[...] = _pk(jnp.concatenate([_unpack(z_s[:, 0, i], odd) for odd in (0, 1) for i in (0, 1)], axis=1))

    def kv01(j):
        c = c_s[c_rows(j), :]
        cu_s[c_rows(j, 2), :] = _pk(c)
        kv = jnp.dot(c, _up(w4_s[...]), preferred_element_type=F32)
        for n, dst in enumerate((k0_s, v0_s, k_s, v_s)):
            dst[c_rows(j, 2), :] = _pk(kv[:, n * D:(n + 1) * D].astype(BF))

    c_copy(0).wait()
    kv01(0)
    for_each(1, nc, lambda j: (c_copy(j).wait(), kv01(j)))
    c_copy(nc).wait()
    w_wait(2, 0)
    x_copy(nq - 1).wait()
    ln1(nq - 1)
    kv01(nc)
    wq0 = get_wq(0, 0)
    wq1 = get_wq(0, 1)
    q_piece(wq0, (nq - 1) * TQ)
    for j in range(XW, nq - 1):
        x_copy(j).wait()

    def pre0(i):
        if i == XW:
            for j in range(XW):
                x_copy(j).wait()

    def gap0(i):
        q_piece(wq1, i * TQ)
        if i > 0:
            ln1(i - 1)
            q_piece(wq0, (i - 1) * TQ)

    attention(0, k0_s, v0_s, pre0, gap0, nop, nodeps)

    def head(h, p, odd, deps):
        wq = get_wq(p, odd)
        wkv = jnp.concatenate([_unpack(z_s[:, p, 0], odd), _unpack(z_s[:, p, 1], odd)], axis=1)

        def gap(i):
            if i > 0:
                q_piece(wq, i * TQ)
            if i + 1 < nq:
                kv_piece(wkv, (i + 1) * TQ)

        def tail():
            kv_piece(wkv, 0)
            q_piece(wq, 0)

        return attention(h, k_s, v_s, nop, gap, tail, deps)

    def two_heads(t):
        p = t + 1

        @pl.when(p == PG[2])
        def _():
            for i in range(3):
                w_wait(i, 2)
            for c in late:
                c.start(priority=1)

        head(2 * t + 2, p, 1, head(2 * t + 1, p, 0, nodeps))

    for i in range(3):
        w_wait(i, 1)
    for_each(0, H // 2 - 1, two_heads)

    late[0].wait()
    late[1].wait()
    wr = wr_s[...].astype(F32).reshape(1, M)

    def post(r0, hv, n, deps, top):
        b1, j1, b2, j2 = top
        for j in range(n // CN - 1, -1, -1):
            rows = pl.ds(r0 + j * CN, CN)
            hf = hv[j * CN:(j + 1) * CN, :].astype(F32)
            hn = _ln_rows(hf, deps.pop(0))
            hnf = hn.astype(F32)
            r = _rb(jnp.sum(hnf * wr, axis=-1, keepdims=True))
            hn_s[rows, :] = hn
            o_s[rows, :] = (hf + hnf).astype(BF)
            deps.append(r)
            tok = lax.broadcasted_iota(jnp.int32, (CN, 1), 0) + (r0 + j * CN)
            ge1 = r >= b1
            ge2 = r >= b2
            b2 = jnp.where(ge1, b1, jnp.where(ge2, r, b2))
            j2 = jnp.where(ge1, j1, jnp.where(ge2, tok, j2))
            b1 = jnp.where(ge1, r, b1)
            j1 = jnp.where(ge1, tok, j1)
        return b1, j1, b2, j2

    def o_proj(r0, n, hv, cols=slice(0, M)):
        rows = pl.ds(r0, n)
        ctx = jnp.concatenate([ctx_s[hh, rows, :] for hh in range(H)], axis=1)
        a = jnp.dot(ctx, wo_s[:, cols], preferred_element_type=F32)
        hv[:, cols] = (x_s[rows, cols].astype(F32) + _rb(a)).astype(BF)

    def o_piece(n):
        o_proj(S - TE, TE, h_s.at[S - TE:S, :], slice(n * (M // nq), (n + 1) * (M // nq)))

    attention(H - 1, k_s, v_s, nop, lambda i: o_piece(i + 1) if i + 1 < nq else None, lambda: o_piece(0), nodeps)

    def epi(t, top):
        i = ne - 1 - (t + 1)
        r0 = pl.multiple_of(i * TE, TE)
        hv = h_s.at[pl.ds(r0, 2 * TE), :]
        top = post(r0 + TE, hv.at[TE:2 * TE, :], TE, [None], top)
        o_proj(r0, TE, hv.at[0:TE, :])
        out_copy(i + 1).start()
        return top

    ninf = jnp.full((CN, 1), -jnp.inf, F32)
    none = jnp.full((CN, 1), S, jnp.int32)
    top = lax.fori_loop(0, ne - 2, epi, (ninf, none, ninf, none))
    for c in late[2:]:
        c.wait()
    deps = [None]
    top = post(TE, h_s.at[TE:2 * TE, :], TE, deps, top)
    o_proj(TB, TE - TB, h_s.at[TB:TE, :])
    out_copy(1).start()
    top = post(TB, h_s.at[TB:TE, :], TE - TB, deps, top)
    o_proj(0, TB, h_s.at[0:TB, :])
    top = post(0, h_s.at[0:TB, :], TB, deps * (TB // CN), top)
    out_copy(0).start()

    r = jnp.concatenate([top[0], top[2]], axis=0)
    idx = jnp.concatenate([top[1], top[3]], axis=0)
    m1 = jnp.max(r, axis=0, keepdims=True)
    i1v = jnp.min(jnp.where(r == m1, idx, S), axis=0, keepdims=True)
    r2 = jnp.where(idx == i1v, -jnp.inf, r)
    m2 = jnp.max(r2, axis=0, keepdims=True)
    i2v = jnp.min(jnp.where((r2 == m2) & (idx != i1v), idx, S), axis=0, keepdims=True)
    i1 = jnp.minimum(jnp.min(i1v), S - 1)
    i2 = jnp.minimum(jnp.min(i2v), S - 1)
    b1 = pl.multiple_of(i1 & (-16), 16)
    b2 = pl.multiple_of(i2 & (-16), 16)
    rows16 = lax.broadcasted_iota(jnp.int32, (16, M), 0)
    hn1 = hn_s[pl.ds(b1, 16), :].astype(F32)
    hn2 = hn_s[pl.ds(b2, 16), :].astype(F32)
    x1 = jnp.sum(jnp.where(rows16 == i1 - b1, hn1, 0.0), axis=0, keepdims=True)
    x2 = jnp.sum(jnp.where(rows16 == i2 - b2, hn2, 0.0), axis=0, keepdims=True)
    xs = jnp.where(rows16 == 0, x1, jnp.where(rows16 == 1, x2, 0.0)).astype(BF)

    g = _rb(jnp.dot(xs, wg_s[...], preferred_element_type=F32)[:8])
    u = _rb(jnp.dot(xs, wu_s[...], preferred_element_type=F32)[:8])
    g = _rb(g * jax.nn.sigmoid(g))
    gu = jnp.concatenate([g * u, jnp.zeros_like(g)], axis=0).astype(BF)
    y = _rb(jnp.dot(gu, wd_s[:, 0:M], preferred_element_type=F32)[:8])
    y1 = _rb(y[0:1, :] * _rb(jax.nn.sigmoid(m1)))
    y2 = _rb(y[1:2, :] * _rb(jax.nn.sigmoid(m2)))

    for i in range(ne):
        out_copy(i).wait()
    patch = []
    for n, (b, hnb) in enumerate(((b1, hn1), (b2, hn2))):
        rows = rows16 + b
        upd = jnp.where(rows == i1, y1, jnp.where(rows == i2, y2, 0.0))
        o_s[pl.ds(b, 16), :] = (h_s[pl.ds(b, 16), :].astype(F32) + _rb(hnb + upd)).astype(BF)
        patch.append(pltpu.make_async_copy(o_s.at[pl.ds(b, 16), :], out_hbm.at[pl.ds(b, 16), :], osem.at[n]))
    patch[0].start()

    @pl.when(b1 != b2)
    def _():
        patch[1].start()
        patch[1].wait()
    patch[0].wait()


@jax.jit
def pallas_sequential_preLN__compressed_kv_cla__moe_arch_mod__prompt_kernel(
        A_x, A_c_kv, A_w_q, A_w_uk, A_w_uv, A_w_o, B_x, B_w_r, B_w_gate, B_w_up, B_w_down):
    del B_x
    B, S, M = A_x.shape
    C = A_c_kv.shape[2]
    _, H, D = A_w_q.shape
    Fd = B_w_gate.shape[1]
    assert B == 1 and A_c_kv.shape[1] == S and M == 2 * C
    vmem = pltpu.VMEM
    dma = pltpu.SemaphoreType.DMA
    anyspec = pl.BlockSpec(memory_space=pl.ANY)
    out = pl.pallas_call(
        _kernel,
        in_specs=[anyspec] * 10,
        out_specs=anyspec,
        out_shape=jax.ShapeDtypeStruct((S, M), BF),
        scratch_shapes=[
            vmem((S, M), BF), vmem((S, C), BF), vmem((S // 2, C), U32),
            vmem((C // 8, H // 2, 4, 16, D), BF),
            vmem((H * D, M + 128), BF),
            vmem((M, Fd), BF), vmem((M, Fd), BF), vmem((Fd, M + 128), BF), vmem((M,), BF),
            vmem((S // 2, M), U32),
            vmem((S, D), BF), vmem((S // 2, D), U32), vmem((S // 2, D), U32),
            vmem((S // 2, D), U32), vmem((S // 2, D), U32), vmem((C // 2, 4 * D), U32),
            vmem((H, S, D), BF),
            vmem((S, M), BF), vmem((S, M), BF), vmem((S, M), BF),
            dma((5,)), dma((S // TQ,)), dma((S // TC + 1,)), dma((9,)), dma((S // TE,)),
        ],
        compiler_params=pltpu.CompilerParams(vmem_limit_bytes=120 * 1024 * 1024),
    )(A_x.reshape(S, M), A_c_kv.reshape(S, C),
      A_w_q.reshape(C // 8, 2, 8, H // 2, 2, D), A_w_uk.reshape(C // 8, 8, H // 2, 2, D),
      A_w_uv.reshape(C // 8, 8, H // 2, 2, D), A_w_o.reshape(H * D, M),
      B_w_r, B_w_gate, B_w_up, B_w_down)
    return out.reshape(B, S, M)
```

```python
import math

import jax
import jax.numpy as jnp
from jax import lax
from jax.experimental import pallas as pl
from jax.experimental.pallas import tpu as pltpu

BF = jnp.bfloat16
F32 = jnp.float32
U32 = jnp.uint32
NT = (((1,), (1,)), ((), ()))
NEG = -1e30
EPS = 1e-5
BIG = 3e38

TQ = 256
TC = 512
TE = 256
TB = 64
CN = 16
XW = 5
DIST = 2


def _rb(x):
    return x.astype(BF).astype(F32)


def _after(x, dep):
    return x if dep is None else jnp.maximum(x, dep - BIG)


def _recip(l):
    r = pl.reciprocal(l, approx=True)
    return r * (2.0 - l * r)


def _ln_rows(x, dep):
    n = x.shape[-1]
    mu = _after(jnp.sum(x, axis=-1, keepdims=True), dep) * (1.0 / n)
    xc = x - mu
    var = jnp.sum(xc * xc, axis=-1, keepdims=True) * (1.0 / n)
    den = _rb(jnp.sqrt(_rb(_rb(var) + EPS)))
    num = _rb(x - _rb(mu))
    return (num * (1.0 / den)).astype(BF)


def _unpack(z, odd):
    u = pltpu.bitcast(z, U32)
    u = u.reshape(u.shape[0] * u.shape[1], u.shape[2])
    u = (u & jnp.uint32(0xFFFF0000)) if odd else (u << 16)
    return pltpu.bitcast(u, F32).astype(BF)


def _pk(x):
    return pltpu.bitcast(x, U32)


def _up(u):
    return pltpu.bitcast(u, BF)


def _kernel(x_hbm, c_hbm, wq_hbm, wk_hbm, wv_hbm, wo_hbm, wr_hbm, wg_hbm, wu_hbm, wd_hbm,
            out_hbm,
            x_s, c_s, cu_s, z_s, wo_s, wg_s, wu_s, wd_s, wr_s,
            xn_s, q_s, k_s, v_s, k0_s, v0_s, w4_s, ctx_s, h_s, hn_s, o_s,
            sem, xsem, csem, wsem, osem):
    S, M = x_s.shape
    H, _, D = ctx_s.shape
    nq = S // TQ
    ne = S // TE
    nc = S // TC
    scale = (D ** -0.5) * math.log2(math.e)
    PG = (0, 1, 2, H // 2)

    def w_start(i, g, priority):
        lo, hi = PG[g], PG[g + 1]
        for r in range(8):
            two = slice(2 * r, 2 * r + 2)
            if i < 2:
                cps = [((wk_hbm, wv_hbm)[i].at[:, r, lo:hi], z_s.at[:, lo:hi, i, two, :])]
            elif hi - lo == 1:
                cps = [(wq_hbm.at[:, :, r, lo], z_s.at[:, lo, 2:4, two, :])]
            else:
                cps = [(wq_hbm.at[:, b, r, lo:hi], z_s.at[:, lo:hi, 2 + b, two, :]) for b in range(2)]
            for src, dst in cps:
                pltpu.make_async_copy(src, dst, wsem.at[3 * g + i]).start(priority=priority)

    def w_wait(i, g):
        z = z_s.at[:, PG[g]:PG[g + 1], i:(i + 1 if i < 2 else 4)]
        pltpu.make_async_copy(z, z, wsem.at[3 * g + i]).wait()

    def x_copy(i):
        rows = pl.ds(pl.multiple_of(i * TQ, TQ), TQ)
        return pltpu.make_async_copy(x_hbm.at[rows, :], x_s.at[rows, :], xsem.at[i])

    def c_rows(i, div=1):
        t = TC // div
        if isinstance(i, int):
            assert i in (0, nc)
            return pl.ds(0 if i == 0 else S // div - t // 2, t // 2)
        return pl.ds(pl.multiple_of(i * t - t // 2, t // 2), t)

    def c_copy(i):
        return pltpu.make_async_copy(c_hbm.at[c_rows(i), :], c_s.at[c_rows(i), :], csem.at[i])

    def out_copy(i):
        rows = pl.ds(pl.multiple_of(i * TE, TE), TE)
        return pltpu.make_async_copy(o_s.at[rows, :], out_hbm.at[rows, :], osem.at[i])

    late = [pltpu.make_async_copy(src, dst, sem.at[i]) for i, (src, dst) in enumerate([
        (wo_hbm, wo_s.at[:, 0:M]), (wr_hbm, wr_s), (wg_hbm, wg_s), (wu_hbm, wu_s), (wd_hbm, wd_s.at[:, 0:M])])]

    def for_each(lo, hi, fn):
        def body(i, c):
            fn(i)
            return c
        lax.fori_loop(lo, hi, body, 0)

    w_start(0, 0, 0)
    w_start(1, 0, 0)
    c_copy(0).start()
    for_each(1, nc, lambda j: c_copy(j).start())
    c_copy(nc).start()
    w_start(2, 0, 0)
    for_each(0, nq, lambda j: x_copy(nq - 1 - j).start())
    for j in range(3):
        w_start(j, 1, 0)

    def get_wq(p, odd):
        z = z_s[:, p, 2:4]
        return _unpack(z.reshape(2 * z.shape[0], 16, D), odd)

    def kv_piece(wkv, r0):
        rows = slice(r0 // 2, (r0 + TQ) // 2)
        kv = jnp.dot(_up(cu_s[rows, :]), wkv, preferred_element_type=F32)
        k_s[rows, :] = _pk(kv[:, :D].astype(BF))
        v_s[rows, :] = _pk(kv[:, D:].astype(BF))

    def q_piece(wq, r0):
        rows = slice(r0 // 2, (r0 + TQ) // 2)
        q = jnp.dot(_up(xn_s[rows, :]), wq, preferred_element_type=F32)
        q_s[r0:r0 + TQ, :] = (q * scale).astype(BF)

    def ln1(i):
        for j in range(TQ // CN):
            r0 = i * TQ + j * CN
            x = x_s[r0:r0 + CN, :].astype(F32)
            xc = x - jnp.sum(x, axis=-1, keepdims=True) * (1.0 / M)
            var = jnp.sum(xc * xc, axis=-1, keepdims=True) * (1.0 / M)
            xn_s[r0 // 2:(r0 + CN) // 2, :] = _pk((xc * lax.rsqrt(var + EPS)).astype(BF))

    def attention(h, kr, vr, pre, gap, tail, deps, lazy=False):
        HB = TQ // 2
        row = lax.broadcasted_iota(jnp.int32, (HB, HB), 0)
        col = lax.broadcasted_iota(jnp.int32, (HB, HB), 1)
        tri = col <= row
        deps = list(deps)
        for i in range(nq - 1, -1, -1):
            n0 = i * TQ
            n1 = n0 + HB
            n2 = n0 + TQ
            pre(i)
            q = q_s[n0:n2, :]
            s = lax.dot_general(q, _up(kr[:n1 // 2, :]), NT, preferred_element_type=F32)
            s2 = lax.dot_general(q[HB:], _up(kr[n1 // 2:n2 // 2, :]), NT, preferred_element_type=F32)
            gap(i)
            sa = jnp.where(tri, s[:HB, n0:], NEG)
            sa = jnp.concatenate([s[:HB, :n0], sa], axis=1) if i > 0 else sa
            sb = s[HB:]
            s2 = jnp.where(tri, s2, NEG)
            da, db = deps.pop(0)()
            ma = _after(jnp.max(sa, axis=1, keepdims=True), da)
            mb = _after(jnp.max(jnp.concatenate([sb, s2], axis=1), axis=1, keepdims=True), db)
            pa = jnp.exp2(sa - ma)
            pb = jnp.exp2(sb - mb)
            p2 = jnp.exp2(s2 - mb)
            p = jnp.concatenate([pa, pb], axis=0).astype(BF)
            o = jnp.dot(p, _up(vr[:n1 // 2, :]), preferred_element_type=F32)
            o2 = jnp.dot(p2.astype(BF), _up(vr[n1 // 2:n2 // 2, :]), preferred_element_type=F32)

            def normalise(pa=pa, pb=pb, p2=p2, o=o, o2=o2, n0=n0, n1=n1, n2=n2):
                la = _recip(jnp.sum(pa, axis=1, keepdims=True))
                lb = _recip(jnp.sum(jnp.concatenate([pb, p2], axis=1), axis=1, keepdims=True))
                ctx_s[h, n0:n1, :] = (o[:HB] * la).astype(BF)
                ctx_s[h, n1:n2, :] = ((o[HB:] + o2) * lb).astype(BF)
                return la, lb

            deps.append(normalise if lazy else (lambda v=normalise(): v))
        if lazy:
            deps = [(lambda v=f(): v) for f in deps]
        tail()
        return deps

    nodeps = [lambda: (None, None)] * DIST

    def nop(*_):
        return None

    w_wait(0, 0)
    w_wait(1, 0)
    for j in range(3):
        w_start(j, 2, 1)
    w4_s[...] = _pk(jnp.concatenate([_unpack(z_s[:, 0, i], odd) for odd in (0, 1) for i in (0, 1)], axis=1))

    def kv01(j):
        c = c_s[c_rows(j), :]
        cu_s[c_rows(j, 2), :] = _pk(c)
        kv = jnp.dot(c, _up(w4_s[...]), preferred_element_type=F32)
        for n, dst in enumerate((k0_s, v0_s, k_s, v_s)):
            dst[c_rows(j, 2), :] = _pk(kv[:, n * D:(n + 1) * D].astype(BF))

    c_copy(0).wait()
    kv01(0)
    for_each(1, nc, lambda j: (c_copy(j).wait(), kv01(j)))
    c_copy(nc).wait()
    w_wait(2, 0)
    x_copy(nq - 1).wait()
    ln1(nq - 1)
    kv01(nc)
    wq0 = get_wq(0, 0)
    wq1 = get_wq(0, 1)
    q_piece(wq0, (nq - 1) * TQ)
    for j in range(XW, nq - 1):
        x_copy(j).wait()

    def pre0(i):
        if i == XW:
            for j in range(XW):
                x_copy(j).wait()

    def gap0(i):
        if i != 1:
            q_piece(wq1, i * TQ)
        if i > 0:
            ln1(i - 1)
            q_piece(wq0, (i - 1) * TQ)

    attention(0, k0_s, v0_s, pre0, gap0, lambda: q_piece(wq1, TQ), nodeps, lazy=True)

    def head(h, p, odd, deps):
        wq = get_wq(p, odd)
        wkv = jnp.concatenate([_unpack(z_s[:, p, 0], odd), _unpack(z_s[:, p, 1], odd)], axis=1)

        def gap(i):
            if i > 0:
                q_piece(wq, i * TQ)
            if i + 1 < nq:
                kv_piece(wkv, (i + 1) * TQ)

        def tail():
            kv_piece(wkv, 0)
            q_piece(wq, 0)

        return attention(h, k_s, v_s, nop, gap, tail, deps)

    def two_heads(t):
        p = t + 1

        @pl.when(p == PG[2])
        def _():
            for i in range(3):
                w_wait(i, 2)
            for c in late:
                c.start(priority=1)

        head(2 * t + 2, p, 1, head(2 * t + 1, p, 0, nodeps))

    for i in range(3):
        w_wait(i, 1)
    for_each(0, H // 2 - 1, two_heads)

    late[0].wait()
    late[1].wait()
    wr = wr_s[...].astype(F32).reshape(1, M)

    def post(r0, hv, n, deps, top):
        b1, j1, b2, j2 = top
        for j in range(n // CN - 1, -1, -1):
            rows = pl.ds(r0 + j * CN, CN)
            hf = hv[j * CN:(j + 1) * CN, :].astype(F32)
            hn = _ln_rows(hf, deps.pop(0))
            hnf = hn.astype(F32)
            r = _rb(jnp.sum(hnf * wr, axis=-1, keepdims=True))
            hn_s[rows, :] = hn
            o_s[rows, :] = (hf + hnf).astype(BF)
            deps.append(r)
            tok = lax.broadcasted_iota(jnp.int32, (CN, 1), 0) + (r0 + j * CN)
            ge1 = r >= b1
            ge2 = r >= b2
            b2 = jnp.where(ge1, b1, jnp.where(ge2, r, b2))
            j2 = jnp.where(ge1, j1, jnp.where(ge2, tok, j2))
            b1 = jnp.where(ge1, r, b1)
            j1 = jnp.where(ge1, tok, j1)
        return b1, j1, b2, j2

    def o_proj(r0, n, hv, cols=slice(0, M)):
        rows = pl.ds(r0, n)
        ctx = jnp.concatenate([ctx_s[hh, rows, :] for hh in range(H)], axis=1)
        a = jnp.dot(ctx, wo_s[:, cols], preferred_element_type=F32)
        hv[:, cols] = (x_s[rows, cols].astype(F32) + _rb(a)).astype(BF)

    def o_piece(n):
        o_proj(S - TE, TE, h_s.at[S - TE:S, :], slice(n * (M // nq), (n + 1) * (M // nq)))

    attention(H - 1, k_s, v_s, nop, lambda i: o_piece(i + 1) if i + 1 < nq else None, lambda: o_piece(0), nodeps)

    def epi(t, top):
        i = ne - 1 - (t + 1)
        r0 = pl.multiple_of(i * TE, TE)
        hv = h_s.at[pl.ds(r0, 2 * TE), :]
        top = post(r0 + TE, hv.at[TE:2 * TE, :], TE, [None], top)
        o_proj(r0, TE, hv.at[0:TE, :])
        out_copy(i + 1).start()
        return top

    ninf = jnp.full((CN, 1), -jnp.inf, F32)
    none = jnp.full((CN, 1), S, jnp.int32)
    top = lax.fori_loop(0, ne - 2, epi, (ninf, none, ninf, none))
    for c in late[2:]:
        c.wait()
    deps = [None]
    top = post(TE, h_s.at[TE:2 * TE, :], TE, deps, top)
    o_proj(TB, TE - TB, h_s.at[TB:TE, :])
    out_copy(1).start()
    top = post(TB, h_s.at[TB:TE, :], TE - TB, deps, top)
    o_proj(0, TB, h_s.at[0:TB, :])
    top = post(0, h_s.at[0:TB, :], TB, deps * (TB // CN), top)
    out_copy(0).start()

    r = jnp.concatenate([top[0], top[2]], axis=0)
    idx = jnp.concatenate([top[1], top[3]], axis=0)
    m1 = jnp.max(r, axis=0, keepdims=True)
    i1v = jnp.min(jnp.where(r == m1, idx, S), axis=0, keepdims=True)
    r2 = jnp.where(idx == i1v, -jnp.inf, r)
    m2 = jnp.max(r2, axis=0, keepdims=True)
    i2v = jnp.min(jnp.where((r2 == m2) & (idx != i1v), idx, S), axis=0, keepdims=True)
    i1 = jnp.minimum(jnp.min(i1v), S - 1)
    i2 = jnp.minimum(jnp.min(i2v), S - 1)
    b1 = pl.multiple_of(i1 & (-16), 16)
    b2 = pl.multiple_of(i2 & (-16), 16)
    rows16 = lax.broadcasted_iota(jnp.int32, (16, M), 0)
    hn1 = hn_s[pl.ds(b1, 16), :].astype(F32)
    hn2 = hn_s[pl.ds(b2, 16), :].astype(F32)
    x1 = jnp.sum(jnp.where(rows16 == i1 - b1, hn1, 0.0), axis=0, keepdims=True)
    x2 = jnp.sum(jnp.where(rows16 == i2 - b2, hn2, 0.0), axis=0, keepdims=True)
    xs = jnp.where(rows16 == 0, x1, jnp.where(rows16 == 1, x2, 0.0)).astype(BF)

    g = _rb(jnp.dot(xs, wg_s[...], preferred_element_type=F32)[:8])
    u = _rb(jnp.dot(xs, wu_s[...], preferred_element_type=F32)[:8])
    g = _rb(g * jax.nn.sigmoid(g))
    gu = jnp.concatenate([g * u, jnp.zeros_like(g)], axis=0).astype(BF)
    y = _rb(jnp.dot(gu, wd_s[:, 0:M], preferred_element_type=F32)[:8])
    y1 = _rb(y[0:1, :] * _rb(jax.nn.sigmoid(m1)))
    y2 = _rb(y[1:2, :] * _rb(jax.nn.sigmoid(m2)))

    for i in range(ne):
        out_copy(i).wait()
    patch = []
    for n, (b, hnb) in enumerate(((b1, hn1), (b2, hn2))):
        rows = rows16 + b
        upd = jnp.where(rows == i1, y1, jnp.where(rows == i2, y2, 0.0))
        o_s[pl.ds(b, 16), :] = (h_s[pl.ds(b, 16), :].astype(F32) + _rb(hnb + upd)).astype(BF)
        patch.append(pltpu.make_async_copy(o_s.at[pl.ds(b, 16), :], out_hbm.at[pl.ds(b, 16), :], osem.at[n]))
    patch[0].start()

    @pl.when(b1 != b2)
    def _():
        patch[1].start()
        patch[1].wait()
    patch[0].wait()


@jax.jit
def pallas_sequential_preLN__compressed_kv_cla__moe_arch_mod__prompt_kernel(
        A_x, A_c_kv, A_w_q, A_w_uk, A_w_uv, A_w_o, B_x, B_w_r, B_w_gate, B_w_up, B_w_down):
    del B_x
    B, S, M = A_x.shape
    C = A_c_kv.shape[2]
    _, H, D = A_w_q.shape
    Fd = B_w_gate.shape[1]
    assert B == 1 and A_c_kv.shape[1] == S and M == 2 * C
    vmem = pltpu.VMEM
    dma = pltpu.SemaphoreType.DMA
    anyspec = pl.BlockSpec(memory_space=pl.ANY)
    out = pl.pallas_call(
        _kernel,
        in_specs=[anyspec] * 10,
        out_specs=anyspec,
        out_shape=jax.ShapeDtypeStruct((S, M), BF),
        scratch_shapes=[
            vmem((S, M), BF), vmem((S, C), BF), vmem((S // 2, C), U32),
            vmem((C // 8, H // 2, 4, 16, D), BF),
            vmem((H * D, M + 128), BF),
            vmem((M, Fd), BF), vmem((M, Fd), BF), vmem((Fd, M + 128), BF), vmem((M,), BF),
            vmem((S // 2, M), U32),
            vmem((S, D), BF), vmem((S // 2, D), U32), vmem((S // 2, D), U32),
            vmem((S // 2, D), U32), vmem((S // 2, D), U32), vmem((C // 2, 4 * D), U32),
            vmem((H, S, D), BF),
            vmem((S, M), BF), vmem((S, M), BF), vmem((S, M), BF),
            dma((5,)), dma((S // TQ,)), dma((S // TC + 1,)), dma((9,)), dma((S // TE,)),
        ],
        compiler_params=pltpu.CompilerParams(vmem_limit_bytes=120 * 1024 * 1024),
    )(A_x.reshape(S, M), A_c_kv.reshape(S, C),
      A_w_q.reshape(C // 8, 2, 8, H // 2, 2, D), A_w_uk.reshape(C // 8, 8, H // 2, 2, D),
      A_w_uv.reshape(C // 8, 8, H // 2, 2, D), A_w_o.reshape(H * D, M),
      B_w_r, B_w_gate, B_w_up, B_w_down)
    return out.reshape(B, S, M)
```

```python
import math

import jax
import jax.numpy as jnp
from jax import lax
from jax.experimental import pallas as pl
from jax.experimental.pallas import tpu as pltpu

BF = jnp.bfloat16
F32 = jnp.float32
U32 = jnp.uint32
NT = (((1,), (1,)), ((), ()))
NEG = -1e30
EPS = 1e-5
BIG = 3e38

TQ = 256
TC = 512
TE = 256
TB = 64
CN = 16
XW = 5
DIST = 2


def _rb(x):
    return x.astype(BF).astype(F32)


def _after(x, dep):
    return x if dep is None else jnp.maximum(x, dep - BIG)


def _recip(l):
    r = pl.reciprocal(l, approx=True)
    return r * (2.0 - l * r)


def _ln_rows(x, dep):
    n = x.shape[-1]
    mu = _after(jnp.sum(x, axis=-1, keepdims=True), dep) * (1.0 / n)
    xc = x - mu
    var = jnp.sum(xc * xc, axis=-1, keepdims=True) * (1.0 / n)
    den = _rb(jnp.sqrt(_rb(_rb(var) + EPS)))
    num = _rb(x - _rb(mu))
    return (num * (1.0 / den)).astype(BF)


def _unpack(z, odd):
    u = pltpu.bitcast(z, U32)
    u = u.reshape(u.shape[0] * u.shape[1], u.shape[2])
    u = (u & jnp.uint32(0xFFFF0000)) if odd else (u << 16)
    return pltpu.bitcast(u, F32).astype(BF)


def _pk(x):
    return pltpu.bitcast(x, U32)


def _up(u):
    return pltpu.bitcast(u, BF)


def _kernel(x_hbm, c_hbm, wq_hbm, wk_hbm, wv_hbm, wo_hbm, wr_hbm, wg_hbm, wu_hbm, wd_hbm,
            out_hbm,
            x_s, c_s, cu_s, z_s, wo_s, wg_s, wu_s, wd_s, wr_s,
            xn_s, q_s, k_s, v_s, k0_s, v0_s, w4_s, ctx_s, h_s, hn_s, o_s, p_s,
            sem):
    S, M = x_s.shape
    H, _, D = ctx_s.shape
    nq = S // TQ
    ne = S // TE
    nc = S // TC
    scale = (D ** -0.5) * math.log2(math.e)
    PG = (0, 1, 2, H // 2)

    S_KV, S_XA, S_XB, S_G1, S_G2, S_C = range(6)
    S_Q = S_C + nc
    S_WO, S_FFN, S_OUT = S_KV, S_XA, S_XB

    def w_sem(i, g):
        return sem.at[(S_KV if i < 2 else S_Q, S_G1, S_G2)[g]]

    def w_start(i, g, priority):
        lo, hi = PG[g], PG[g + 1]
        for r in range(8):
            two = slice(2 * r, 2 * r + 2)
            if i < 2:
                cps = [((wk_hbm, wv_hbm)[i].at[:, r, lo:hi], z_s.at[:, lo:hi, i, two, :])]
            elif hi - lo == 1:
                cps = [(wq_hbm.at[:, :, r, lo], z_s.at[:, lo, 2:4, two, :])]
            else:
                cps = [(wq_hbm.at[:, b, r, lo:hi], z_s.at[:, lo:hi, 2 + b, two, :]) for b in range(2)]
            for src, dst in cps:
                pltpu.make_async_copy(src, dst, w_sem(i, g)).start(priority=priority)

    def w_wait(i, g):
        z = z_s.at[:, PG[g]:PG[g + 1], i:(i + 1 if i < 2 else 4)]
        pltpu.make_async_copy(z, z, w_sem(i, g)).wait()

    def x_copy(i, s):
        rows = pl.ds(pl.multiple_of(i * TQ, TQ), TQ)
        return pltpu.make_async_copy(x_hbm.at[rows, :], x_s.at[rows, :], sem.at[s])

    def c_rows(i, div=1):
        t = TC // div
        if isinstance(i, int):
            assert i in (0, nc)
            return pl.ds(0 if i == 0 else S // div - t // 2, t // 2)
        return pl.ds(pl.multiple_of(i * t - t // 2, t // 2), t)

    def c_copy(i):
        return pltpu.make_async_copy(c_hbm.at[c_rows(i), :], c_s.at[c_rows(i), :], sem.at[S_C + i])

    def out_copy(i):
        rows = pl.ds(pl.multiple_of(i * TE, TE), TE)
        return pltpu.make_async_copy(o_s.at[rows, :], out_hbm.at[rows, :], sem.at[S_OUT])

    late = [pltpu.make_async_copy(src, dst, sem.at[S_WO if i < 2 else S_FFN]) for i, (src, dst) in enumerate([
        (wo_hbm, wo_s.at[:, 0:M]), (wr_hbm, wr_s), (wg_hbm, wg_s), (wu_hbm, wu_s), (wd_hbm, wd_s.at[:, 0:M])])]

    def for_each(lo, hi, fn):
        def body(i, c):
            fn(i)
            return c
        lax.fori_loop(lo, hi, body, 0)

    w_start(0, 0, 0)
    w_start(1, 0, 0)
    c_copy(0).start()
    for_each(1, nc, lambda j: c_copy(j).start())
    c_copy(nc).start()
    w_start(2, 0, 0)
    x_copy(nq - 1, S_Q).start()
    for_each(XW, nq - 1, lambda j: x_copy(j, S_XA).start())
    for_each(0, XW, lambda j: x_copy(j, S_XB).start())
    for j in range(3):
        w_start(j, 1, 0)

    def get_wq(p, odd):
        z = z_s[:, p, 2:4]
        return _unpack(z.reshape(2 * z.shape[0], 16, D), odd)

    def kv_piece(wkv, r0):
        rows = slice(r0 // 2, (r0 + TQ) // 2)
        kv = jnp.dot(_up(cu_s[rows, :]), wkv, preferred_element_type=F32)
        k_s[rows, :] = _pk(kv[:, :D].astype(BF))
        v_s[rows, :] = _pk(kv[:, D:].astype(BF))

    def q_piece(wq, r0):
        rows = slice(r0 // 2, (r0 + TQ) // 2)
        q = jnp.dot(_up(xn_s[rows, :]), wq, preferred_element_type=F32)
        q_s[r0:r0 + TQ, :] = (q * scale).astype(BF)

    def ln1(i):
        for j in range(TQ // CN):
            r0 = i * TQ + j * CN
            x = x_s[r0:r0 + CN, :].astype(F32)
            xc = x - jnp.sum(x, axis=-1, keepdims=True) * (1.0 / M)
            var = jnp.sum(xc * xc, axis=-1, keepdims=True) * (1.0 / M)
            xn_s[r0 // 2:(r0 + CN) // 2, :] = _pk((xc * lax.rsqrt(var + EPS)).astype(BF))

    def attention(h, kr, vr, pre, gap, tail, deps, lazy=False):
        HB = TQ // 2
        row = lax.broadcasted_iota(jnp.int32, (HB, HB), 0)
        col = lax.broadcasted_iota(jnp.int32, (HB, HB), 1)
        tri = col <= row
        deps = list(deps)
        for i in range(nq - 1, -1, -1):
            n0 = i * TQ
            n1 = n0 + HB
            n2 = n0 + TQ
            pre(i)
            q = q_s[n0:n2, :]
            s = lax.dot_general(q, _up(kr[:n1 // 2, :]), NT, preferred_element_type=F32)
            s2 = lax.dot_general(q[HB:], _up(kr[n1 // 2:n2 // 2, :]), NT, preferred_element_type=F32)
            gap(i)
            sa = jnp.where(tri, s[:HB, n0:], NEG)
            sa = jnp.concatenate([s[:HB, :n0], sa], axis=1) if i > 0 else sa
            sb = s[HB:]
            s2 = jnp.where(tri, s2, NEG)
            da, db = deps.pop(0)()
            ma = _after(jnp.max(sa, axis=1, keepdims=True), da)
            mb = _after(jnp.max(jnp.concatenate([sb, s2], axis=1), axis=1, keepdims=True), db)
            pa = jnp.exp2(sa - ma)
            pb = jnp.exp2(sb - mb)
            p2 = jnp.exp2(s2 - mb)
            p = jnp.concatenate([pa, pb], axis=0).astype(BF)
            o = jnp.dot(p, _up(vr[:n1 // 2, :]), preferred_element_type=F32)
            o2 = jnp.dot(p2.astype(BF), _up(vr[n1 // 2:n2 // 2, :]), preferred_element_type=F32)

            def normalise(pa=pa, pb=pb, p2=p2, o=o, o2=o2, n0=n0, n1=n1, n2=n2):
                la = _recip(jnp.sum(pa, axis=1, keepdims=True))
                lb = _recip(jnp.sum(jnp.concatenate([pb, p2], axis=1), axis=1, keepdims=True))
                ctx_s[h, n0:n1, :] = (o[:HB] * la).astype(BF)
                ctx_s[h, n1:n2, :] = ((o[HB:] + o2) * lb).astype(BF)
                return la, lb

            deps.append(normalise if lazy else (lambda v=normalise(): v))
        if lazy:
            deps = [(lambda v=f(): v) for f in deps]
        tail()
        return deps

    nodeps = [lambda: (None, None)] * DIST

    def nop(*_):
        return None

    w_wait(0, 0)
    w_wait(1, 0)
    for j in range(3):
        w_start(j, 2, 1)
    w4_s[...] = _pk(jnp.concatenate([_unpack(z_s[:, 0, i], odd) for odd in (0, 1) for i in (0, 1)], axis=1))

    def kv01(j):
        c = c_s[c_rows(j), :]
        cu_s[c_rows(j, 2), :] = _pk(c)
        kv = jnp.dot(c, _up(w4_s[...]), preferred_element_type=F32)
        for n, dst in enumerate((k0_s, v0_s, k_s, v_s)):
            dst[c_rows(j, 2), :] = _pk(kv[:, n * D:(n + 1) * D].astype(BF))

    c_copy(0).wait()
    kv01(0)
    for_each(1, nc, lambda j: (c_copy(j).wait(), kv01(j)))
    c_copy(nc).wait()
    w_wait(2, 0)
    x_copy(nq - 1, S_Q).wait()
    ln1(nq - 1)
    kv01(nc)
    wq0 = get_wq(0, 0)
    wq1 = get_wq(0, 1)
    q_piece(wq0, (nq - 1) * TQ)
    for j in range(XW, nq - 1):
        x_copy(j, S_XA).wait()

    def pre0(i):
        if i == XW:
            for j in range(XW):
                x_copy(j, S_XB).wait()

    def gap0(i):
        if i != 1:
            q_piece(wq1, i * TQ)
        if i > 0:
            ln1(i - 1)
            q_piece(wq0, (i - 1) * TQ)

    attention(0, k0_s, v0_s, pre0, gap0, lambda: q_piece(wq1, TQ), nodeps, lazy=True)

    def head(h, p, odd, deps):
        wq = get_wq(p, odd)
        wkv = jnp.concatenate([_unpack(z_s[:, p, 0], odd), _unpack(z_s[:, p, 1], odd)], axis=1)

        def gap(i):
            if i > 0:
                q_piece(wq, i * TQ)
            if i + 1 < nq:
                kv_piece(wkv, (i + 1) * TQ)

        def tail():
            kv_piece(wkv, 0)
            q_piece(wq, 0)

        return attention(h, k_s, v_s, nop, gap, tail, deps)

    def two_heads(t):
        p = t + 1

        @pl.when(p == PG[2])
        def _():
            for i in range(3):
                w_wait(i, 2)
            for c in late:
                c.start(priority=1)

        head(2 * t + 2, p, 1, head(2 * t + 1, p, 0, nodeps))

    for i in range(3):
        w_wait(i, 1)
    for_each(0, H // 2 - 1, two_heads)

    late[0].wait()
    late[1].wait()
    wr = wr_s[...].astype(F32).reshape(1, M)

    def post(r0, hv, n, deps, top):
        b1, j1, b2, j2 = top
        for j in range(n // CN - 1, -1, -1):
            rows = pl.ds(r0 + j * CN, CN)
            hf = hv[j * CN:(j + 1) * CN, :].astype(F32)
            hn = _ln_rows(hf, deps.pop(0))
            hnf = hn.astype(F32)
            r = _rb(jnp.sum(hnf * wr, axis=-1, keepdims=True))
            hn_s[rows, :] = hn
            o_s[rows, :] = (hf + hnf).astype(BF)
            deps.append(r)
            tok = lax.broadcasted_iota(jnp.int32, (CN, 1), 0) + (r0 + j * CN)
            ge1 = r >= b1
            ge2 = r >= b2
            b2 = jnp.where(ge1, b1, jnp.where(ge2, r, b2))
            j2 = jnp.where(ge1, j1, jnp.where(ge2, tok, j2))
            b1 = jnp.where(ge1, r, b1)
            j1 = jnp.where(ge1, tok, j1)
        return b1, j1, b2, j2

    def o_proj(r0, n, hv, cols=slice(0, M)):
        rows = pl.ds(r0, n)
        ctx = jnp.concatenate([ctx_s[hh, rows, :] for hh in range(H)], axis=1)
        a = jnp.dot(ctx, wo_s[:, cols], preferred_element_type=F32)
        hv[:, cols] = (x_s[rows, cols].astype(F32) + _rb(a)).astype(BF)

    def o_piece(n):
        o_proj(S - TE, TE, h_s.at[S - TE:S, :], slice(n * (M // nq), (n + 1) * (M // nq)))

    attention(H - 1, k_s, v_s, nop, lambda i: o_piece(i + 1) if i + 1 < nq else None, lambda: o_piece(0), nodeps)

    def epi(t, top):
        i = ne - 1 - (t + 1)
        r0 = pl.multiple_of(i * TE, TE)
        hv = h_s.at[pl.ds(r0, 2 * TE), :]
        top = post(r0 + TE, hv.at[TE:2 * TE, :], TE, [None], top)
        o_proj(r0, TE, hv.at[0:TE, :])
        out_copy(i + 1).start()
        return top

    ninf = jnp.full((CN, 1), -jnp.inf, F32)
    none = jnp.full((CN, 1), S, jnp.int32)
    top = lax.fori_loop(0, ne - 2, epi, (ninf, none, ninf, none))
    for c in late[2:]:
        c.wait()
    deps = [None]
    top = post(TE, h_s.at[TE:2 * TE, :], TE, deps, top)
    o_proj(TB, TE - TB, h_s.at[TB:TE, :])
    out_copy(1).start()
    top = post(TB, h_s.at[TB:TE, :], TE - TB, deps, top)
    o_proj(0, TB, h_s.at[0:TB, :])
    top = post(0, h_s.at[0:TB, :], TB, deps * (TB // CN), top)
    out_copy(0).start()

    r = jnp.concatenate([top[0], top[2]], axis=0)
    idx = jnp.concatenate([top[1], top[3]], axis=0)
    m1 = jnp.max(r, axis=0, keepdims=True)
    i1v = jnp.min(jnp.where(r == m1, idx, S), axis=0, keepdims=True)
    r2 = jnp.where(idx == i1v, -jnp.inf, r)
    m2 = jnp.max(r2, axis=0, keepdims=True)
    i2v = jnp.min(jnp.where((r2 == m2) & (idx != i1v), idx, S), axis=0, keepdims=True)
    i1 = jnp.minimum(jnp.min(i1v), S - 1)
    i2 = jnp.minimum(jnp.min(i2v), S - 1)
    b1 = pl.multiple_of(i1 & (-16), 16)
    b2 = pl.multiple_of(i2 & (-16), 16)
    rows16 = lax.broadcasted_iota(jnp.int32, (16, M), 0)
    hn1 = hn_s[pl.ds(b1, 16), :].astype(F32)
    hn2 = hn_s[pl.ds(b2, 16), :].astype(F32)
    x1 = jnp.sum(jnp.where(rows16 == i1 - b1, hn1, 0.0), axis=0, keepdims=True)
    x2 = jnp.sum(jnp.where(rows16 == i2 - b2, hn2, 0.0), axis=0, keepdims=True)
    xs = jnp.where(rows16 == 0, x1, jnp.where(rows16 == 1, x2, 0.0)).astype(BF)

    g = _rb(jnp.dot(xs, wg_s[...], preferred_element_type=F32)[:8])
    u = _rb(jnp.dot(xs, wu_s[...], preferred_element_type=F32)[:8])
    g = _rb(g * jax.nn.sigmoid(g))
    gu = jnp.concatenate([g * u, jnp.zeros_like(g)], axis=0).astype(BF)
    y = _rb(jnp.dot(gu, wd_s[:, 0:M], preferred_element_type=F32)[:8])
    y1 = _rb(y[0:1, :] * _rb(jax.nn.sigmoid(m1)))
    y2 = _rb(y[1:2, :] * _rb(jax.nn.sigmoid(m2)))

    patch = []
    for n, (b, hnb) in enumerate(((b1, hn1), (b2, hn2))):
        rows = rows16 + b
        upd = jnp.where(rows == i1, y1, jnp.where(rows == i2, y2, 0.0))
        p_s[n] = (h_s[pl.ds(b, 16), :].astype(F32) + _rb(hnb + upd)).astype(BF)
        patch.append(pltpu.make_async_copy(p_s.at[n], out_hbm.at[pl.ds(b, 16), :], sem.at[n]))
    pltpu.make_async_copy(o_s, out_hbm, sem.at[S_OUT]).wait()
    patch[0].start()

    @pl.when(b1 != b2)
    def _():
        patch[1].start()
        patch[1].wait()
    patch[0].wait()


@jax.jit
def pallas_sequential_preLN__compressed_kv_cla__moe_arch_mod__prompt_kernel(
        A_x, A_c_kv, A_w_q, A_w_uk, A_w_uv, A_w_o, B_x, B_w_r, B_w_gate, B_w_up, B_w_down):
    del B_x
    B, S, M = A_x.shape
    C = A_c_kv.shape[2]
    _, H, D = A_w_q.shape
    Fd = B_w_gate.shape[1]
    assert B == 1 and A_c_kv.shape[1] == S and M == 2 * C
    vmem = pltpu.VMEM
    anyspec = pl.BlockSpec(memory_space=pl.ANY)
    out = pl.pallas_call(
        _kernel,
        in_specs=[anyspec] * 10,
        out_specs=anyspec,
        out_shape=jax.ShapeDtypeStruct((S, M), BF),
        scratch_shapes=[
            vmem((S, M), BF), vmem((S, C), BF), vmem((S // 2, C), U32),
            vmem((C // 8, H // 2, 4, 16, D), BF),
            vmem((H * D, M + 128), BF),
            vmem((M, Fd), BF), vmem((M, Fd), BF), vmem((Fd, M + 128), BF), vmem((M,), BF),
            vmem((S // 2, M), U32),
            vmem((S, D), BF), vmem((S // 2, D), U32), vmem((S // 2, D), U32),
            vmem((S // 2, D), U32), vmem((S // 2, D), U32), vmem((C // 2, 4 * D), U32),
            vmem((H, S, D), BF),
            vmem((S, M), BF), vmem((S, M), BF), vmem((S, M), BF),
            vmem((2, 16, M), BF),
            pltpu.SemaphoreType.DMA((6 + S // TC,)),
        ],
        compiler_params=pltpu.CompilerParams(vmem_limit_bytes=120 * 1024 * 1024),
    )(A_x.reshape(S, M), A_c_kv.reshape(S, C),
      A_w_q.reshape(C // 8, 2, 8, H // 2, 2, D), A_w_uk.reshape(C // 8, 8, H // 2, 2, D),
      A_w_uv.reshape(C // 8, 8, H // 2, 2, D), A_w_o.reshape(H * D, M),
      B_w_r, B_w_gate, B_w_up, B_w_down)
    return out.reshape(B, S, M)
```

```python
import math

import jax
import jax.numpy as jnp
from jax import lax
from jax.experimental import pallas as pl
from jax.experimental.pallas import tpu as pltpu

BF = jnp.bfloat16
F32 = jnp.float32
U32 = jnp.uint32
NT = (((1,), (1,)), ((), ()))
NEG = -1e30
EPS = 1e-5
BIG = 3e38

TQ = 256
TC = 512
TE = 256
TB = 64
CN = 16
XW = 5
DIST = 2


def _rb(x):
    return x.astype(BF).astype(F32)


def _after(x, dep):
    return x if dep is None else jnp.maximum(x, dep - BIG)


def _recip(l):
    r = pl.reciprocal(l, approx=True)
    return r * (2.0 - l * r)


def _ln_rows(x, dep):
    n = x.shape[-1]
    mu = _after(jnp.sum(x, axis=-1, keepdims=True), dep) * (1.0 / n)
    xc = x - mu
    var = jnp.sum(xc * xc, axis=-1, keepdims=True) * (1.0 / n)
    den = _rb(jnp.sqrt(_rb(_rb(var) + EPS)))
    num = _rb(x - _rb(mu))
    return (num * (1.0 / den)).astype(BF)


def _unpack(z, odd):
    u = pltpu.bitcast(z, U32)
    u = u.reshape(u.shape[0] * u.shape[1], u.shape[2])
    u = (u & jnp.uint32(0xFFFF0000)) if odd else (u << 16)
    return pltpu.bitcast(u, F32).astype(BF)


def _pk(x):
    return pltpu.bitcast(x, U32)


def _up(u):
    return pltpu.bitcast(u, BF)


def _kernel(x_hbm, c_hbm, wq_hbm, wk_hbm, wv_hbm, wo_hbm, wr_hbm, wg_hbm, wu_hbm, wd_hbm,
            out_hbm,
            x_s, c_s, cu_s, z_s, wo_s, wg_s, wu_s, wd_s, wr_s,
            xn_s, q_s, k_s, v_s, k0_s, v0_s, w4_s, ctx_s, h_s, hn_s, o_s, p_s,
            sem):
    S, M = x_s.shape
    H, _, D = ctx_s.shape
    nq = S // TQ
    ne = S // TE
    nc = S // TC
    scale = (D ** -0.5) * math.log2(math.e)
    PG = (0, 1, 2, H // 2)

    S_KV, S_XA, S_XB, S_G1, S_G2, S_Q, S_C = range(7)
    S_XL = S_C + nc
    S_WO, S_FFN, S_OUT = S_KV, S_XA, S_XB

    def w_sem(i, g):
        return sem.at[(S_KV if i < 2 else S_Q, S_G1, S_G2)[g]]

    def w_start(i, g, priority):
        lo, hi = PG[g], PG[g + 1]
        for r in range(8):
            two = slice(2 * r, 2 * r + 2)
            if i < 2:
                cps = [((wk_hbm, wv_hbm)[i].at[:, r, lo:hi], z_s.at[:, lo:hi, i, two, :])]
            elif hi - lo == 1:
                cps = [(wq_hbm.at[:, :, r, lo], z_s.at[:, lo, 2:4, two, :])]
            else:
                cps = [(wq_hbm.at[:, b, r, lo:hi], z_s.at[:, lo:hi, 2 + b, two, :]) for b in range(2)]
            for src, dst in cps:
                pltpu.make_async_copy(src, dst, w_sem(i, g)).start(priority=priority)

    def w_wait(g, lo=0, hi=4):
        z = z_s.at[:, PG[g]:PG[g + 1], lo:hi]
        pltpu.make_async_copy(z, z, w_sem(lo, g)).wait()

    def x_copy(i, s):
        rows = pl.ds(pl.multiple_of(i * TQ, TQ), TQ)
        return pltpu.make_async_copy(x_hbm.at[rows, :], x_s.at[rows, :], sem.at[s])

    def c_rows(i, div=1):
        t = TC // div
        if isinstance(i, int):
            assert i in (0, nc)
            return pl.ds(0 if i == 0 else S // div - t // 2, t // 2)
        return pl.ds(pl.multiple_of(i * t - t // 2, t // 2), t)

    def c_copy(i):
        return pltpu.make_async_copy(c_hbm.at[c_rows(i), :], c_s.at[c_rows(i), :], sem.at[S_C + i])

    def out_copy(i):
        rows = pl.ds(pl.multiple_of(i * TE, TE), TE)
        return pltpu.make_async_copy(o_s.at[rows, :], out_hbm.at[rows, :], sem.at[S_OUT])

    late = [pltpu.make_async_copy(src, dst, sem.at[S_WO if i < 2 else S_FFN]) for i, (src, dst) in enumerate([
        (wo_hbm, wo_s.at[:, 0:M]), (wr_hbm, wr_s), (wg_hbm, wg_s), (wu_hbm, wu_s), (wd_hbm, wd_s.at[:, 0:M])])]

    def for_each(lo, hi, fn):
        def body(i, c):
            fn(i)
            return c
        lax.fori_loop(lo, hi, body, 0)

    w_start(0, 0, 0)
    w_start(1, 0, 0)
    c_copy(0).start()
    for_each(1, nc, lambda j: c_copy(j).start())
    c_copy(nc).start()
    w_start(2, 0, 0)
    x_copy(nq - 1, S_XL).start()
    for_each(XW, nq - 1, lambda j: x_copy(j, S_XA).start())
    for_each(0, XW, lambda j: x_copy(j, S_XB).start())
    for j in range(3):
        w_start(j, 1, 0)

    def get_wq(p, odd):
        z = z_s[:, p, 2:4]
        return _unpack(z.reshape(2 * z.shape[0], 16, D), odd)

    def kv_piece(wkv, r0):
        rows = slice(r0 // 2, (r0 + TQ) // 2)
        kv = jnp.dot(_up(cu_s[rows, :]), wkv, preferred_element_type=F32)
        k_s[rows, :] = _pk(kv[:, :D].astype(BF))
        v_s[rows, :] = _pk(kv[:, D:].astype(BF))

    def q_piece(wq, r0):
        rows = slice(r0 // 2, (r0 + TQ) // 2)
        q = jnp.dot(_up(xn_s[rows, :]), wq, preferred_element_type=F32)
        q_s[r0:r0 + TQ, :] = (q * scale).astype(BF)

    def ln1(i):
        for j in range(TQ // CN):
            r0 = i * TQ + j * CN
            x = x_s[r0:r0 + CN, :].astype(F32)
            xc = x - jnp.sum(x, axis=-1, keepdims=True) * (1.0 / M)
            var = jnp.sum(xc * xc, axis=-1, keepdims=True) * (1.0 / M)
            xn_s[r0 // 2:(r0 + CN) // 2, :] = _pk((xc * lax.rsqrt(var + EPS)).astype(BF))

    def attention(h, kr, vr, pre, gap, tail, deps, lazy=False):
        HB = TQ // 2
        row = lax.broadcasted_iota(jnp.int32, (HB, HB), 0)
        col = lax.broadcasted_iota(jnp.int32, (HB, HB), 1)
        tri = col <= row
        deps = list(deps)
        for i in range(nq - 1, -1, -1):
            n0 = i * TQ
            n1 = n0 + HB
            n2 = n0 + TQ
            pre(i)
            q = q_s[n0:n2, :]
            s = lax.dot_general(q, _up(kr[:n1 // 2, :]), NT, preferred_element_type=F32)
            s2 = lax.dot_general(q[HB:], _up(kr[n1 // 2:n2 // 2, :]), NT, preferred_element_type=F32)
            gap(i)
            sa = jnp.where(tri, s[:HB, n0:], NEG)
            sa = jnp.concatenate([s[:HB, :n0], sa], axis=1) if i > 0 else sa
            sb = s[HB:]
            s2 = jnp.where(tri, s2, NEG)
            da, db = deps.pop(0)()
            ma = _after(jnp.max(sa, axis=1, keepdims=True), da)
            mb = _after(jnp.max(jnp.concatenate([sb, s2], axis=1), axis=1, keepdims=True), db)
            pa = jnp.exp2(sa - ma)
            pb = jnp.exp2(sb - mb)
            p2 = jnp.exp2(s2 - mb)
            p = jnp.concatenate([pa, pb], axis=0).astype(BF)
            o = jnp.dot(p, _up(vr[:n1 // 2, :]), preferred_element_type=F32)
            o2 = jnp.dot(p2.astype(BF), _up(vr[n1 // 2:n2 // 2, :]), preferred_element_type=F32)

            def normalise(pa=pa, pb=pb, p2=p2, o=o, o2=o2, n0=n0, n1=n1, n2=n2):
                la = _recip(jnp.sum(pa, axis=1, keepdims=True))
                lb = _recip(jnp.sum(jnp.concatenate([pb, p2], axis=1), axis=1, keepdims=True))
                ctx_s[h, n0:n1, :] = (o[:HB] * la).astype(BF)
                ctx_s[h, n1:n2, :] = ((o[HB:] + o2) * lb).astype(BF)
                return la, lb

            deps.append(normalise if lazy else (lambda v=normalise(): v))
        if lazy:
            deps = [(lambda v=f(): v) for f in deps]
        tail()
        return deps

    nodeps = [lambda: (None, None)] * DIST

    def nop(*_):
        return None

    w_wait(0, 0, 2)
    for j in range(3):
        w_start(j, 2, 1)
    w4_s[...] = _pk(jnp.concatenate([_unpack(z_s[:, 0, i], odd) for odd in (0, 1) for i in (0, 1)], axis=1))

    def kv01(j):
        c = c_s[c_rows(j), :]
        cu_s[c_rows(j, 2), :] = _pk(c)
        kv = jnp.dot(c, _up(w4_s[...]), preferred_element_type=F32)
        for n, dst in enumerate((k0_s, v0_s, k_s, v_s)):
            dst[c_rows(j, 2), :] = _pk(kv[:, n * D:(n + 1) * D].astype(BF))

    c_copy(0).wait()
    kv01(0)
    for_each(1, nc, lambda j: (c_copy(j).wait(), kv01(j)))
    c_copy(nc).wait()
    w_wait(0, 2, 4)
    x_copy(nq - 1, S_XL).wait()
    ln1(nq - 1)
    kv01(nc)
    wq0 = get_wq(0, 0)
    wq1 = get_wq(0, 1)
    q_piece(wq0, (nq - 1) * TQ)
    for j in range(XW, nq - 1):
        x_copy(j, S_XA).wait()

    def pre0(i):
        if i == XW:
            for j in range(XW):
                x_copy(j, S_XB).wait()

    def gap0(i):
        if i != 1:
            q_piece(wq1, i * TQ)
        if i > 0:
            ln1(i - 1)
            q_piece(wq0, (i - 1) * TQ)

    attention(0, k0_s, v0_s, pre0, gap0, lambda: q_piece(wq1, TQ), nodeps, lazy=True)

    def head(h, p, odd, deps):
        wq = get_wq(p, odd)
        wkv = jnp.concatenate([_unpack(z_s[:, p, 0], odd), _unpack(z_s[:, p, 1], odd)], axis=1)

        def gap(i):
            if i > 0:
                q_piece(wq, i * TQ)
            if i + 1 < nq:
                kv_piece(wkv, (i + 1) * TQ)

        def tail():
            kv_piece(wkv, 0)
            q_piece(wq, 0)

        return attention(h, k_s, v_s, nop, gap, tail, deps)

    def two_heads(t):
        p = t + 1

        @pl.when(p == PG[2])
        def _():
            w_wait(2)
            for c in late:
                c.start(priority=1)

        head(2 * t + 2, p, 1, head(2 * t + 1, p, 0, nodeps))

    w_wait(1)
    for_each(0, H // 2 - 1, two_heads)

    late[0].wait()
    late[1].wait()
    wr = wr_s[...].astype(F32).reshape(1, M)

    def post(r0, hv, n, deps, top):
        b1, j1, b2, j2 = top
        for j in range(n // CN - 1, -1, -1):
            rows = pl.ds(r0 + j * CN, CN)
            hf = hv[j * CN:(j + 1) * CN, :].astype(F32)
            hn = _ln_rows(hf, deps.pop(0))
            hnf = hn.astype(F32)
            r = _rb(jnp.sum(hnf * wr, axis=-1, keepdims=True))
            hn_s[rows, :] = hn
            o_s[rows, :] = (hf + hnf).astype(BF)
            deps.append(r)
            tok = lax.broadcasted_iota(jnp.int32, (CN, 1), 0) + (r0 + j * CN)
            ge1 = r >= b1
            ge2 = r >= b2
            b2 = jnp.where(ge1, b1, jnp.where(ge2, r, b2))
            j2 = jnp.where(ge1, j1, jnp.where(ge2, tok, j2))
            b1 = jnp.where(ge1, r, b1)
            j1 = jnp.where(ge1, tok, j1)
        return b1, j1, b2, j2

    def o_proj(r0, n, hv, cols=slice(0, M)):
        rows = pl.ds(r0, n)
        ctx = jnp.concatenate([ctx_s[hh, rows, :] for hh in range(H)], axis=1)
        a = jnp.dot(ctx, wo_s[:, cols], preferred_element_type=F32)
        hv[:, cols] = (x_s[rows, cols].astype(F32) + _rb(a)).astype(BF)

    def o_piece(n):
        o_proj(S - TE, TE, h_s.at[S - TE:S, :], slice(n * (M // nq), (n + 1) * (M // nq)))

    attention(H - 1, k_s, v_s, nop, lambda i: o_piece(i + 1) if i + 1 < nq else None, lambda: o_piece(0), nodeps)

    def epi(t, top):
        i = ne - 1 - (t + 1)
        r0 = pl.multiple_of(i * TE, TE)
        hv = h_s.at[pl.ds(r0, 2 * TE), :]
        top = post(r0 + TE, hv.at[TE:2 * TE, :], TE, [None], top)
        o_proj(r0, TE, hv.at[0:TE, :])
        out_copy(i + 1).start()
        return top

    ninf = jnp.full((CN, 1), -jnp.inf, F32)
    none = jnp.full((CN, 1), S, jnp.int32)
    top = lax.fori_loop(0, ne - 2, epi, (ninf, none, ninf, none))
    for c in late[2:]:
        c.wait()
    deps = [None]
    top = post(TE, h_s.at[TE:2 * TE, :], TE, deps, top)
    o_proj(TB, TE - TB, h_s.at[TB:TE, :])
    out_copy(1).start()
    top = post(TB, h_s.at[TB:TE, :], TE - TB, deps, top)
    o_proj(0, TB, h_s.at[0:TB, :])
    top = post(0, h_s.at[0:TB, :], TB, deps * (TB // CN), top)
    out_copy(0).start()

    r = jnp.concatenate([top[0], top[2]], axis=0)
    idx = jnp.concatenate([top[1], top[3]], axis=0)
    m1 = jnp.max(r, axis=0, keepdims=True)
    i1v = jnp.min(jnp.where(r == m1, idx, S), axis=0, keepdims=True)
    r2 = jnp.where(idx == i1v, -jnp.inf, r)
    m2 = jnp.max(r2, axis=0, keepdims=True)
    i2v = jnp.min(jnp.where((r2 == m2) & (idx != i1v), idx, S), axis=0, keepdims=True)
    i1 = jnp.minimum(jnp.min(i1v), S - 1)
    i2 = jnp.minimum(jnp.min(i2v), S - 1)
    b1 = pl.multiple_of(i1 & (-16), 16)
    b2 = pl.multiple_of(i2 & (-16), 16)
    rows16 = lax.broadcasted_iota(jnp.int32, (16, M), 0)
    hn1 = hn_s[pl.ds(b1, 16), :].astype(F32)
    hn2 = hn_s[pl.ds(b2, 16), :].astype(F32)
    x1 = jnp.sum(jnp.where(rows16 == i1 - b1, hn1, 0.0), axis=0, keepdims=True)
    x2 = jnp.sum(jnp.where(rows16 == i2 - b2, hn2, 0.0), axis=0, keepdims=True)
    xs = jnp.where(rows16 == 0, x1, jnp.where(rows16 == 1, x2, 0.0)).astype(BF)

    g = _rb(jnp.dot(xs, wg_s[...], preferred_element_type=F32)[:8])
    u = _rb(jnp.dot(xs, wu_s[...], preferred_element_type=F32)[:8])
    g = _rb(g * jax.nn.sigmoid(g))
    gu = jnp.concatenate([g * u, jnp.zeros_like(g)], axis=0).astype(BF)
    y = _rb(jnp.dot(gu, wd_s[:, 0:M], preferred_element_type=F32)[:8])
    y1 = _rb(y[0:1, :] * _rb(jax.nn.sigmoid(m1)))
    y2 = _rb(y[1:2, :] * _rb(jax.nn.sigmoid(m2)))

    patch = []
    for n, (b, hnb) in enumerate(((b1, hn1), (b2, hn2))):
        rows = rows16 + b
        upd = jnp.where(rows == i1, y1, jnp.where(rows == i2, y2, 0.0))
        p_s[n] = (h_s[pl.ds(b, 16), :].astype(F32) + _rb(hnb + upd)).astype(BF)
        patch.append(pltpu.make_async_copy(p_s.at[n], out_hbm.at[pl.ds(b, 16), :], sem.at[n]))
    pltpu.make_async_copy(o_s, out_hbm, sem.at[S_OUT]).wait()
    patch[0].start()

    @pl.when(b1 != b2)
    def _():
        patch[1].start()
        patch[1].wait()
    patch[0].wait()


@jax.jit
def pallas_sequential_preLN__compressed_kv_cla__moe_arch_mod__prompt_kernel(
        A_x, A_c_kv, A_w_q, A_w_uk, A_w_uv, A_w_o, B_x, B_w_r, B_w_gate, B_w_up, B_w_down):
    del B_x
    B, S, M = A_x.shape
    C = A_c_kv.shape[2]
    _, H, D = A_w_q.shape
    Fd = B_w_gate.shape[1]
    assert B == 1 and A_c_kv.shape[1] == S and M == 2 * C
    vmem = pltpu.VMEM
    anyspec = pl.BlockSpec(memory_space=pl.ANY)
    out = pl.pallas_call(
        _kernel,
        in_specs=[anyspec] * 10,
        out_specs=anyspec,
        out_shape=jax.ShapeDtypeStruct((S, M), BF),
        scratch_shapes=[
            vmem((S, M), BF), vmem((S, C), BF), vmem((S // 2, C), U32),
            vmem((C // 8, H // 2, 4, 16, D), BF),
            vmem((H * D, M + 128), BF),
            vmem((M, Fd), BF), vmem((M, Fd), BF), vmem((Fd, M + 128), BF), vmem((M,), BF),
            vmem((S // 2, M), U32),
            vmem((S, D), BF), vmem((S // 2, D), U32), vmem((S // 2, D), U32),
            vmem((S // 2, D), U32), vmem((S // 2, D), U32), vmem((C // 2, 4 * D), U32),
            vmem((H, S, D), BF),
            vmem((S, M), BF), vmem((S, M), BF), vmem((S, M), BF),
            vmem((2, 16, M), BF),
            pltpu.SemaphoreType.DMA((7 + S // TC,)),
        ],
        compiler_params=pltpu.CompilerParams(vmem_limit_bytes=120 * 1024 * 1024),
    )(A_x.reshape(S, M), A_c_kv.reshape(S, C),
      A_w_q.reshape(C // 8, 2, 8, H // 2, 2, D), A_w_uk.reshape(C // 8, 8, H // 2, 2, D),
      A_w_uv.reshape(C // 8, 8, H // 2, 2, D), A_w_o.reshape(H * D, M),
      B_w_r, B_w_gate, B_w_up, B_w_down)
    return out.reshape(B, S, M)
```
